```python
import jax
import jax.numpy as jnp

def _softmax(x, axis=-1):
    return jax.nn.softmax(x, axis=axis)
def _gelu(x):
    return jax.nn.gelu(x, approximate=True)
def _silu(x):
    return jax.nn.silu(x)
def _sigmoid(x):
    return jax.nn.sigmoid(x)
def _layernorm(x, axis=-1, eps=1e-5):
    m = jnp.mean(x, axis=axis, keepdims=True)
    v = jnp.var(x, axis=axis, keepdims=True)
    return (x - m) / jnp.sqrt(v + eps)
def _scatter_add(tgt, idx, src, axis=0):
    return tgt.at[idx].add(src)
def _segment_sum(src, seg, n):
    return jax.ops.segment_sum(src, seg, n)
class _Rng:
    def __init__(self, key):
        self._k = key
    def _next(self):
        self._k, sub = jax.random.split(self._k)
        return sub
    def normal(self, shape):
        return jax.random.normal(self._next(), shape, dtype=jnp.bfloat16)
    def randint(self, lo, hi, shape):
        return jax.random.randint(self._next(), shape, lo, hi, dtype=jnp.int32)
    def uniform(self, shape, lo=0.0, hi=1.0):
        return jax.random.uniform(self._next(), shape, jnp.bfloat16, lo, hi)
    def permutation(self, n):
        return jax.random.permutation(self._next(), n)


kernel_name = 'interleave_layers__sliding_local_dilated__dense_activation_squared_relu__prompt'

def setup_inputs():
    _rng = _Rng(jax.random.key(int.from_bytes(__import__("os").urandom(4), "little")))
    _w = (lambda a: (lambda t: t.astype(jnp.bfloat16) if jnp.issubdtype(t.dtype, jnp.floating) else t)(jnp.asarray(a)))
    def _A_setup():
        B, S, D = 1, 2048, 1024
        return {
            "x": _w((lambda *s: _rng.normal(s) * 0.05)(B, S, D)),
            "wqkv": _w((lambda *s: _rng.normal(s) * 0.05)(D, 3 * D)),
            "wo": _w((lambda *s: _rng.normal(s) * 0.05)(D, D)),
        }
    _A_in = _A_setup()

    def _B_setup():
        B, S, D, F = 1, 2048, 1024, 3584
        return {
            "x": _w((lambda *s: _rng.normal(s) * 0.05)(B, S, D)),
            "w1": _w((lambda *s: _rng.normal(s) * 0.05)(D, F)),
            "b1": _w((lambda *s: _rng.normal(s) * 0.05)(F)),
            "w2": _w((lambda *s: _rng.normal(s) * 0.05)(F, D)),
            "b2": _w((lambda *s: _rng.normal(s) * 0.05)(D)),
        }
    _B_in = _B_setup()

    return {
        "A_x": _A_in["x"],
        "A_wqkv": _A_in["wqkv"],
        "A_wo": _A_in["wo"],
        "B_x": _B_in["x"],
        "B_w1": _B_in["w1"],
        "B_b1": _B_in["b1"],
        "B_w2": _B_in["w2"],
        "B_b2": _B_in["b2"],
    }

def reference(A_x, A_wqkv, A_wo, B_x, B_w1, B_b1, B_w2, B_b2):
    def _A_ref(x, wqkv, wo):
        B, S, D = x.shape
        H = 32; Dh = D // H
        W, dil = 8, 2
        qkv = (lambda x, *d: x.transpose(*d))((x @ wqkv).reshape(B, S, 3, H, Dh), 2, 0, 3, 1, 4)
        q, k, v = qkv[0], qkv[1], qkv[2]
        scale = Dh ** -0.5
        pos = jnp.arange(S)
        off = jnp.arange(W) * dil
        idx = pos[:, None] - off[None, :]
        mask = idx >= 0
        idx_c = jnp.where(mask, idx, 0).reshape(-1)
        kg = k[:, :, idx_c, :].reshape(B, H, S, W, Dh)
        vg = v[:, :, idx_c, :].reshape(B, H, S, W, Dh)
        logits = jnp.einsum("bhsd,bhswd->bhsw", q, kg) * scale
        logits = jnp.where(mask[None, None, :, :], logits, -1e9)
        attn = _softmax(logits, axis=-1)
        o = jnp.einsum("bhsw,bhswd->bhsd", attn, vg)
        return (lambda x, *d: x.transpose(*d))(o, 0, 2, 1, 3).reshape(B, S, D) @ wo

    def _B_ref(x, w1, b1, w2, b2):
        h = jnp.einsum("bsd,df->bsf", x, w1) + b1
        zero = jnp.zeros_like(h)
        r = jnp.where(h > zero, h, zero)
        h = r * r
        out = jnp.einsum("bsf,fd->bsd", h, w2) + b2
        return out

    x = A_x
    x = x + _A_ref(_layernorm(x, axis=-1), A_wqkv, A_wo)
    x = x + _B_ref(_layernorm(x, axis=-1), B_w1, B_b1, B_w2, B_b2)
    x = x + _A_ref(_layernorm(x, axis=-1), A_wqkv, A_wo)
    x = x + _B_ref(_layernorm(x, axis=-1), B_w1, B_b1, B_w2, B_b2)
    return x
```

```python
import jax
import jax.numpy as jnp
import numpy as np
from jax import lax
from jax.experimental import pallas as pl
from jax.experimental.pallas import tpu as pltpu

S, D, F = 2048, 1024, 3584
H, DH, W, DIL = 32, 32, 8, 2
HALO = 16
NC = D // 128
NF = F // 128
EPS = 1e-5
TINY = 1e-36
SCALE = DH ** -0.5
NEG = -1e9
T = 256
TH = T // 2
NT = S // T
SKEW = 3

f32 = jnp.float32
bf16 = jnp.bfloat16
u32 = jnp.uint32
DN = (((1,), (0,)), ((), ()))


def _pack(x):
    return pltpu.bitcast(x.astype(bf16), u32)


def _unpack(u):
    return pltpu.bitcast(u, bf16)


class Phase:
    def __init__(self, n, gen):
        self.n, self.gen = n, gen


def phase(n):
    def deco(f):
        return lambda *a: Phase(n, f(*a))
    return deco


def chain(*ps):
    def g():
        for p in ps:
            yield from p.gen
    return Phase(sum(p.n for p in ps), g())


def make(GATE=1, CS=8, CM=8, LEAD=2, MARGIN=24, KSPLIT=0, flags=None, NJ=None):
    def kernel(x_hbm, wqkv_hbm, wo_hbm, w1_hbm, b1_ref, w2_hbm, b2_ref, o_hbm,
               xb, wraw, wtmp, woraw, wou, w1raw, w2raw,
               wq7, wk7, wv7, wo7, w17, w27, bias,
               xa7, xb7, xf7, o7, o7b, h7, sa, sb, sf, so, sob, sh,
               tx, tix, to, tio, th, tih, tss,
               qa, qb, kk, vv, pp, zero_ref,
               sem_x, sem_w, sem_o):
        def x_copy(t):
            return pltpu.make_async_copy(x_hbm.at[pl.ds(t * T, T)], xb.at[pl.ds(t * T, T)], sem_x.at[t])

        def o_copy(t):
            return pltpu.make_async_copy(xb.at[pl.ds(t * T, T)], o_hbm.at[pl.ds(t * T, T)], sem_o.at[t])

        def wqkv_copy(i):
            return pltpu.make_async_copy(wqkv_hbm.at[:, pl.ds(i * D, D)], wraw.at[i], sem_w.at[i])

        wo_copy = pltpu.make_async_copy(wo_hbm, woraw, sem_w.at[3])
        w1_copy = pltpu.make_async_copy(w1_hbm, w1raw, sem_w.at[4])
        w2_copy = pltpu.make_async_copy(w2_hbm, w2raw, sem_w.at[5])

        x_copy(0).start()
        wqkv_copy(0).start()
        x_copy(1).start()
        wqkv_copy(1).start()
        wqkv_copy(2).start()
        wo_copy.start()
        x_copy(2).start()
        w1_copy.start()
        x_copy(3).start()
        w2_copy.start()
        for t in range(4, NT):
            x_copy(t).start()

        bias[0:NF, :] = b1_ref[...].astype(f32)
        bias[32:32 + NC, :] = b2_ref[...].astype(f32)
        zero_ref[...] = jnp.zeros((8, 128), u32)

        fresh = []
        tok = [None]

        def gate(*xs):
            if tok[0] is None:
                return xs
            z = pltpu.bitcast(tok[0], u32) & zero_ref[...]
            out = []
            for x in xs:
                u = pltpu.bitcast(x, u32)
                out.append(pltpu.bitcast(u | jnp.tile(z, (u.shape[0] // 8, u.shape[1] // 128)), x.dtype))
            return out

        def run(main, *side, lead=LEAD):
            side = chain(*side)
            slots = max(main.n - lead, 1)
            done = 0
            for i in range(main.n):
                del fresh[:]
                next(main.gen)
                toks = [y[r:r + 8, c:c + 128] for y in fresh for c in range(0, y.shape[1], 128)
                        for r in range(0, y.shape[0], 8)]
                want = min(side.n, -(-side.n * (i + 1) // slots))
                k = want - done
                for j in range(k):
                    tok[0] = toks[j * len(toks) // k] if (toks and GATE) else None
                    next(side.gen)
                done = want
            tok[0] = None
            for p in (main, side):
                for _ in p.gen:
                    raise AssertionError("piece count mismatch")

        def store_b7(dst, prow, col, u11, u12, u21, u22):
            b11, b12, b21, b22 = (_unpack(u).astype(f32) for u in (u11, u12, u21, u22))
            at = (pl.ds(prow, 8), pl.ds(col, 128))
            dst[(0,) + at] = _pack(b11 + b22)
            dst[(1,) + at] = u11
            dst[(2,) + at] = _pack(b12 - b22)
            dst[(3,) + at] = _pack(b21 - b11)
            dst[(4,) + at] = u22
            dst[(5,) + at] = _pack(b11 + b12)
            dst[(6,) + at] = _pack(b21 + b22)

        def combine_pieces(src, inv, dst):
            nk = src.shape[0] // 2
            for r in range(0, TH, 16):
                it = inv[r:r + 16, :]
                ib = inv[TH + r:TH + r + 16, :]
                for j in range(nk):
                    it, ib = gate(it, ib) if j % 2 == 0 else (it, ib)
                    a11 = src[j, r:r + 16, :] * it
                    a12 = src[nk + j, r:r + 16, :] * it
                    a21 = src[j, TH + r:TH + r + 16, :] * ib
                    a22 = src[nk + j, TH + r:TH + r + 16, :] * ib
                    at = (slice(r // 2, r // 2 + 8), slice(j * 128, (j + 1) * 128))
                    dst[(0,) + at] = _pack(a11 + a22)
                    dst[(1,) + at] = _pack(a21 + a22)
                    dst[(2,) + at] = _pack(a11)
                    dst[(3,) + at] = _pack(a22)
                    dst[(4,) + at] = _pack(a11 + a12)
                    dst[(5,) + at] = _pack(a21 - a11)
                    dst[(6,) + at] = _pack(a12 - a22)
                    yield

        def smm(a7, b7, j, emit):
            cols = slice(j * 128, (j + 1) * 128)
            kh = a7.shape[2]

            def m(i):
                step = KSPLIT if KSPLIT else kh
                y = None
                for k in range(0, kh, step):
                    ke = min(k + step, kh)
                    yk = lax.dot_general(_unpack(a7[i, :, k:ke]), _unpack(b7[i, k // 2:ke // 2, cols]), DN,
                                         preferred_element_type=f32)
                    fresh.append(yk)
                    y = yk if y is None else y + yk
                return y

            nh = b7.shape[2] // 128
            m1 = m(0)
            m2 = m(1)
            c22 = m1 - m2
            m4 = m(3)
            emit(1, j, m2 + m4)
            c11 = m1 + m4
            c11 = c11 + m(6)
            m5 = m(4)
            emit(0, j, c11 - m5)
            m3 = m(2)
            emit(0, nh + j, m3 + m5)
            c22 = c22 + m3
            emit(1, nh + j, c22 + m(5))

        @phase(D // 64 + NC // 2)
        def prep_qkv(i, dst, G=4):
            lane8 = lax.broadcasted_iota(jnp.int32, (8, 128), 1)
            bits = [(lane8 & (1 << b)) != 0 for b in range(3)]
            for g0 in range(0, D // 16, G):
                xs = [[None] * NC for _ in range(G)]
                for c in range(NC):
                    for g in range(G):
                        u = pltpu.bitcast(wraw[i, (g0 + g) * 16:(g0 + g + 1) * 16, c * 128:(c + 1) * 128], u32)
                        xs[g][c] = pltpu.roll(u, c, 1) if c else u
                for g in range(G):
                    ws = [xs[g][(-c) % NC] for c in range(NC)]
                    for b in range(3):
                        ws = [jnp.where(bits[b], ws[(c - (1 << b)) % NC], ws[c]) for c in range(NC)]
                    for c in range(NC):
                        wtmp[c, (g0 + g) * 8:(g0 + g + 1) * 8, :] = ws[c]
                yield
            lane = lax.broadcasted_iota(jnp.int32, (64, 128), 1)
            base = (lane & 3) * 32 + (lane >> 5) * 8 + ((lane >> 2) & 7)
            for j in range(NC // 2):
                for c in (j, NC // 2 + j):
                    gidx = (base + c) & 127
                    for r in range(0, D // 2, 64):
                        wtmp[c, r:r + 64, :] = jnp.take_along_axis(wtmp[c, r:r + 64, :], gidx, axis=1)
                for r in range(0, D // 4, 8):
                    store_b7(dst, r, j * 128,
                             wtmp[j, r:r + 8, :], wtmp[NC // 2 + j, r:r + 8, :],
                             wtmp[j, D // 4 + r:D // 4 + r + 8, :], wtmp[NC // 2 + j, D // 4 + r:D // 4 + r + 8, :])
                yield

        @phase(NC + NC * NC // 4)
        def prep_o():
            for n in range(NC):
                wou[n] = pltpu.bitcast(woraw[:, n * 128:(n + 1) * 128], u32)
                yield

            def rows16(n, cp, a):
                st = ((16 * (a % 2)) * 32 + (a // 2) * 8) // 2 + cp
                lo = wou[n, pl.ds(st, 8, stride=32), :]
                hi = wou[n, pl.ds(st + 16, 8, stride=32), :]
                return (lo & u32(0xFFFF)) | (hi << 16), (lo >> 16) | (hi & u32(0xFFFF0000))

            for j in range(NC // 2):
                for cp in range(NC // 4):
                    for a in range(8):
                        u11, u12 = rows16(j, cp, a), rows16(NC // 2 + j, cp, a)
                        u21, u22 = rows16(j, NC // 4 + cp, a), rows16(NC // 2 + j, NC // 4 + cp, a)
                        for par in range(2):
                            store_b7(wo7, (2 * cp + par) * 64 + 8 * a, j * 128, u11[par], u12[par], u21[par], u22[par])
                    yield
                    yield

        def prep_plain_pieces(raw, dst):
            kh, nh = raw.shape[0] // 2, raw.shape[1] // 2
            for r in range(0, kh, 16):
                for c in range(0, nh, 128):
                    q = [pltpu.bitcast(raw[r0:r0 + 16, c0:c0 + 128], u32)
                         for r0 in (r, kh + r) for c0 in (c, nh + c)]
                    store_b7(dst, r // 2, c, *q)
                yield

        @phase(D // 32)
        def prep_1():
            yield from prep_plain_pieces(w1raw, w17)

        @phase(F // 32)
        def prep_2():
            yield from prep_plain_pieces(w2raw, w27)

        @phase(T // 16 + TH // 16 * NC // 2)
        def ln_tile(row, a7, s_ref):
            for r in range(0, T, 16):
                xu, = gate(xb[pl.ds(pl.multiple_of(row + r, 16), 16), :])
                x = xu.astype(f32)
                m = jnp.sum(x, axis=-1, keepdims=True) * (1.0 / D)
                xc = x - m
                for c in range(NC):
                    tx[c, r:r + 16, :] = xc[:, c * 128:(c + 1) * 128]
                v = jnp.sum(xc * xc, axis=-1, keepdims=True) * (1.0 / D)
                inv = lax.rsqrt(v + TINY)
                tix[r:r + 16, :] = jnp.broadcast_to(inv, (16, 128))
                s_ref[r:r + 16, :] = jnp.broadcast_to((v + TINY) * inv * lax.rsqrt(v + EPS), (16, 128))
                yield
            yield from combine_pieces(tx, tix, a7)

        @phase(NC // 2)
        def proj(a7, s_ref, b7, dst, row0):
            def emit(half, c, y):
                dst[c, pl.ds(row0 + half * TH, TH), :] = y * s_ref[half * TH:(half + 1) * TH, :]
            for j in range(NC // 2):
                smm(a7, b7, j, emit)
                yield

        @phase(T // 8 * (NC // CS))
        def attn_scores(q, row0, first):
            R = 8
            for r in range(0, T, R):
                ls = [None] * W
                for c in range(NC):
                    qv, = gate(q[c, r:r + R, :])
                    for w in range(W):
                        t = qv * kk[c, pl.ds(HALO + row0 + r - DIL * w, R), :]
                        ls[w] = t if ls[w] is None else ls[w] + t
                    if c % CS == CS - 1 and c != NC - 1:
                        yield
                for w in range(W):
                    t = ls[w] + pltpu.roll(ls[w], 64, 1)
                    t = t + pltpu.roll(t, 32, 1)
                    t = t * SCALE
                    if first is not None and r < DIL * w:
                        row = lax.broadcasted_iota(jnp.int32, (R, 128), 0) + r
                        t = jnp.where(row < first * (DIL * w), NEG, t)
                    ls[w] = t
                m = ls[0]
                for w in range(1, W):
                    m = jnp.maximum(m, ls[w])
                es = [jnp.exp(ls[w] - m) for w in range(W)]
                s = es[0]
                for w in range(1, W):
                    s = s + es[w]
                inv = 1.0 / s
                for w in range(W):
                    pp[w, r:r + R, :] = es[w] * inv
                yield

        @phase(T // 8 * (NC // CM) + TH // 16 * NC // 2)
        def attn_mix(row0, o7, so):
            R = 8
            for r in range(0, T, R):
                es = [pp[w, r:r + R, :] for w in range(W)]
                ss = None
                for c in range(NC):
                    if c % CM == 0:
                        es = gate(*es)
                    acc = None
                    for w in range(W):
                        t = es[w] * vv[c, pl.ds(HALO + row0 + r - DIL * w, R), :]
                        acc = t if acc is None else acc + t
                    to[c, r:r + R, :] = acc
                    ss = acc * acc if ss is None else ss + acc * acc
                    if c % CM == CM - 1 and c != NC - 1:
                        yield
                ss = jnp.sum(ss, axis=-1, keepdims=True) + TINY
                inv = lax.rsqrt(ss)
                tio[r:r + R, :] = jnp.broadcast_to(inv, (R, 128))
                so[r:r + R, :] = jnp.broadcast_to(ss * inv, (R, 128))
                yield
            yield from combine_pieces(to, tio, o7)

        @phase(NC // 2)
        def proj_res(a7, s_ref, b7, row, with_bias):
            def emit(half, c, y):
                rows = pl.ds(pl.multiple_of(row + half * TH, TH), TH)
                cols = slice(c * 128, (c + 1) * 128)
                z = y * s_ref[half * TH:(half + 1) * TH, :]
                if with_bias:
                    z = z + bias[32 + c:33 + c, :]
                xb[rows, cols] = (xb[rows, cols].astype(f32) + z).astype(bf16)
            for j in range(NC // 2):
                smm(a7, b7, j, emit)
                yield

        @phase(NF // 2)
        def ffn1():
            started = [False, False]

            def emit(half, c, y):
                rows = slice(half * TH, (half + 1) * TH)
                z = jnp.maximum(y * sf[rows, :] + bias[c:c + 1, :], 0.0)
                z = z * z
                th[c, rows, :] = z
                tss[rows, :] = tss[rows, :] + z * z if started[half] else z * z
                started[half] = True
            for j in range(NF // 2):
                smm(xf7, w17, j, emit)
                yield

        @phase(T // 32 + TH // 16 * NF // 2)
        def h_combine():
            for r in range(0, T, 32):
                ss, = gate(tss[r:r + 32, :])
                ss = jnp.sum(ss, axis=-1, keepdims=True) + TINY
                inv = lax.rsqrt(ss)
                tih[r:r + 32, :] = jnp.broadcast_to(inv, (32, 128))
                sh[r:r + 32, :] = jnp.broadcast_to(ss * inv, (32, 128))
                yield
            yield from combine_pieces(th, tih, h7)

        def ffn2(row):
            return proj_res(h7, sh, w27, row, True)

        def proj_o(row, o7, so):
            return proj_res(o7, so, wo7, row, False)

        nothing = Phase(0, iter(()))
        dummy = Phase(1, iter([None]))

        def solo(*ps):
            for p in ps:
                for _ in p.gen:
                    pass

        def first_halo():
            for c in range(NC):
                kk[c, 0:HALO, :] = jnp.zeros((HALO, 128), f32)
                vv[c, 0:HALO, :] = jnp.broadcast_to(vv[c, HALO:HALO + 1, :], (HALO, 128))

        def move_halo(ref, src, dst):
            for c in range(NC):
                ref[c, pl.ds(dst, HALO), :] = ref[c, pl.ds(src, HALO), :]

        x_copy(0).wait()
        solo(ln_tile(0, xa7, sa))
        x_copy(1).wait()
        solo(ln_tile(T, xb7, sb))
        wqkv_copy(0).wait()
        solo(prep_qkv(0, wq7))
        wqkv_copy(1).wait()
        run(chain(proj(xa7, sa, wq7, qa, 0), proj(xb7, sb, wq7, qb, 0)), prep_qkv(1, wk7))
        wqkv_copy(2).wait()
        run(chain(proj(xa7, sa, wk7, kk, HALO), proj(xb7, sb, wk7, kk, HALO + T)), prep_qkv(2, wv7))
        for c in range(NC):
            kk[c, 0:HALO, :] = jnp.zeros((HALO, 128), f32)
        wo_copy.wait()
        x_copy(2).wait()
        run(proj(xa7, sa, wv7, vv, HALO), attn_scores(qa, 0, 1), lead=1)
        for c in range(NC):
            vv[c, 0:HALO, :] = jnp.broadcast_to(vv[c, HALO:HALO + 1, :], (HALO, 128))
        run(proj(xb7, sb, wv7, vv, HALO + T), ln_tile(2 * T, xa7, sa), prep_o(), lead=1)
        run(proj(xa7, sa, wq7, qa, 0), attn_mix(0, o7, so), lead=1)
        run(proj(xa7, sa, wk7, kk, HALO + 2 * T), attn_scores(qb, T, None), lead=1)
        w1_copy.wait()
        run(proj(xa7, sa, wv7, vv, HALO + 2 * T), attn_mix(T, o7b, sob), lead=1)
        run(proj_o(0, o7, so), attn_scores(qa, 2 * T, None), lead=1)
        run(proj_o(T, o7b, sob), attn_mix(2 * T, o7, so), lead=1)
        move_halo(kk, 3 * T, T)
        move_halo(vv, 3 * T, T)
        w2_copy.wait()
        x_copy(3).wait()
        run(proj_o(2 * T, o7, so), ln_tile(0, xf7, sf), lead=1)
        solo(prep_1(), prep_2())

        def step(i, carry):
            t0 = i % NT
            t1 = (i + 1) % NT
            t3 = (i + SKEW) % NT

            @pl.when(jnp.logical_and(i > 0, i + SKEW < NT))
            def _():
                x_copy(i + SKEW).wait()

            move_halo(kk, T, 0)
            vh = [vv[c, pl.ds(T, HALO), :] for c in range(NC)]
            for c in range(NC):
                vv[c, 0:HALO, :] = vh[c]
            run(ffn1(), ln_tile(t3 * T, xa7, sa))
            run(chain(proj(xa7, sa, wq7, qa, 0), proj(xa7, sa, wk7, kk, HALO)), h_combine(), ln_tile(t1 * T, xf7, sf), lead=1)
            run(proj(xa7, sa, wv7, vv, HALO), attn_scores(qa, 0, (t3 == 0).astype(jnp.int32)), lead=1)
            for c in range(NC):
                v0 = jnp.broadcast_to(vv[c, HALO:HALO + 1, :], (HALO, 128))
                vv[c, 0:HALO, :] = jnp.where(t3 == 0, v0, vv[c, 0:HALO, :])
            run(ffn2(t0 * T), attn_mix(0, o7, so), lead=1)
            solo(proj_o(t3 * T, o7, so))

            @pl.when(i >= NT)
            def _():
                o_copy(t0).start()
            return carry

        lax.fori_loop(0, NJ or (2 * NT - SKEW), step, 0)

        def tail(t, carry):
            solo(ffn1())
            solo(h_combine())
            run(ffn2(t * T), ln_tile((t + 1) % NT * T, xf7, sf), lead=1)
            o_copy(t).start()
            return carry

        lax.fori_loop(NT - SKEW, NT, tail, 0)
        for t in range(NT):
            o_copy(t).wait()

    V = pltpu.VMEM
    scratch = [
        V((S, D), bf16),
        V((3, D, D), bf16),
        V((NC, D // 2, 128), u32),
        V((D, D), bf16),
        V((NC, D // 2, 128), u32),
        V((D, F), bf16),
        V((F, D), bf16),
        V((7, D // 4, D // 2), u32), V((7, D // 4, D // 2), u32), V((7, D // 4, D // 2), u32), V((7, D // 4, D // 2), u32),
        V((7, D // 4, F // 2), u32), V((7, F // 4, D // 2), u32),
        V((40, 128), f32),
        V((7, T // 4, D // 2), u32), V((7, T // 4, D // 2), u32), V((7, T // 4, D // 2), u32), V((7, T // 4, D // 2), u32),
        V((7, T // 4, D // 2), u32), V((7, T // 4, F // 2), u32),
        V((T, 128), f32), V((T, 128), f32), V((T, 128), f32), V((T, 128), f32), V((T, 128), f32), V((T, 128), f32),
        V((NC, T, 128), f32), V((T, 128), f32), V((NC, T, 128), f32), V((T, 128), f32),
        V((NF, T, 128), f32), V((T, 128), f32), V((T, 128), f32),
        V((NC, T, 128), f32), V((NC, T, 128), f32),
        V((NC, HALO + 3 * T, 128), f32), V((NC, HALO + 3 * T, 128), f32),
        V((W, T, 128), f32),
        V((8, 128), u32),
        pltpu.SemaphoreType.DMA((NT,)),
        pltpu.SemaphoreType.DMA((6,)),
        pltpu.SemaphoreType.DMA((NT,)),
    ]

    @jax.jit
    def fn(A_x, A_wqkv, A_wo, B_x, B_w1, B_b1, B_w2, B_b2):
        any_spec = pl.BlockSpec(memory_space=pl.ANY)
        vm = pl.BlockSpec(memory_space=pltpu.VMEM)
        out = pl.pallas_call(
            kernel,
            in_specs=[any_spec, any_spec, any_spec, any_spec, vm, any_spec, vm],
            out_specs=any_spec,
            out_shape=jax.ShapeDtypeStruct((S, D), bf16),
            scratch_shapes=scratch,
            compiler_params=pltpu.CompilerParams(vmem_limit_bytes=110 * 2 ** 20, flags=flags),
        )(A_x.reshape(S, D), A_wqkv, A_wo, B_w1, B_b1.reshape(NF, 128), B_w2, B_b2.reshape(NC, 128))
        return out.reshape(1, S, D)

    return fn


@jax.jit
def pallas_interleave_layers__sliding_local_dilated__dense_activation_squared_relu__prompt_kernel(A_x, A_wqkv, A_wo, B_x, B_w1, B_b1, B_w2, B_b2):
    return make()(A_x, A_wqkv, A_wo, B_x, B_w1, B_b1, B_w2, B_b2)
```

```python
import jax
import jax.numpy as jnp
import numpy as np
from jax import lax
from jax.experimental import pallas as pl
from jax.experimental.pallas import tpu as pltpu

S, D, F = 2048, 1024, 3584
H, DH, W, DIL = 32, 32, 8, 2
HALO = 16
NC = D // 128
NF = F // 128
EPS = 1e-5
TINY = 1e-36
SCALE = DH ** -0.5
NEG = -1e9
LOG2E = 1.4426950408889634
T = 256
TH = T // 2
NT = S // T
SKEW = 3

f32 = jnp.float32
bf16 = jnp.bfloat16
u32 = jnp.uint32
DN = (((1,), (0,)), ((), ()))


def _pack(even, odd):
    return pltpu.pack_elementwise([even, odd], packed_dtype=bf16)


def _pack_rows(x):
    return pltpu.bitcast(x.astype(bf16), u32)


def _halves(u):
    return [pltpu.unpack_elementwise(u, index=i, packed_dtype=bf16, unpacked_dtype=f32) for i in range(2)]


def _pack_op(op, a, b):
    return _pack(op(a[0], b[0]), op(a[1], b[1]))


def _unpack(u):
    return pltpu.bitcast(u, bf16)


class Phase:
    def __init__(self, n, gen):
        self.n, self.gen = n, gen


def phase(n):
    def deco(f):
        return lambda *a: Phase(n, f(*a))
    return deco


def chain(*ps):
    def g():
        for p in ps:
            yield from p.gen
    return Phase(sum(p.n for p in ps), g())


def make(GATE=1, CS=4, CM=4, CC=2, GP=1, LAG=2, RS=96, KSPLIT=512, flags=None, NJ=None):
    def kernel(x_hbm, wqkv_hbm, wo_hbm, w1_hbm, b1_ref, w2_hbm, b2_ref, o_hbm,
               xb, wraw, wtmp, woraw, wou, w1raw, w2raw,
               wq7, wk7, wv7, wo7, w17, w27, bias,
               xa7, xb7, xf7, o7, o7b, o7c, h7, sa, sb, sf, so, sob, soc, sh,
               tx, tix, to, tio, th, tih, tss,
               qa, qb, kk, vv, pp, zero_ref,
               sem_x, sem_w, sem_o):
        def x_copy(t):
            return pltpu.make_async_copy(x_hbm.at[pl.ds(t * T, T)], xb.at[pl.ds(t * T, T)], sem_x.at[t])

        def o_copy(t):
            return pltpu.make_async_copy(xb.at[pl.ds(t * T, T)], o_hbm.at[pl.ds(t * T, T)], sem_o.at[t])

        def wqkv_copy(i):
            return pltpu.make_async_copy(wqkv_hbm.at[:, pl.ds(i * D, D)], wraw.at[i], sem_w.at[i])

        wo_copy = pltpu.make_async_copy(wo_hbm, woraw, sem_w.at[3])
        w1_copy = pltpu.make_async_copy(w1_hbm, w1raw, sem_w.at[4])
        w2_copy = pltpu.make_async_copy(w2_hbm, w2raw, sem_w.at[5])

        x_copy(0).start()
        wqkv_copy(0).start()
        x_copy(1).start()
        wqkv_copy(1).start()
        wqkv_copy(2).start()
        wo_copy.start()
        x_copy(2).start()
        w1_copy.start()
        x_copy(3).start()
        w2_copy.start()
        for t in range(4, NT):
            x_copy(t).start()

        bias[0:NF, :] = b1_ref[...].astype(f32)
        bias[32:32 + NC, :] = b2_ref[...].astype(f32)
        zero_ref[...] = jnp.zeros((8, 128), u32)

        fresh = []
        tok = [None]
        due = [None]

        def after(z, x):
            u = pltpu.bitcast(x, u32)
            return pltpu.bitcast(u | jnp.tile(z, (u.shape[0] // 8, u.shape[1] // 128)), x.dtype)

        def gate(*xs):
            if tok[0] is None:
                return xs
            z = pltpu.bitcast(tok[0], u32) & zero_ref[...]
            return [after(z, x) for x in xs]

        def run(main, *side, lead=1, lag=LAG):
            side = chain(*side)
            slots = max(main.n - lead, 1)
            done = 0
            dues = {}
            for i in range(main.n):
                del fresh[:]
                due[0] = dues.pop(i, None)
                next(main.gen)
                toks = [y[r:r + 8, c:c + 128] for y in fresh for c in range(0, y.shape[1], 128)
                        for r in range(0, y.shape[0], 8)]
                want = min(side.n, -(-side.n * (i + 1) // slots))
                k = want - done
                z = None
                for j in range(k):
                    tok[0] = toks[j * len(toks) // k] if (toks and GATE) else None
                    last = next(side.gen)
                    if last is not None and lag:
                        last = pltpu.bitcast(last, u32)[:8, :128]
                        z = last if z is None else z & last
                if z is not None:
                    dues[i + lag] = z & zero_ref[...]
                done = want
            tok[0] = None
            for z in dues.values():
                due[0] = z if due[0] is None else due[0] | z
            for p in (main, side):
                for _ in p.gen:
                    raise AssertionError("piece count mismatch")

        def store_b7(dst, prow, col, u11, u12, u21, u22):
            b11, b12, b21, b22 = (_halves(u) for u in (u11, u12, u21, u22))
            at = (pl.ds(prow, u11.shape[0]), pl.ds(col, 128))
            dst[(0,) + at] = _pack_op(lax.add, b11, b22)
            dst[(1,) + at] = u11
            dst[(2,) + at] = _pack_op(lax.sub, b12, b22)
            dst[(3,) + at] = _pack_op(lax.sub, b21, b11)
            dst[(4,) + at] = u22
            dst[(5,) + at] = _pack_op(lax.add, b11, b12)
            last = _pack_op(lax.add, b21, b22)
            dst[(6,) + at] = last
            return last

        def combine_pieces(src, inv, dst):
            nk = src.shape[0] // 2
            for r in range(0, TH, 16):
                it, ib = inv[r:r + 16, :], inv[TH + r:TH + r + 16, :]
                for j in range(nk):
                    if j % CC == 0:
                        it, ib = gate(it, ib)
                    a11, a12, a21, a22 = (src[c, r0:r0 + 16, :] * sc
                                          for r0, sc in ((r, it), (TH + r, ib)) for c in (j, nk + j))
                    at = (slice(r // 2, r // 2 + 8), slice(j * 128, (j + 1) * 128))
                    dst[(0,) + at] = _pack_rows(a11 + a22)
                    dst[(1,) + at] = _pack_rows(a21 + a22)
                    dst[(2,) + at] = _pack_rows(a11)
                    dst[(3,) + at] = _pack_rows(a22)
                    dst[(4,) + at] = _pack_rows(a11 + a12)
                    dst[(5,) + at] = _pack_rows(a21 - a11)
                    last = _pack_rows(a12 - a22)
                    dst[(6,) + at] = last
                    yield last

        def smm(a7, b7, j, emit):
            cols = slice(j * 128, (j + 1) * 128)
            kh = a7.shape[2]
            step = KSPLIT if KSPLIT else kh

            def m(i):
                y = None
                for k in range(0, kh, step):
                    ke = min(k + step, kh)
                    lhs = a7[i, :, k:ke]
                    if due[0] is not None:
                        head = jnp.concatenate([lhs[:8, c:c + 128] | due[0] for c in range(0, min(512, ke - k), 128)], axis=1)
                        if ke - k > 512:
                            head = jnp.concatenate([head, lhs[:8, 512:]], axis=1)
                        lhs = jnp.concatenate([head, lhs[8:]], axis=0)
                        due[0] = None
                    yk = lax.dot_general(_unpack(lhs), _unpack(b7[i, k // 2:ke // 2, cols]), DN,
                                         preferred_element_type=f32)
                    fresh.append(yk)
                    y = yk if y is None else y + yk
                return y

            nh = b7.shape[2] // 128
            m1 = m(0)
            m2 = m(1)
            c22 = m1 - m2
            m4 = m(3)
            emit(1, j, m2 + m4)
            c11 = m1 + m4
            c11 = c11 + m(6)
            m5 = m(4)
            emit(0, j, c11 - m5)
            m3 = m(2)
            emit(0, nh + j, m3 + m5)
            c22 = c22 + m3
            emit(1, nh + j, c22 + m(5))

        @phase(D // 64)
        def prep_qkv_skew(i, G=4):
            lane8 = lax.broadcasted_iota(jnp.int32, (8, 128), 1)
            bits = [(lane8 & (1 << b)) != 0 for b in range(3)]
            for g0 in range(0, D // 16, G):
                xs = [[None] * NC for _ in range(G)]
                for c in range(NC):
                    for g in range(G):
                        u = pltpu.bitcast(wraw[i, (g0 + g) * 16:(g0 + g + 1) * 16, c * 128:(c + 1) * 128], u32)
                        u, = gate(u)
                        xs[g][c] = pltpu.roll(u, c, 1) if c else u
                for g in range(G):
                    ws = [xs[g][(-c) % NC] for c in range(NC)]
                    for b in range(3):
                        ws = [jnp.where(bits[b], ws[(c - (1 << b)) % NC], ws[c]) for c in range(NC)]
                    for c in range(NC):
                        wtmp[c, (g0 + g) * 8:(g0 + g + 1) * 8, :] = ws[c]
                yield ws[0]

        @phase(3)
        def prep_qkv_cols(j, dst):
            lane = lax.broadcasted_iota(jnp.int32, (64, 128), 1)
            base = (lane & 3) * 32 + (lane >> 5) * 8 + ((lane >> 2) & 7)
            for c in (j, NC // 2 + j):
                gidx = (base + c) & 127
                for r in range(0, D // 2, 64):
                    u, = gate(wtmp[c, r:r + 64, :])
                    u = jnp.take_along_axis(u, gidx, axis=1)
                    wtmp[c, r:r + 64, :] = u
                yield u
            for r in range(0, D // 4, 16):
                last = store_b7(dst, r, j * 128,
                                wtmp[j, r:r + 16, :], wtmp[NC // 2 + j, r:r + 16, :],
                                wtmp[j, D // 4 + r:D // 4 + r + 16, :],
                                wtmp[NC // 2 + j, D // 4 + r:D // 4 + r + 16, :])
            yield last

        def prep_qkv(i, dst):
            return chain(prep_qkv_skew(i), *[prep_qkv_cols(j, dst) for j in range(NC // 2)])

        @phase(NC)
        def stage_o():
            for n in range(NC):
                u, = gate(pltpu.bitcast(woraw[:, n * 128:(n + 1) * 128], u32))
                wou[n] = u
                yield u

        @phase(NC * NC // 8)
        def prep_o():
            def rows16(n, cp, a):
                st = ((16 * (a % 2)) * 32 + (a // 2) * 8) // 2 + cp
                lo = wou[n, pl.ds(st, 8, stride=32), :]
                hi = wou[n, pl.ds(st + 16, 8, stride=32), :]
                return (lo & u32(0xFFFF)) | (hi << 16), (lo >> 16) | (hi & u32(0xFFFF0000))

            for j in range(NC // 2):
                for cp in range(NC // 4):
                    for a in range(8):
                        u11, u12 = rows16(j, cp, a), rows16(NC // 2 + j, cp, a)
                        u21, u22 = rows16(j, NC // 4 + cp, a), rows16(NC // 2 + j, NC // 4 + cp, a)
                        for par in range(2):
                            last = store_b7(wo7, (2 * cp + par) * 64 + 8 * a, j * 128,
                                            u11[par], u12[par], u21[par], u22[par])
                    yield last

        def prep_plain_pieces(raw, dst, rows):
            kh, nh = raw.shape[0] // 2, raw.shape[1] // 2
            for r in range(0, kh, rows):
                for c in range(0, nh, 128):
                    q = [pltpu.bitcast(raw[r0:r0 + rows, c0:c0 + 128], u32)
                         for r0 in (r, kh + r) for c0 in (c, nh + c)]
                    if GP:
                        q = gate(*q)
                    yield store_b7(dst, r // 2, c, *q)

        @phase(D // 128 * NF // 2)
        def prep_1():
            yield from prep_plain_pieces(w1raw, w17, 64)

        @phase(F // 128 * NC // 2)
        def prep_2():
            yield from prep_plain_pieces(w2raw, w27, 64)

        @phase(T // 16 + TH // 16 * NC // 2)
        def ln_tile(row, a7, s_ref):
            for r in range(0, T, 16):
                xu, = gate(xb[pl.ds(pl.multiple_of(row + r, 16), 16), :])
                x = xu.astype(f32)
                m = jnp.sum(x, axis=-1, keepdims=True) * (1.0 / D)
                xc = x - m
                for c in range(NC):
                    tx[c, r:r + 16, :] = xc[:, c * 128:(c + 1) * 128]
                v = jnp.sum(xc * xc, axis=-1, keepdims=True) * (1.0 / D)
                inv = lax.rsqrt(v + TINY)
                tix[r:r + 16, :] = jnp.broadcast_to(inv, (16, 128))
                sc = jnp.broadcast_to((v + TINY) * inv * lax.rsqrt(v + EPS), (16, 128))
                s_ref[r:r + 16, :] = sc
                yield sc
            yield from combine_pieces(tx, tix, a7)

        @phase(NC // 2)
        def proj(a7, s_ref, b7, dst, row0):
            def emit(half, c, y):
                dst[c, pl.ds(row0 + half * TH, TH), :] = y * s_ref[half * TH:(half + 1) * TH, :]
            for j in range(NC // 2):
                smm(a7, b7, j, emit)
                yield

        def attn_scores(q, row0, first, r0=0, r1=T):
            return Phase((r1 - r0) // 8 * (NC // CS), attn_scores_gen(q, row0, first, r0, r1))

        def attn_scores_gen(q, row0, first, r0, r1):
            R = 8
            for r in range(r0, r1, R):
                ls = [None] * W
                for c in range(NC):
                    qv, = gate(q[c, r:r + R, :])
                    for w in range(W):
                        t = qv * kk[c, pl.ds(HALO + row0 + r - DIL * w, R), :]
                        ls[w] = t if ls[w] is None else ls[w] + t
                    if c % CS == CS - 1 and c != NC - 1:
                        yield None
                for w in range(W):
                    t = ls[w] + pltpu.roll(ls[w], 64, 1)
                    t = t + pltpu.roll(t, 32, 1)
                    if first is not None and r < DIL * w:
                        row = lax.broadcasted_iota(jnp.int32, (R, 128), 0) + r
                        t = jnp.where(row < first * (DIL * w), NEG / SCALE, t)
                    ls[w] = t
                m = ls[0]
                for w in range(1, W):
                    m = jnp.maximum(m, ls[w])
                es = [jnp.exp2((ls[w] - m) * (SCALE * LOG2E)) for w in range(W)]
                s = es[0]
                for w in range(1, W):
                    s = s + es[w]
                inv = 1.0 / s
                for w in range(W):
                    pp[w, r:r + R, :] = es[w] * inv
                yield inv

        @phase(T // 8 * (NC // CM) + TH // 16 * NC // 2)
        def attn_mix(row0, o7, so):
            R = 8
            for r in range(0, T, R):
                es = [pp[w, r:r + R, :] for w in range(W)]
                ss = None
                for c in range(NC):
                    if c % CM == 0:
                        es = gate(*es)
                    acc = None
                    for w in range(W):
                        t = es[w] * vv[c, pl.ds(HALO + row0 + r - DIL * w, R), :]
                        acc = t if acc is None else acc + t
                    to[c, r:r + R, :] = acc
                    ss = acc * acc if ss is None else ss + acc * acc
                    if c % CM == CM - 1 and c != NC - 1:
                        yield None
                ss = jnp.sum(ss, axis=-1, keepdims=True) + TINY
                inv = lax.rsqrt(ss)
                tio[r:r + R, :] = jnp.broadcast_to(inv, (R, 128))
                sc = jnp.broadcast_to(ss * inv, (R, 128))
                so[r:r + R, :] = sc
                yield sc
            yield from combine_pieces(to, tio, o7)

        @phase(NC // 2)
        def proj_res(a7, s_ref, b7, row, with_bias):
            def emit(half, c, y):
                rows = pl.ds(pl.multiple_of(row + half * TH, TH), TH)
                cols = slice(c * 128, (c + 1) * 128)
                z = y * s_ref[half * TH:(half + 1) * TH, :]
                if with_bias:
                    z = z + bias[32 + c:33 + c, :]
                xb[rows, cols] = (xb[rows, cols].astype(f32) + z).astype(bf16)
            for j in range(NC // 2):
                smm(a7, b7, j, emit)
                yield

        @phase(NF // 2)
        def ffn1():
            started = [False, False]

            def emit(half, c, y):
                rows = slice(half * TH, (half + 1) * TH)
                z = jnp.maximum(y * sf[rows, :] + bias[c:c + 1, :], 0.0)
                z = z * z
                th[c, rows, :] = z
                tss[rows, :] = tss[rows, :] + z * z if started[half] else z * z
                started[half] = True
            for j in range(NF // 2):
                smm(xf7, w17, j, emit)
                yield

        @phase(T // 32 + TH // 16 * NF // 2)
        def h_combine():
            for r in range(0, T, 32):
                ss, = gate(tss[r:r + 32, :])
                ss = jnp.sum(ss, axis=-1, keepdims=True) + TINY
                inv = lax.rsqrt(ss)
                tih[r:r + 32, :] = jnp.broadcast_to(inv, (32, 128))
                sc = jnp.broadcast_to(ss * inv, (32, 128))
                sh[r:r + 32, :] = sc
                yield sc
            yield from combine_pieces(th, tih, h7)

        def ffn2(row):
            return proj_res(h7, sh, w27, row, True)

        def proj_o(row, o7, so):
            return proj_res(o7, so, wo7, row, False)

        nothing = Phase(0, iter(()))
        dummy = Phase(1, iter([None]))

        def solo(*ps):
            for p in ps:
                for _ in p.gen:
                    pass

        def first_halo():
            for c in range(NC):
                kk[c, 0:HALO, :] = jnp.zeros((HALO, 128), f32)
                vv[c, 0:HALO, :] = jnp.broadcast_to(vv[c, HALO:HALO + 1, :], (HALO, 128))

        def move_halo(ref, src, dst):
            for c in range(NC):
                ref[c, pl.ds(dst, HALO), :] = ref[c, pl.ds(src, HALO), :]

        x_copy(0).wait()
        solo(ln_tile(0, xa7, sa))
        x_copy(1).wait()
        solo(ln_tile(T, xb7, sb))
        wqkv_copy(0).wait()
        solo(prep_qkv_skew(0))
        solo(prep_qkv_cols(0, wq7))
        run(proj(xa7, sa, wq7, qa, 0), *[prep_qkv_cols(j, wq7) for j in range(1, NC // 2)], lag=1)
        wqkv_copy(1).wait()
        run(proj(xb7, sb, wq7, qb, 0), prep_qkv_skew(1), prep_qkv_cols(0, wk7), prep_qkv_cols(1, wk7))
        wqkv_copy(2).wait()
        run(chain(proj(xa7, sa, wk7, kk, HALO), proj(xb7, sb, wk7, kk, HALO + T)),
            prep_qkv_cols(2, wk7), prep_qkv_cols(3, wk7), prep_qkv(2, wv7), lag=1)
        for c in range(NC):
            kk[c, 0:HALO, :] = jnp.zeros((HALO, 128), f32)
        wo_copy.wait()
        run(proj(xa7, sa, wv7, vv, HALO), attn_scores(qa, 0, 1), stage_o())
        for c in range(NC):
            vv[c, 0:HALO, :] = jnp.broadcast_to(vv[c, HALO:HALO + 1, :], (HALO, 128))
        x_copy(2).wait()
        run(proj(xb7, sb, wv7, vv, HALO + T), ln_tile(2 * T, xa7, sa), attn_mix(0, o7, so))
        run(proj(xa7, sa, wq7, qa, 0), attn_scores(qb, T, None))
        run(proj(xa7, sa, wk7, kk, HALO + 2 * T), attn_mix(T, o7b, sob))
        run(proj(xa7, sa, wv7, vv, HALO + 2 * T), attn_scores(qa, 2 * T, None), prep_o())
        w1_copy.wait()
        run(chain(proj_o(0, o7, so), proj_o(T, o7b, sob)), attn_mix(2 * T, o7c, soc), prep_1())
        move_halo(kk, 3 * T, T)
        move_halo(vv, 3 * T, T)
        w2_copy.wait()
        x_copy(3).wait()
        run(proj_o(2 * T, o7c, soc), ln_tile(0, xf7, sf), prep_2())

        def step(i, carry):
            t0 = i % NT
            t1 = (i + 1) % NT
            t3 = (i + SKEW) % NT

            @pl.when(jnp.logical_and(i > 0, i + SKEW < NT))
            def _():
                x_copy(i + SKEW).wait()

            move_halo(kk, T, 0)
            vh = [vv[c, pl.ds(T, HALO), :] for c in range(NC)]
            for c in range(NC):
                vv[c, 0:HALO, :] = vh[c]
            first = (t3 == 0).astype(jnp.int32)
            run(ffn1(), ln_tile(t3 * T, xa7, sa), lead=3)
            run(chain(proj(xa7, sa, wq7, qa, 0), proj(xa7, sa, wk7, kk, HALO)), h_combine(), ln_tile(t1 * T, xf7, sf))
            run(proj(xa7, sa, wv7, vv, HALO), attn_scores(qa, 0, first, 0, RS))
            for c in range(NC):
                v0 = jnp.broadcast_to(vv[c, HALO:HALO + 1, :], (HALO, 128))
                vv[c, 0:HALO, :] = jnp.where(t3 == 0, v0, vv[c, 0:HALO, :])
            run(ffn2(t0 * T), attn_scores(qa, 0, first, RS, T), attn_mix(0, o7, so))
            solo(proj_o(t3 * T, o7, so))

            @pl.when(i >= NT)
            def _():
                o_copy(t0).start()
            return carry

        lax.fori_loop(0, NJ or (2 * NT - SKEW), step, 0)

        def tail(t, carry):
            solo(ffn1())
            solo(h_combine())
            run(ffn2(t * T), ln_tile((t + 1) % NT * T, xf7, sf), lead=2)
            o_copy(t).start()
            return carry

        lax.fori_loop(NT - SKEW, NT, tail, 0)
        for t in range(NT):
            o_copy(t).wait()

    V = pltpu.VMEM
    scratch = [
        V((S, D), bf16),
        V((3, D, D), bf16),
        V((NC, D // 2, 128), u32),
        V((D, D), bf16),
        V((NC, D // 2, 128), u32),
        V((D, F), bf16),
        V((F, D), bf16),
        V((7, D // 4, D // 2), u32), V((7, D // 4, D // 2), u32), V((7, D // 4, D // 2), u32), V((7, D // 4, D // 2), u32),
        V((7, D // 4, F // 2), u32), V((7, F // 4, D // 2), u32),
        V((40, 128), f32),
        V((7, T // 4, D // 2), u32), V((7, T // 4, D // 2), u32), V((7, T // 4, D // 2), u32), V((7, T // 4, D // 2), u32),
        V((7, T // 4, D // 2), u32), V((7, T // 4, D // 2), u32), V((7, T // 4, F // 2), u32),
        V((T, 128), f32), V((T, 128), f32), V((T, 128), f32), V((T, 128), f32), V((T, 128), f32), V((T, 128), f32), V((T, 128), f32),
        V((NC, T, 128), f32), V((T, 128), f32), V((NC, T, 128), f32), V((T, 128), f32),
        V((NF, T, 128), f32), V((T, 128), f32), V((T, 128), f32),
        V((NC, T, 128), f32), V((NC, T, 128), f32),
        V((NC, HALO + 3 * T, 128), f32), V((NC, HALO + 3 * T, 128), f32),
        V((W, T, 128), f32),
        V((8, 128), u32),
        pltpu.SemaphoreType.DMA((NT,)),
        pltpu.SemaphoreType.DMA((6,)),
        pltpu.SemaphoreType.DMA((NT,)),
    ]

    @jax.jit
    def fn(A_x, A_wqkv, A_wo, B_x, B_w1, B_b1, B_w2, B_b2):
        any_spec = pl.BlockSpec(memory_space=pl.ANY)
        vm = pl.BlockSpec(memory_space=pltpu.VMEM)
        out = pl.pallas_call(
            kernel,
            in_specs=[any_spec, any_spec, any_spec, any_spec, vm, any_spec, vm],
            out_specs=any_spec,
            out_shape=jax.ShapeDtypeStruct((S, D), bf16),
            scratch_shapes=scratch,
            compiler_params=pltpu.CompilerParams(vmem_limit_bytes=110 * 2 ** 20, flags=flags),
        )(A_x.reshape(S, D), A_wqkv, A_wo, B_w1, B_b1.reshape(NF, 128), B_w2, B_b2.reshape(NC, 128))
        return out.reshape(1, S, D)

    return fn


@jax.jit
def pallas_interleave_layers__sliding_local_dilated__dense_activation_squared_relu__prompt_kernel(A_x, A_wqkv, A_wo, B_x, B_w1, B_b1, B_w2, B_b2):
    return make(RS=112)(A_x, A_wqkv, A_wo, B_x, B_w1, B_b1, B_w2, B_b2)
```

```python
import jax
import jax.numpy as jnp
import numpy as np
from jax import lax
from jax.experimental import pallas as pl
from jax.experimental.pallas import tpu as pltpu

S, D, F = 2048, 1024, 3584
H, DH, W, DIL = 32, 32, 8, 2
HALO = 16
NC = D // 128
NF = F // 128
EPS = 1e-5
TINY = 1e-36
SCALE = DH ** -0.5
NEG = -1e9
LOG2E = 1.4426950408889634
T = 256
TH = T // 2
NT = S // T
SKEW = 3

f32 = jnp.float32
bf16 = jnp.bfloat16
u32 = jnp.uint32
DN = (((1,), (0,)), ((), ()))


def _pack(even, odd):
    return pltpu.pack_elementwise([even, odd], packed_dtype=bf16)


def _pack_rows(x):
    return pltpu.bitcast(x.astype(bf16), u32)


def _halves(u):
    return [pltpu.unpack_elementwise(u, index=i, packed_dtype=bf16, unpacked_dtype=f32) for i in range(2)]


def _pack_op(op, a, b):
    return _pack(op(a[0], b[0]), op(a[1], b[1]))


def _unpack(u):
    return pltpu.bitcast(u, bf16)


class Phase:
    def __init__(self, n, gen):
        self.n, self.gen = n, gen


def phase(n):
    def deco(f):
        return lambda *a: Phase(n, f(*a))
    return deco


def chain(*ps):
    def g():
        for p in ps:
            yield from p.gen
    return Phase(sum(p.n for p in ps), g())


def make(GATE=1, CS=4, CM=4, CC=1, GP=2, PL=0, P0=0, LN2P=1, ORD=1, L1=2, G1=2, PR=64, LAG=2, RS=112, KSPLIT=512, flags=None, NJ=None):
    def kernel(x_hbm, wqkv_hbm, wo_hbm, w1_hbm, b1_ref, w2_hbm, b2_ref, o_hbm,
               xb, wraw, wtmp, woraw, wou, w1raw, w2raw,
               wq7, wk7, wv7, wo7, w17, w27, bias,
               xab7, xf7, o7, o7b, h7, sab, sf, so, sob, sh,
               tx, tix, to, tio, th, tih, tss,
               qa, qb, kk, vv, pp, zero_ref,
               sem_x, sem_w, sem_o):
        xa7, xb7, sa, sb = xab7.at[0], xab7.at[1], sab.at[0], sab.at[1]

        def x_copy(t):
            return pltpu.make_async_copy(x_hbm.at[pl.ds(t * T, T)], xb.at[pl.ds(t * T, T)], sem_x.at[t])

        def o_copy(t):
            return pltpu.make_async_copy(xb.at[pl.ds(t * T, T)], o_hbm.at[pl.ds(t * T, T)], sem_o.at[t])

        def wqkv_copy(i):
            return pltpu.make_async_copy(wqkv_hbm.at[:, pl.ds(i * D, D)], wraw.at[i], sem_w.at[i])

        wo_copy = pltpu.make_async_copy(wo_hbm, woraw, sem_w.at[3])
        w1_copy = pltpu.make_async_copy(w1_hbm, w1raw, sem_w.at[4])
        w2_copy = pltpu.make_async_copy(w2_hbm, w2raw, sem_w.at[5])

        def wait(copy):
            carry.clear()
            copy.wait()

        x_copy(0).start()
        wqkv_copy(0).start()
        x_copy(1).start()
        wqkv_copy(1).start()
        wqkv_copy(2).start()
        wo_copy.start()
        x_copy(2).start()
        w1_copy.start()
        x_copy(3).start()
        w2_copy.start()
        for t in range(4, NT):
            x_copy(t).start()

        bias[0:NF, :] = b1_ref[...].astype(f32)
        bias[32:32 + NC, :] = b2_ref[...].astype(f32)
        zero_ref[...] = jnp.zeros((8, 128), u32)

        fresh = []
        tok = [None]
        carry = {}
        due = [None]

        def after(z, x):
            u = pltpu.bitcast(x, u32)
            return pltpu.bitcast(u | jnp.tile(z, (u.shape[0] // 8, u.shape[1] // 128)), x.dtype)

        def gate(*xs):
            if tok[0] is None:
                return xs
            z = pltpu.bitcast(tok[0], u32) & zero_ref[...]
            return [after(z, x) for x in xs]

        def run(main, *side, lead=1, lag=LAG):
            side = chain(*side)
            slots = max(main.n - lead, 1)
            done = 0
            dues = dict(carry)
            carry.clear()
            for i in range(main.n):
                del fresh[:]
                due[0] = dues.pop(i, None)
                next(main.gen)
                toks = [y[r:r + 8, c:c + 128] for y in fresh for c in range(0, y.shape[1], 128)
                        for r in range(0, y.shape[0], 8)]
                want = min(side.n, -(-side.n * (i + 1) // slots))
                k = want - done
                z = None
                for j in range(k):
                    tok[0] = toks[j * len(toks) // k] if (toks and GATE) else None
                    last = next(side.gen)
                    if last is not None and lag:
                        last = pltpu.bitcast(last, u32)[:8, :128]
                        z = last if z is None else z & last
                if z is not None:
                    dues[i + lag] = z & zero_ref[...]
                done = want
            tok[0] = None
            due[0] = None
            for i, z in dues.items():
                carry[i - main.n] = z
            for p in (main, side):
                for _ in p.gen:
                    raise AssertionError("piece count mismatch")

        def store_b7(dst, prow, col, u11, u12, u21, u22):
            b11, b12, b21, b22 = (_halves(u) for u in (u11, u12, u21, u22))
            at = (pl.ds(prow, u11.shape[0]), pl.ds(col, 128))
            dst[(0,) + at] = _pack_op(lax.add, b11, b22)
            dst[(1,) + at] = u11
            dst[(2,) + at] = _pack_op(lax.sub, b12, b22)
            dst[(3,) + at] = _pack_op(lax.sub, b21, b11)
            dst[(4,) + at] = u22
            dst[(5,) + at] = _pack_op(lax.add, b11, b12)
            last = _pack_op(lax.add, b21, b22)
            dst[(6,) + at] = last
            return last

        def combine_pieces(src, inv, dst):
            nk = src.shape[0] // 2
            for r in range(0, TH, 16):
                it, ib = inv[r:r + 16, :], inv[TH + r:TH + r + 16, :]
                for j in range(nk):
                    if j % CC == 0:
                        it, ib = gate(it, ib)
                    a11, a12, a21, a22 = (src[c, r0:r0 + 16, :] * sc
                                          for r0, sc in ((r, it), (TH + r, ib)) for c in (j, nk + j))
                    at = (slice(r // 2, r // 2 + 8), slice(j * 128, (j + 1) * 128))
                    dst[(0,) + at] = _pack_rows(a11 + a22)
                    dst[(1,) + at] = _pack_rows(a21 + a22)
                    dst[(2,) + at] = _pack_rows(a11)
                    dst[(3,) + at] = _pack_rows(a22)
                    dst[(4,) + at] = _pack_rows(a11 + a12)
                    dst[(5,) + at] = _pack_rows(a21 - a11)
                    last = _pack_rows(a12 - a22)
                    dst[(6,) + at] = last
                    yield last

        def smm(a7, b7, j, emit):
            cols = slice(j * 128, (j + 1) * 128)
            kh = a7.shape[2]
            step = KSPLIT if KSPLIT else kh

            def m(i):
                y = None
                for k in range(0, kh, step):
                    ke = min(k + step, kh)
                    lhs = a7[i, :, k:ke]
                    if due[0] is not None:
                        head = jnp.concatenate([lhs[:8, c:c + 128] | due[0] for c in range(0, min(512, ke - k), 128)], axis=1)
                        if ke - k > 512:
                            head = jnp.concatenate([head, lhs[:8, 512:]], axis=1)
                        lhs = jnp.concatenate([head, lhs[8:]], axis=0)
                        due[0] = None
                    yk = lax.dot_general(_unpack(lhs), _unpack(b7[i, k // 2:ke // 2, cols]), DN,
                                         preferred_element_type=f32)
                    fresh.append(yk)
                    y = yk if y is None else y + yk
                return y

            nh = b7.shape[2] // 128
            m1 = m(0)
            m2 = m(1)
            c22 = m1 - m2
            m4 = m(3)
            emit(1, j, m2 + m4)
            c11 = m1 + m4
            c11 = c11 + m(6)
            m5 = m(4)
            emit(0, j, c11 - m5)
            m3 = m(2)
            emit(0, nh + j, m3 + m5)
            c22 = c22 + m3
            emit(1, nh + j, c22 + m(5))

        @phase(D // 64)
        def prep_qkv_skew(i, G=4):
            lane8 = lax.broadcasted_iota(jnp.int32, (8, 128), 1)
            bits = [(lane8 & (1 << b)) != 0 for b in range(3)]
            for g0 in range(0, D // 16, G):
                xs = [[None] * NC for _ in range(G)]
                for c in range(NC):
                    for g in range(G):
                        u = pltpu.bitcast(wraw[i, (g0 + g) * 16:(g0 + g + 1) * 16, c * 128:(c + 1) * 128], u32)
                        u, = gate(u)
                        xs[g][c] = pltpu.roll(u, c, 1) if c else u
                for g in range(G):
                    ws = [xs[g][(-c) % NC] for c in range(NC)]
                    for b in range(3):
                        ws = [jnp.where(bits[b], ws[(c - (1 << b)) % NC], ws[c]) for c in range(NC)]
                    for c in range(NC):
                        wtmp[c, (g0 + g) * 8:(g0 + g + 1) * 8, :] = ws[c]
                yield ws[0]

        @phase(3)
        def prep_qkv_cols(j, dst):
            lane = lax.broadcasted_iota(jnp.int32, (64, 128), 1)
            base = (lane & 3) * 32 + (lane >> 5) * 8 + ((lane >> 2) & 7)
            for c in (j, NC // 2 + j):
                gidx = (base + c) & 127
                for r in range(0, D // 2, 64):
                    u, = gate(wtmp[c, r:r + 64, :])
                    u = jnp.take_along_axis(u, gidx, axis=1)
                    wtmp[c, r:r + 64, :] = u
                yield u
            for r in range(0, D // 4, 16):
                last = store_b7(dst, r, j * 128,
                                wtmp[j, r:r + 16, :], wtmp[NC // 2 + j, r:r + 16, :],
                                wtmp[j, D // 4 + r:D // 4 + r + 16, :],
                                wtmp[NC // 2 + j, D // 4 + r:D // 4 + r + 16, :])
            yield last

        def prep_qkv(i, dst):
            return chain(prep_qkv_skew(i), *[prep_qkv_cols(j, dst) for j in range(NC // 2)])

        @phase(NC)
        def stage_o():
            for n in range(NC):
                u, = gate(pltpu.bitcast(woraw[:, n * 128:(n + 1) * 128], u32))
                wou[n] = u
                yield u

        @phase(NC * NC // 2)
        def prep_o():
            def rows16(n, cp, a):
                st = ((16 * (a % 2)) * 32 + (a // 2) * 8) // 2 + cp
                lo = wou[n, pl.ds(st, 8, stride=32), :]
                hi = wou[n, pl.ds(st + 16, 8, stride=32), :]
                return (lo & u32(0xFFFF)) | (hi << 16), (lo >> 16) | (hi & u32(0xFFFF0000))

            for j in range(NC // 2):
                for cp in range(NC // 4):
                    for a in range(8):
                        u11, u12 = rows16(j, cp, a), rows16(NC // 2 + j, cp, a)
                        u21, u22 = rows16(j, NC // 4 + cp, a), rows16(NC // 2 + j, NC // 4 + cp, a)
                        u11, u22 = gate(*u11), gate(*u22)
                        for par in range(2):
                            last = store_b7(wo7, (2 * cp + par) * 64 + 8 * a, j * 128,
                                            u11[par], u12[par], u21[par], u22[par])
                        if a % 2:
                            yield last

        def prep_plain_pieces(raw, dst, rows):
            kh, nh = raw.shape[0] // 2, raw.shape[1] // 2
            for r in range(0, kh, rows):
                for c in range(0, nh, 128):
                    q = [pltpu.bitcast(raw[r0:r0 + rows, c0:c0 + 128], u32)
                         for r0 in (r, kh + r) for c0 in (c, nh + c)]
                    if GP:
                        q = gate(*q) if GP == 1 else list(gate(q[0], q[3])) [:1] + q[1:3] + list(gate(q[3]))
                    yield store_b7(dst, r // 2, c, *q)

        @phase(D // 2 // PR * NF // 2)
        def prep_1():
            yield from prep_plain_pieces(w1raw, w17, PR)

        @phase(F // 2 // PR * NC // 2)
        def prep_2():
            yield from prep_plain_pieces(w2raw, w27, PR)

        @phase((2 if LN2P else 1) * T // 16 + TH // 16 * NC // 2)
        def ln_tile(row, a7, s_ref):
            for r in range(0, T, 16):
                rows = pl.ds(pl.multiple_of(row + r, 16), 16)
                if LN2P:
                    acc = None
                    for c in range(NC):
                        xu = xb[rows, c * 128:(c + 1) * 128]
                        if c == 0:
                            xu, = gate(xu)
                        acc = xu.astype(f32) if acc is None else acc + xu.astype(f32)
                    m = jnp.broadcast_to(jnp.sum(acc, axis=-1, keepdims=True) * (1.0 / D), (16, 128))
                    yield m
                    m, = gate(m)
                    acc = None
                    for c in range(NC):
                        xc = xb[rows, c * 128:(c + 1) * 128].astype(f32) - m
                        tx[c, r:r + 16, :] = xc
                        acc = xc * xc if acc is None else acc + xc * xc
                    v = jnp.sum(acc, axis=-1, keepdims=True) * (1.0 / D)
                else:
                    xu, = gate(xb[rows, :])
                    x = xu.astype(f32)
                    m = jnp.sum(x, axis=-1, keepdims=True) * (1.0 / D)
                    xc = x - m
                    for c in range(NC):
                        tx[c, r:r + 16, :] = xc[:, c * 128:(c + 1) * 128]
                    v = jnp.sum(xc * xc, axis=-1, keepdims=True) * (1.0 / D)
                inv = lax.rsqrt(v + TINY)
                tix[r:r + 16, :] = jnp.broadcast_to(inv, (16, 128))
                sc = jnp.broadcast_to((v + TINY) * inv * lax.rsqrt(v + EPS), (16, 128))
                s_ref[r:r + 16, :] = sc
                yield sc
            yield from combine_pieces(tx, tix, a7)

        @phase(NC // 2)
        def proj(a7, s_ref, b7, dst, row0):
            def emit(half, c, y):
                dst[c, pl.ds(row0 + half * TH, TH), :] = y * s_ref[half * TH:(half + 1) * TH, :]
            for j in range(NC // 2):
                smm(a7, b7, j, emit)
                yield

        def attn_scores(q, row0, first, r0=0, r1=T):
            return Phase((r1 - r0) // 8 * (NC // CS), attn_scores_gen(q, row0, first, r0, r1))

        def attn_scores_gen(q, row0, first, r0, r1):
            R = 8
            for r in range(r0, r1, R):
                ls = [None] * W
                for c in range(NC):
                    qv, = gate(q[c, r:r + R, :])
                    for w in range(W):
                        t = qv * kk[c, pl.ds(HALO + row0 + r - DIL * w, R), :]
                        ls[w] = t if ls[w] is None else ls[w] + t
                    if c % CS == CS - 1 and c != NC - 1:
                        yield None
                for w in range(W):
                    t = ls[w] + pltpu.roll(ls[w], 64, 1)
                    t = t + pltpu.roll(t, 32, 1)
                    if first is not None and r < DIL * w:
                        row = lax.broadcasted_iota(jnp.int32, (R, 128), 0) + r
                        t = jnp.where(row < first * (DIL * w), NEG / SCALE, t)
                    ls[w] = t
                m = ls[0]
                for w in range(1, W):
                    m = jnp.maximum(m, ls[w])
                es = [jnp.exp2((ls[w] - m) * (SCALE * LOG2E)) for w in range(W)]
                s = es[0]
                for w in range(1, W):
                    s = s + es[w]
                inv = 1.0 / s
                for w in range(W):
                    pp[w, r:r + R, :] = es[w] * inv
                yield inv

        def attn_mix(row0, o7, so, r0=0, r1=T):
            return Phase((r1 - r0) // 8 * (NC // CM) + (TH // 16 * NC // 2 if r1 == T else 0),
                         attn_mix_gen(row0, o7, so, r0, r1))

        def attn_mix_gen(row0, o7, so, r0, r1):
            R = 8
            for r in range(r0, r1, R):
                es = [pp[w, r:r + R, :] for w in range(W)]
                ss = None
                for c in range(NC):
                    if c % CM == 0:
                        es = gate(*es)
                    acc = None
                    for w in range(W):
                        t = es[w] * vv[c, pl.ds(HALO + row0 + r - DIL * w, R), :]
                        acc = t if acc is None else acc + t
                    to[c, r:r + R, :] = acc
                    ss = acc * acc if ss is None else ss + acc * acc
                    if c % CM == CM - 1 and c != NC - 1:
                        yield None
                ss = jnp.sum(ss, axis=-1, keepdims=True) + TINY
                inv = lax.rsqrt(ss)
                tio[r:r + R, :] = jnp.broadcast_to(inv, (R, 128))
                sc = jnp.broadcast_to(ss * inv, (R, 128))
                so[r:r + R, :] = sc
                yield sc
            if r1 == T:
                yield from combine_pieces(to, tio, o7)

        @phase(NC // 2)
        def proj_res(a7, s_ref, b7, row, with_bias):
            def emit(half, c, y):
                rows = pl.ds(pl.multiple_of(row + half * TH, TH), TH)
                cols = slice(c * 128, (c + 1) * 128)
                z = y * s_ref[half * TH:(half + 1) * TH, :]
                if with_bias:
                    z = z + bias[32 + c:33 + c, :]
                xb[rows, cols] = (xb[rows, cols].astype(f32) + z).astype(bf16)
            for j in range(NC // 2):
                smm(a7, b7, j, emit)
                yield

        @phase(NF // 2)
        def ffn1():
            started = [False, False]

            def emit(half, c, y):
                rows = slice(half * TH, (half + 1) * TH)
                z = jnp.maximum(y * sf[rows, :] + bias[c:c + 1, :], 0.0)
                z = z * z
                th[c, rows, :] = z
                tss[rows, :] = tss[rows, :] + z * z if started[half] else z * z
                started[half] = True
            for j in range(NF // 2):
                smm(xf7, w17, j, emit)
                yield

        @phase(T // 32 + TH // 16 * NF // 2)
        def h_combine():
            for r in range(0, T, 32):
                ss, = gate(tss[r:r + 32, :])
                ss = jnp.sum(ss, axis=-1, keepdims=True) + TINY
                inv = lax.rsqrt(ss)
                tih[r:r + 32, :] = jnp.broadcast_to(inv, (32, 128))
                sc = jnp.broadcast_to(ss * inv, (32, 128))
                sh[r:r + 32, :] = sc
                yield sc
            yield from combine_pieces(th, tih, h7)

        def ffn2(row):
            return proj_res(h7, sh, w27, row, True)

        def proj_o(row, o7, so):
            return proj_res(o7, so, wo7, row, False)

        nothing = Phase(0, iter(()))
        dummy = Phase(1, iter([None]))

        def solo(*ps):
            due[0] = carry.pop(0, None)
            carry.clear()
            for p in ps:
                for _ in p.gen:
                    pass

        def first_halo():
            for c in range(NC):
                kk[c, 0:HALO, :] = jnp.zeros((HALO, 128), f32)
                vv[c, 0:HALO, :] = jnp.broadcast_to(vv[c, HALO:HALO + 1, :], (HALO, 128))

        def move_halo(ref, src, dst):
            for c in range(NC):
                ref[c, pl.ds(dst, HALO), :] = ref[c, pl.ds(src, HALO), :]

        def head(t, _):
            wait(x_copy(t))
            solo(ln_tile(t * T, xab7.at[t], sab.at[t]))
            return 0

        lax.fori_loop(0, 2, head, 0)
        wait(wqkv_copy(0))
        solo(prep_qkv_skew(0))
        solo(prep_qkv_cols(0, wq7))
        run(proj(xa7, sa, wq7, qa, 0), *[prep_qkv_cols(j, wq7) for j in range(1, NC // 2)], lag=1)
        wait(wqkv_copy(1))
        run(proj(xb7, sb, wq7, qb, 0), prep_qkv_skew(1), prep_qkv_cols(0, wk7), prep_qkv_cols(1, wk7))
        wait(wqkv_copy(2))
        run(chain(proj(xa7, sa, wk7, kk, HALO), proj(xb7, sb, wk7, kk, HALO + T)),
            prep_qkv_cols(2, wk7), prep_qkv_cols(3, wk7), prep_qkv(2, wv7), lag=1)
        for c in range(NC):
            kk[c, 0:HALO, :] = jnp.zeros((HALO, 128), f32)
        wait(wo_copy)
        run(proj(xa7, sa, wv7, vv, HALO), attn_scores(qa, 0, 1), stage_o())
        for c in range(NC):
            vv[c, 0:HALO, :] = jnp.broadcast_to(vv[c, HALO:HALO + 1, :], (HALO, 128))
        wait(x_copy(2))
        run(proj(xb7, sb, wv7, vv, HALO + T), ln_tile(2 * T, xa7, sa), lead=P0)
        run(proj(xa7, sa, wq7, qa, 0), prep_o(), attn_mix(0, o7, so, 0, 128), lead=P0)
        run(proj(xa7, sa, wk7, kk, HALO + 2 * T), attn_mix(0, o7, so, 128, T), attn_scores(qb, T, None, 0, 128), lead=P0)
        run(proj(xa7, sa, wv7, vv, HALO + 2 * T), attn_scores(qb, T, None, 128, T), attn_mix(T, o7b, sob, 0, 128), lead=P0)
        run(proj_o(0, o7, so), attn_mix(T, o7b, sob, 128, T))
        wait(w1_copy)
        wait(x_copy(3))
        run(proj_o(T, o7b, sob), ln_tile(0, xf7, sf), prep_1(), lead=PL, lag=1)
        run(ffn1(), attn_scores(qa, 2 * T, None), attn_mix(2 * T, o7, so), ln_tile(3 * T, xa7, sa))
        move_halo(kk, 3 * T, T)
        move_halo(vv, 3 * T, T)
        wait(w2_copy)
        run(proj_o(2 * T, o7, so), prep_2(), lead=PL)

        carry.clear()

        def step(i, _):
            t0 = i % NT
            t1 = (i + 1) % NT
            t3 = (i + SKEW) % NT
            t4 = (i + SKEW + 1) % NT

            @pl.when(i + SKEW + 1 < NT)
            def _():
                x_copy(i + SKEW + 1).wait()

            move_halo(kk, T, 0)
            move_halo(vv, T, 0)
            first = (t3 == 0).astype(jnp.int32)
            if ORD == 0:
                run(chain(proj(xa7, sa, wq7, qa, 0), proj(xa7, sa, wk7, kk, HALO)), h_combine(), ln_tile(t1 * T, xf7, sf))
            elif ORD == 1:
                run(chain(proj(xa7, sa, wq7, qa, 0), proj(xa7, sa, wk7, kk, HALO)), ln_tile(t1 * T, xf7, sf), h_combine())
            else:
                run(chain(proj(xa7, sa, wq7, qa, 0), proj(xa7, sa, wk7, kk, HALO)), h_combine())
            run(proj(xa7, sa, wv7, vv, HALO), attn_scores(qa, 0, first, 0, RS))
            for c in range(NC):
                v0 = jnp.broadcast_to(vv[c, HALO:HALO + 1, :], (HALO, 128))
                vv[c, 0:HALO, :] = jnp.where(t3 == 0, v0, vv[c, 0:HALO, :])
            if ORD == 3:
                run(ffn2(t0 * T), attn_scores(qa, 0, first, RS, T), ln_tile(t1 * T, xf7, sf), attn_mix(0, o7, so, 0, T))
                solo(proj_o(t3 * T, o7, so))
            else:
                run(ffn2(t0 * T), attn_scores(qa, 0, first, RS, T), attn_mix(0, o7, so, 0, T))
            if ORD == 2:
                run(proj_o(t3 * T, o7, so), ln_tile(t1 * T, xf7, sf), lead=2, lag=1)
            elif ORD == 3:
                pass
            else:
                solo(proj_o(t3 * T, o7, so))
            run(ffn1(), ln_tile(t4 * T, xa7, sa), lead=L1, lag=G1)

            @pl.when(jnp.logical_and(i >= NT, i < 2 * NT - SKEW))
            def _():
                o_copy(t0).start()
            carry.clear()
            return 0

        lax.fori_loop(0, NJ or (2 * NT - SKEW), step, 0)

        def tail(t, _):
            solo(h_combine())
            run(ffn2(t * T), ln_tile((t + 1) % NT * T, xf7, sf), lead=2)
            carry.clear()
            o_copy(t).start()

            @pl.when(t < NT - 1)
            def _():
                solo(ffn1())
            return 0

        lax.fori_loop(NT - SKEW, NT, tail, 0)
        for t in range(NT):
            o_copy(t).wait()

    V = pltpu.VMEM
    scratch = [
        V((S, D), bf16),
        V((3, D, D), bf16),
        V((NC, D // 2, 128), u32),
        V((D, D), bf16),
        V((NC, D // 2, 128), u32),
        V((D, F), bf16),
        V((F, D), bf16),
        V((7, D // 4, D // 2), u32), V((7, D // 4, D // 2), u32), V((7, D // 4, D // 2), u32), V((7, D // 4, D // 2), u32),
        V((7, D // 4, F // 2), u32), V((7, F // 4, D // 2), u32),
        V((40, 128), f32),
        V((2, 7, T // 4, D // 2), u32), V((7, T // 4, D // 2), u32), V((7, T // 4, D // 2), u32),
        V((7, T // 4, D // 2), u32), V((7, T // 4, F // 2), u32),
        V((2, T, 128), f32), V((T, 128), f32), V((T, 128), f32), V((T, 128), f32), V((T, 128), f32),
        V((NC, T, 128), f32), V((T, 128), f32), V((NC, T, 128), f32), V((T, 128), f32),
        V((NF, T, 128), f32), V((T, 128), f32), V((T, 128), f32),
        V((NC, T, 128), f32), V((NC, T, 128), f32),
        V((NC, HALO + 3 * T, 128), f32), V((NC, HALO + 3 * T, 128), f32),
        V((W, T, 128), f32),
        V((8, 128), u32),
        pltpu.SemaphoreType.DMA((NT,)),
        pltpu.SemaphoreType.DMA((6,)),
        pltpu.SemaphoreType.DMA((NT,)),
    ]

    @jax.jit
    def fn(A_x, A_wqkv, A_wo, B_x, B_w1, B_b1, B_w2, B_b2):
        any_spec = pl.BlockSpec(memory_space=pl.ANY)
        vm = pl.BlockSpec(memory_space=pltpu.VMEM)
        out = pl.pallas_call(
            kernel,
            in_specs=[any_spec, any_spec, any_spec, any_spec, vm, any_spec, vm],
            out_specs=any_spec,
            out_shape=jax.ShapeDtypeStruct((S, D), bf16),
            scratch_shapes=scratch,
            compiler_params=pltpu.CompilerParams(vmem_limit_bytes=110 * 2 ** 20, flags=flags),
        )(A_x.reshape(S, D), A_wqkv, A_wo, B_w1, B_b1.reshape(NF, 128), B_w2, B_b2.reshape(NC, 128))
        return out.reshape(1, S, D)

    return fn


@jax.jit
def pallas_interleave_layers__sliding_local_dilated__dense_activation_squared_relu__prompt_kernel(A_x, A_wqkv, A_wo, B_x, B_w1, B_b1, B_w2, B_b2):
    return make()(A_x, A_wqkv, A_wo, B_x, B_w1, B_b1, B_w2, B_b2)
```

```python
import jax
import jax.numpy as jnp
import numpy as np
from jax import lax
from jax.experimental import pallas as pl
from jax.experimental.pallas import tpu as pltpu

S, D, F = 2048, 1024, 3584
H, DH, W, DIL = 32, 32, 8, 2
HALO = 16
NC = D // 128
NF = F // 128
EPS = 1e-5
TINY = 1e-36
SCALE = DH ** -0.5
NEG = -1e9
LOG2E = 1.4426950408889634
T = 256
TH = T // 2
NT = S // T
SKEW = 3

f32 = jnp.float32
bf16 = jnp.bfloat16
u32 = jnp.uint32
DN = (((1,), (0,)), ((), ()))


def _pack(even, odd):
    return pltpu.pack_elementwise([even, odd], packed_dtype=bf16)


def _pack_rows(x):
    return pltpu.bitcast(x.astype(bf16), u32)


def _halves(u):
    return [pltpu.unpack_elementwise(u, index=i, packed_dtype=bf16, unpacked_dtype=f32) for i in range(2)]


def _pack_op(op, a, b):
    return _pack(op(a[0], b[0]), op(a[1], b[1]))


def _unpack(u):
    return pltpu.bitcast(u, bf16)


def mix(a, b):
    def g():
        done = 0
        for i in range(a.n):
            yield next(a.gen)
            while done < (i + 1) * b.n // a.n:
                yield next(b.gen)
                done += 1
    return Phase(a.n + b.n, g())


class Phase:
    def __init__(self, n, gen):
        self.n, self.gen = n, gen


def phase(n):
    def deco(f):
        return lambda *a: Phase(n, f(*a))
    return deco


def chain(*ps):
    def g():
        for p in ps:
            yield from p.gen
    return Phase(sum(p.n for p in ps), g())


def make(GATE=1, CS=4, CM=4, CC=1, GP=2, PL=0, P0=0, PCS=8, PLAG=3, V2=5, XW=0, LN2P=1, ORD=1, L1=2, G1=2, PR=64, LAG=2, RS=112, KSPLIT=512, flags=None, NJ=None):
    def kernel(x_hbm, wqkv_hbm, wo_hbm, w1_hbm, b1_ref, w2_hbm, b2_ref, o_hbm,
               xb, wraw, wtmp, woraw, wou, w1raw, w2raw,
               wq7, wk7, wv7, wo7, w17, w27, bias,
               xab7, xf7, o7, o7b, h7, sab, sf, so, sob, sh,
               tx, tix, to, tio, th, tih, tss,
               qa, qb, kk, vv, pp, zero_ref,
               sem_x, sem_w, sem_o):
        xa7, xb7, sa, sb = xab7.at[0], xab7.at[1], sab.at[0], sab.at[1]

        def x_copy(t):
            return pltpu.make_async_copy(x_hbm.at[pl.ds(t * T, T)], xb.at[pl.ds(t * T, T)], sem_x.at[t])

        def o_copy(t):
            return pltpu.make_async_copy(xb.at[pl.ds(t * T, T)], o_hbm.at[pl.ds(t * T, T)], sem_o.at[t])

        def wqkv_copy(i):
            return pltpu.make_async_copy(wqkv_hbm.at[:, pl.ds(i * D, D)], wraw.at[i], sem_w.at[i])

        wo_copy = pltpu.make_async_copy(wo_hbm, woraw, sem_w.at[3])
        w1_copy = pltpu.make_async_copy(w1_hbm, w1raw, sem_w.at[4])
        w2_copy = pltpu.make_async_copy(w2_hbm, w2raw, sem_w.at[5])

        def wait(copy):
            carry.clear()
            copy.wait()

        x_copy(0).start()
        wqkv_copy(0).start()
        x_copy(1).start()
        wqkv_copy(1).start()
        wqkv_copy(2).start()
        wo_copy.start()
        x_copy(2).start()
        w1_copy.start()
        x_copy(3).start()
        w2_copy.start()
        for t in range(4, NT):
            x_copy(t).start()

        bias[0:NF, :] = b1_ref[...].astype(f32)
        bias[32:32 + NC, :] = b2_ref[...].astype(f32)
        zero_ref[...] = jnp.zeros((8, 128), u32)

        fresh = []
        cs = [PCS]
        lags = [PLAG]
        tok = [None]
        carry = {}
        due = [None]

        def after(z, x):
            u = pltpu.bitcast(x, u32)
            return pltpu.bitcast(u | jnp.tile(z, (u.shape[0] // 8, u.shape[1] // 128)), x.dtype)

        def gate(*xs):
            if tok[0] is None:
                return xs
            z = pltpu.bitcast(tok[0], u32) & zero_ref[...]
            return [after(z, x) for x in xs]

        def run(main, *side, lead=1, lag=None):
            lag = lags[0] if lag is None else lag
            side = chain(*side)
            slots = max(main.n - lead, 1)
            done = 0
            dues = dict(carry)
            carry.clear()
            for i in range(main.n):
                del fresh[:]
                due[0] = dues.pop(i, None)
                next(main.gen)
                toks = [y[r:r + 8, c:c + 128] for y in fresh for c in range(0, y.shape[1], 128)
                        for r in range(0, y.shape[0], 8)]
                want = min(side.n, -(-side.n * (i + 1) // slots))
                k = want - done
                z = None
                for j in range(k):
                    tok[0] = toks[j * len(toks) // k] if (toks and GATE) else None
                    last = next(side.gen)
                    if last is not None and lag:
                        last = pltpu.bitcast(last, u32)[:8, :128]
                        z = last if z is None else z & last
                if z is not None:
                    dues[i + lag] = z & zero_ref[...]
                done = want
            tok[0] = None
            due[0] = None
            for i, z in dues.items():
                carry[i - main.n] = z
            for p in (main, side):
                for _ in p.gen:
                    raise AssertionError("piece count mismatch")

        def store_b7(dst, prow, col, u11, u12, u21, u22):
            b11, b12, b21, b22 = (_halves(u) for u in (u11, u12, u21, u22))
            at = (pl.ds(prow, u11.shape[0]), pl.ds(col, 128))
            dst[(0,) + at] = _pack_op(lax.add, b11, b22)
            dst[(1,) + at] = u11
            dst[(2,) + at] = _pack_op(lax.sub, b12, b22)
            dst[(3,) + at] = _pack_op(lax.sub, b21, b11)
            dst[(4,) + at] = u22
            dst[(5,) + at] = _pack_op(lax.add, b11, b12)
            last = _pack_op(lax.add, b21, b22)
            dst[(6,) + at] = last
            return last

        def combine_pieces(src, inv, dst):
            nk = src.shape[0] // 2
            for r in range(0, TH, 16):
                it, ib = inv[r:r + 16, :], inv[TH + r:TH + r + 16, :]
                for j in range(nk):
                    if j % CC == 0:
                        it, ib = gate(it, ib)
                    a11, a12, a21, a22 = (src[c, r0:r0 + 16, :] * sc
                                          for r0, sc in ((r, it), (TH + r, ib)) for c in (j, nk + j))
                    at = (slice(r // 2, r // 2 + 8), slice(j * 128, (j + 1) * 128))
                    dst[(0,) + at] = _pack_rows(a11 + a22)
                    dst[(1,) + at] = _pack_rows(a21 + a22)
                    dst[(2,) + at] = _pack_rows(a11)
                    dst[(3,) + at] = _pack_rows(a22)
                    dst[(4,) + at] = _pack_rows(a11 + a12)
                    dst[(5,) + at] = _pack_rows(a21 - a11)
                    last = _pack_rows(a12 - a22)
                    dst[(6,) + at] = last
                    yield last

        def smm(a7, b7, j, emit):
            cols = slice(j * 128, (j + 1) * 128)
            kh = a7.shape[2]
            step = KSPLIT if KSPLIT else kh

            def m(i):
                y = None
                for k in range(0, kh, step):
                    ke = min(k + step, kh)
                    lhs = a7[i, :, k:ke]
                    if due[0] is not None:
                        head = jnp.concatenate([lhs[:8, c:c + 128] | due[0] for c in range(0, min(512, ke - k), 128)], axis=1)
                        if ke - k > 512:
                            head = jnp.concatenate([head, lhs[:8, 512:]], axis=1)
                        lhs = jnp.concatenate([head, lhs[8:]], axis=0)
                        due[0] = None
                    yk = lax.dot_general(_unpack(lhs), _unpack(b7[i, k // 2:ke // 2, cols]), DN,
                                         preferred_element_type=f32)
                    fresh.append(yk)
                    y = yk if y is None else y + yk
                return y

            nh = b7.shape[2] // 128
            m1 = m(0)
            m2 = m(1)
            c22 = m1 - m2
            m4 = m(3)
            emit(1, j, m2 + m4)
            c11 = m1 + m4
            c11 = c11 + m(6)
            m5 = m(4)
            emit(0, j, c11 - m5)
            m3 = m(2)
            emit(0, nh + j, m3 + m5)
            c22 = c22 + m3
            emit(1, nh + j, c22 + m(5))

        @phase(D // 64)
        def prep_qkv_skew(i, G=4):
            lane8 = lax.broadcasted_iota(jnp.int32, (8, 128), 1)
            bits = [(lane8 & (1 << b)) != 0 for b in range(3)]
            for g0 in range(0, D // 16, G):
                xs = [[None] * NC for _ in range(G)]
                for c in range(NC):
                    for g in range(G):
                        u = pltpu.bitcast(wraw[i, (g0 + g) * 16:(g0 + g + 1) * 16, c * 128:(c + 1) * 128], u32)
                        u, = gate(u)
                        xs[g][c] = pltpu.roll(u, c, 1) if c else u
                for g in range(G):
                    ws = [xs[g][(-c) % NC] for c in range(NC)]
                    for b in range(3):
                        ws = [jnp.where(bits[b], ws[(c - (1 << b)) % NC], ws[c]) for c in range(NC)]
                    for c in range(NC):
                        wtmp[c, (g0 + g) * 8:(g0 + g + 1) * 8, :] = ws[c]
                yield ws[0]

        @phase(3)
        def prep_qkv_cols(j, dst):
            lane = lax.broadcasted_iota(jnp.int32, (64, 128), 1)
            base = (lane & 3) * 32 + (lane >> 5) * 8 + ((lane >> 2) & 7)
            for c in (j, NC // 2 + j):
                gidx = (base + c) & 127
                for r in range(0, D // 2, 64):
                    u, = gate(wtmp[c, r:r + 64, :])
                    u = jnp.take_along_axis(u, gidx, axis=1)
                    wtmp[c, r:r + 64, :] = u
                yield u
            for r in range(0, D // 4, 16):
                last = store_b7(dst, r, j * 128,
                                wtmp[j, r:r + 16, :], wtmp[NC // 2 + j, r:r + 16, :],
                                wtmp[j, D // 4 + r:D // 4 + r + 16, :],
                                wtmp[NC // 2 + j, D // 4 + r:D // 4 + r + 16, :])
            yield last

        def prep_qkv(i, dst):
            return chain(prep_qkv_skew(i), *[prep_qkv_cols(j, dst) for j in range(NC // 2)])

        @phase(NC)
        def stage_o():
            for n in range(NC):
                u, = gate(pltpu.bitcast(woraw[:, n * 128:(n + 1) * 128], u32))
                for g in range(DH // 2):
                    wou[n, pl.ds(33 * g, 32), :] = u[32 * g:32 * (g + 1)]
                yield u

        @phase(NC * NC // 2)
        def prep_o():
            def rows16(n, cp, a):
                st = 33 * 8 * (a % 2) + 4 * (a // 2) + cp
                lo = wou[n, pl.ds(st, 8, stride=33), :]
                hi = wou[n, pl.ds(st + 16, 8, stride=33), :]
                return (lo & u32(0xFFFF)) | (hi << 16), (lo >> 16) | (hi & u32(0xFFFF0000))

            for j in range(NC // 2):
                for cp in range(NC // 4):
                    for a in range(8):
                        u11, u12 = rows16(j, cp, a), rows16(NC // 2 + j, cp, a)
                        u21, u22 = rows16(j, NC // 4 + cp, a), rows16(NC // 2 + j, NC // 4 + cp, a)
                        u11, u22 = gate(*u11), gate(*u22)
                        for par in range(2):
                            last = store_b7(wo7, (2 * cp + par) * 64 + 8 * a, j * 128,
                                            u11[par], u12[par], u21[par], u22[par])
                        if a % 2:
                            yield last

        def prep_plain(raw, dst, j0, j1):
            kh, nh = raw.shape[0] // 2, raw.shape[1] // 2

            def pieces():
                for c in range(j0 * 128, j1 * 128, 128):
                    for r in range(0, kh, PR):
                        q = [pltpu.bitcast(raw[r0:r0 + PR, c0:c0 + 128], u32)
                             for r0 in (r, kh + r) for c0 in (c, nh + c)]
                        q[0], q[3] = gate(q[0], q[3])
                        yield store_b7(dst, r // 2, c, *q)
            return Phase((j1 - j0) * kh // PR, pieces())

        def prep_1(j0, j1):
            return prep_plain(w1raw, w17, j0, j1)

        def prep_2(j0=0, j1=NC // 2):
            return prep_plain(w2raw, w27, j0, j1)

        @phase((2 if LN2P else 1) * T // 16 + TH // 16 * NC // 2)
        def ln_tile(row, a7, s_ref):
            for r in range(0, T, 16):
                rows = pl.ds(pl.multiple_of(row + r, 16), 16)
                if LN2P:
                    acc = None
                    for c in range(NC):
                        xu = xb[rows, c * 128:(c + 1) * 128]
                        if c == 0:
                            xu, = gate(xu)
                        acc = xu.astype(f32) if acc is None else acc + xu.astype(f32)
                    m = jnp.broadcast_to(jnp.sum(acc, axis=-1, keepdims=True) * (1.0 / D), (16, 128))
                    yield m
                    m, = gate(m)
                    acc = None
                    for c in range(NC):
                        xc = xb[rows, c * 128:(c + 1) * 128].astype(f32) - m
                        tx[c, r:r + 16, :] = xc
                        acc = xc * xc if acc is None else acc + xc * xc
                    v = jnp.sum(acc, axis=-1, keepdims=True) * (1.0 / D)
                else:
                    xu, = gate(xb[rows, :])
                    x = xu.astype(f32)
                    m = jnp.sum(x, axis=-1, keepdims=True) * (1.0 / D)
                    xc = x - m
                    for c in range(NC):
                        tx[c, r:r + 16, :] = xc[:, c * 128:(c + 1) * 128]
                    v = jnp.sum(xc * xc, axis=-1, keepdims=True) * (1.0 / D)
                inv = lax.rsqrt(v + TINY)
                tix[r:r + 16, :] = jnp.broadcast_to(inv, (16, 128))
                sc = jnp.broadcast_to((v + TINY) * inv * lax.rsqrt(v + EPS), (16, 128))
                s_ref[r:r + 16, :] = sc
                yield sc
            yield from combine_pieces(tx, tix, a7)

        @phase(NC // 2)
        def proj(a7, s_ref, b7, dst, row0):
            def emit(half, c, y):
                dst[c, pl.ds(row0 + half * TH, TH), :] = y * s_ref[half * TH:(half + 1) * TH, :]
            for j in range(NC // 2):
                smm(a7, b7, j, emit)
                yield

        def attn_scores(q, row0, first, r0=0, r1=T):
            return Phase((r1 - r0) // 8 * (NC // cs[0]), attn_scores_gen(q, row0, first, r0, r1, cs[0]))

        def attn_scores_gen(q, row0, first, r0, r1, CS):
            R = 8
            for r in range(r0, r1, R):
                ls = [None] * W
                for c in range(NC):
                    qv, = gate(q[c, r:r + R, :])
                    for w in range(W):
                        t = qv * kk[c, pl.ds(HALO + row0 + r - DIL * w, R), :]
                        ls[w] = t if ls[w] is None else ls[w] + t
                    if c % CS == CS - 1 and c != NC - 1:
                        yield None
                for w in range(W):
                    t = ls[w] + pltpu.roll(ls[w], 64, 1)
                    t = t + pltpu.roll(t, 32, 1)
                    if first is not None and r < DIL * w:
                        row = lax.broadcasted_iota(jnp.int32, (R, 128), 0) + r
                        t = jnp.where(row < first * (DIL * w), NEG / SCALE, t)
                    ls[w] = t
                m = ls[0]
                for w in range(1, W):
                    m = jnp.maximum(m, ls[w])
                es = [jnp.exp2((ls[w] - m) * (SCALE * LOG2E)) for w in range(W)]
                s = es[0]
                for w in range(1, W):
                    s = s + es[w]
                inv = 1.0 / s
                for w in range(W):
                    pp[w, r:r + R, :] = es[w] * inv
                yield inv

        def attn_mix(row0, o7, so, r0=0, r1=T):
            return Phase((r1 - r0) // 8 * (NC // cs[0]) + (TH // 16 * NC // 2 if r1 == T else 0),
                         attn_mix_gen(row0, o7, so, r0, r1, cs[0]))

        def attn_mix_gen(row0, o7, so, r0, r1, CM):
            R = 8
            for r in range(r0, r1, R):
                es = [pp[w, r:r + R, :] for w in range(W)]
                ss = None
                for c in range(NC):
                    if c % CM == 0:
                        es = gate(*es)
                    acc = None
                    for w in range(W):
                        t = es[w] * vv[c, pl.ds(HALO + row0 + r - DIL * w, R), :]
                        acc = t if acc is None else acc + t
                    to[c, r:r + R, :] = acc
                    ss = acc * acc if ss is None else ss + acc * acc
                    if c % CM == CM - 1 and c != NC - 1:
                        yield None
                ss = jnp.sum(ss, axis=-1, keepdims=True) + TINY
                inv = lax.rsqrt(ss)
                tio[r:r + R, :] = jnp.broadcast_to(inv, (R, 128))
                sc = jnp.broadcast_to(ss * inv, (R, 128))
                so[r:r + R, :] = sc
                yield sc
            if r1 == T:
                yield from combine_pieces(to, tio, o7)

        @phase(NC // 2)
        def proj_res(a7, s_ref, b7, row, with_bias):
            def emit(half, c, y):
                rows = pl.ds(pl.multiple_of(row + half * TH, TH), TH)
                cols = slice(c * 128, (c + 1) * 128)
                z = y * s_ref[half * TH:(half + 1) * TH, :]
                if with_bias:
                    z = z + bias[32 + c:33 + c, :]
                xb[rows, cols] = (xb[rows, cols].astype(f32) + z).astype(bf16)
            for j in range(NC // 2):
                smm(a7, b7, j, emit)
                yield

        @phase(NF // 2)
        def ffn1():
            started = [False, False]

            def emit(half, c, y):
                rows = slice(half * TH, (half + 1) * TH)
                z = jnp.maximum(y * sf[rows, :] + bias[c:c + 1, :], 0.0)
                z = z * z
                th[c, rows, :] = z
                tss[rows, :] = tss[rows, :] + z * z if started[half] else z * z
                started[half] = True
            for j in range(NF // 2):
                smm(xf7, w17, j, emit)
                yield

        @phase(T // 32 + TH // 16 * NF // 2)
        def h_combine():
            for r in range(0, T, 32):
                ss, = gate(tss[r:r + 32, :])
                ss = jnp.sum(ss, axis=-1, keepdims=True) + TINY
                inv = lax.rsqrt(ss)
                tih[r:r + 32, :] = jnp.broadcast_to(inv, (32, 128))
                sc = jnp.broadcast_to(ss * inv, (32, 128))
                sh[r:r + 32, :] = sc
                yield sc
            yield from combine_pieces(th, tih, h7)

        def ffn2(row):
            return proj_res(h7, sh, w27, row, True)

        def proj_o(row, o7, so):
            return proj_res(o7, so, wo7, row, False)

        nothing = Phase(0, iter(()))
        dummy = Phase(1, iter([None]))

        def solo(*ps):
            due[0] = carry.pop(0, None)
            carry.clear()
            for p in ps:
                for _ in p.gen:
                    pass

        def first_halo():
            for c in range(NC):
                kk[c, 0:HALO, :] = jnp.zeros((HALO, 128), f32)
                vv[c, 0:HALO, :] = jnp.broadcast_to(vv[c, HALO:HALO + 1, :], (HALO, 128))

        def move_halo(ref, src, dst):
            for c in range(NC):
                ref[c, pl.ds(dst, HALO), :] = ref[c, pl.ds(src, HALO), :]

        wait(x_copy(0))
        solo(ln_tile(0, xa7, sa))
        wait(wqkv_copy(0))
        solo(prep_qkv_skew(0))
        wait(x_copy(1))
        solo(prep_qkv_cols(0, wq7))
        run(proj(xa7, sa, wq7, qa, 0), mix(chain(*[prep_qkv_cols(j, wq7) for j in range(1, NC // 2)]), ln_tile(T, xb7, sb)), lag=1)
        wait(wqkv_copy(1))
        run(proj(xb7, sb, wq7, qb, 0), prep_qkv_skew(1), prep_qkv_cols(0, wk7), prep_qkv_cols(1, wk7))
        if XW:
            run(proj(xa7, sa, wk7, kk, HALO), prep_qkv_cols(2, wk7), prep_qkv_cols(3, wk7), lead=2, lag=1)
            wait(wqkv_copy(2))
            run(proj(xb7, sb, wk7, kk, HALO + T), prep_qkv_skew(2), prep_qkv_cols(0, wv7), prep_qkv_cols(1, wv7))
        else:
            wait(wqkv_copy(2))
            run(chain(proj(xa7, sa, wk7, kk, HALO), proj(xb7, sb, wk7, kk, HALO + T)),
                prep_qkv_cols(2, wk7), prep_qkv_cols(3, wk7), prep_qkv(2, wv7), lag=1)
        for c in range(NC):
            kk[c, 0:HALO, :] = jnp.zeros((HALO, 128), f32)
        if XW:
            run(proj(xa7, sa, wv7, vv, HALO), prep_qkv_cols(2, wv7), prep_qkv_cols(3, wv7), attn_scores(qa, 0, 1, 0, 128), lag=1)
        else:
            wait(wo_copy)
            run(proj(xa7, sa, wv7, vv, HALO), attn_scores(qa, 0, 1), stage_o())
        for c in range(NC):
            vv[c, 0:HALO, :] = jnp.broadcast_to(vv[c, HALO:HALO + 1, :], (HALO, 128))
        if XW:
            wait(wo_copy)
            run(proj(xb7, sb, wv7, vv, HALO + T), attn_scores(qa, 0, 1, 128, T), stage_o(), lead=P0)
            wait(x_copy(2))
        else:
            wait(x_copy(2))
            run(proj(xb7, sb, wv7, vv, HALO + T), ln_tile(2 * T, xa7, sa), lead=P0)
        if XW:
            raise NotImplementedError
        run(proj(xa7, sa, wq7, qa, 0), prep_o(), attn_mix(0, o7, so, 0, 128), lead=P0)
        run(proj(xa7, sa, wk7, kk, HALO + 2 * T), attn_mix(0, o7, so, 128, T), attn_scores(qb, T, None, 0, 128), lead=P0)
        if V2:
            wait(w1_copy)
            run(proj(xa7, sa, wv7, vv, HALO + 2 * T), attn_scores(qb, T, None, 128, T), attn_mix(T, o7b, sob, 0, 64), prep_1(0, V2), lead=P0)
        else:
            run(proj(xa7, sa, wv7, vv, HALO + 2 * T), attn_scores(qb, T, None, 128, T), attn_mix(T, o7b, sob, 0, 128), lead=P0)
        run(proj_o(0, o7, so), attn_mix(T, o7b, sob, 64 if V2 else 128, T))
        if not V2:
            wait(w1_copy)
        wait(x_copy(3))
        run(proj_o(T, o7b, sob), ln_tile(0, xf7, sf), prep_1(V2, NF // 2), lead=PL, lag=1)
        run(ffn1(), attn_scores(qa, 2 * T, None), attn_mix(2 * T, o7, so), ln_tile(3 * T, xa7, sa))
        move_halo(kk, 3 * T, T)
        move_halo(vv, 3 * T, T)
        wait(w2_copy)
        run(proj_o(2 * T, o7, so), prep_2(), lead=PL)

        carry.clear()

        cs[0] = CS
        lags[0] = LAG

        def step(i, _):
            t0 = i % NT
            t1 = (i + 1) % NT
            t3 = (i + SKEW) % NT
            t4 = (i + SKEW + 1) % NT

            @pl.when(i + SKEW + 1 < NT)
            def _():
                x_copy(i + SKEW + 1).wait()

            move_halo(kk, T, 0)
            move_halo(vv, T, 0)
            first = (t3 == 0).astype(jnp.int32)
            if ORD == 0:
                run(chain(proj(xa7, sa, wq7, qa, 0), proj(xa7, sa, wk7, kk, HALO)), h_combine(), ln_tile(t1 * T, xf7, sf))
            elif ORD == 1:
                run(chain(proj(xa7, sa, wq7, qa, 0), proj(xa7, sa, wk7, kk, HALO)), ln_tile(t1 * T, xf7, sf), h_combine())
            else:
                run(chain(proj(xa7, sa, wq7, qa, 0), proj(xa7, sa, wk7, kk, HALO)), h_combine())
            run(proj(xa7, sa, wv7, vv, HALO), attn_scores(qa, 0, first, 0, RS))
            for c in range(NC):
                v0 = jnp.broadcast_to(vv[c, HALO:HALO + 1, :], (HALO, 128))
                vv[c, 0:HALO, :] = jnp.where(t3 == 0, v0, vv[c, 0:HALO, :])
            if ORD == 3:
                run(ffn2(t0 * T), attn_scores(qa, 0, first, RS, T), ln_tile(t1 * T, xf7, sf), attn_mix(0, o7, so, 0, T))
                solo(proj_o(t3 * T, o7, so))
            else:
                run(ffn2(t0 * T), attn_scores(qa, 0, first, RS, T), attn_mix(0, o7, so, 0, T))
            if ORD == 2:
                run(proj_o(t3 * T, o7, so), ln_tile(t1 * T, xf7, sf), lead=2, lag=1)
            elif ORD == 3:
                pass
            else:
                solo(proj_o(t3 * T, o7, so))
            run(ffn1(), ln_tile(t4 * T, xa7, sa), lead=L1, lag=G1)

            @pl.when(jnp.logical_and(i >= NT, i < 2 * NT - SKEW))
            def _():
                o_copy(t0).start()
            carry.clear()
            return 0

        lax.fori_loop(0, NJ or (2 * NT - SKEW), step, 0)

        def tail(t, _):
            solo(h_combine())
            run(ffn2(t * T), ln_tile((t + 1) % NT * T, xf7, sf), lead=2)
            carry.clear()
            o_copy(t).start()

            @pl.when(t < NT - 1)
            def _():
                solo(ffn1())
            return 0

        lax.fori_loop(NT - SKEW, NT, tail, 0)
        for t in range(NT):
            o_copy(t).wait()

    V = pltpu.VMEM
    scratch = [
        V((S, D), bf16),
        V((3, D, D), bf16),
        V((NC, D // 2, 128), u32),
        V((D, D), bf16),
        V((NC, 33 * 16, 128), u32),
        V((D, F), bf16),
        V((F, D), bf16),
        V((7, D // 4, D // 2), u32), V((7, D // 4, D // 2), u32), V((7, D // 4, D // 2), u32), V((7, D // 4, D // 2), u32),
        V((7, D // 4, F // 2), u32), V((7, F // 4, D // 2), u32),
        V((40, 128), f32),
        V((2, 7, T // 4, D // 2), u32), V((7, T // 4, D // 2), u32), V((7, T // 4, D // 2), u32),
        V((7, T // 4, D // 2), u32), V((7, T // 4, F // 2), u32),
        V((2, T, 128), f32), V((T, 128), f32), V((T, 128), f32), V((T, 128), f32), V((T, 128), f32),
        V((NC, T, 128), f32), V((T, 128), f32), V((NC, T, 128), f32), V((T, 128), f32),
        V((NF, T, 128), f32), V((T, 128), f32), V((T, 128), f32),
        V((NC, T, 128), f32), V((NC, T, 128), f32),
        V((NC, HALO + 3 * T, 128), f32), V((NC, HALO + 3 * T, 128), f32),
        V((W, T, 128), f32),
        V((8, 128), u32),
        pltpu.SemaphoreType.DMA((NT,)),
        pltpu.SemaphoreType.DMA((6,)),
        pltpu.SemaphoreType.DMA((NT,)),
    ]

    @jax.jit
    def fn(A_x, A_wqkv, A_wo, B_x, B_w1, B_b1, B_w2, B_b2):
        any_spec = pl.BlockSpec(memory_space=pl.ANY)
        vm = pl.BlockSpec(memory_space=pltpu.VMEM)
        out = pl.pallas_call(
            kernel,
            in_specs=[any_spec, any_spec, any_spec, any_spec, vm, any_spec, vm],
            out_specs=any_spec,
            out_shape=jax.ShapeDtypeStruct((S, D), bf16),
            scratch_shapes=scratch,
            compiler_params=pltpu.CompilerParams(vmem_limit_bytes=110 * 2 ** 20, flags=flags),
        )(A_x.reshape(S, D), A_wqkv, A_wo, B_w1, B_b1.reshape(NF, 128), B_w2, B_b2.reshape(NC, 128))
        return out.reshape(1, S, D)

    return fn


@jax.jit
def pallas_interleave_layers__sliding_local_dilated__dense_activation_squared_relu__prompt_kernel(A_x, A_wqkv, A_wo, B_x, B_w1, B_b1, B_w2, B_b2):
    return make()(A_x, A_wqkv, A_wo, B_x, B_w1, B_b1, B_w2, B_b2)
```

```python
import jax
import jax.numpy as jnp
from jax import lax
from jax.experimental import pallas as pl
from jax.experimental.pallas import tpu as pltpu

S, D, F = 2048, 1024, 3584
DH, W, DIL = 32, 8, 2
EPS = 1e-5
SCALE = DH ** -0.5
MASKED = -1e9
LOG2E = 1.4426950408889634
TINY = 1e-36

T = 256
TH = T // 2
NT = S // T
HALO = 16
NC = D // 128
NF = F // 128
SKEW = 3
PAD = DH + 1

f32 = jnp.float32
bf16 = jnp.bfloat16
u32 = jnp.uint32


def _pack_rows(x):
    return pltpu.bitcast(x.astype(bf16), u32)


def _as_bf16(u):
    return pltpu.bitcast(u, bf16)


def _halves(u):
    return [pltpu.unpack_elementwise(u, index=i, packed_dtype=bf16, unpacked_dtype=f32) for i in range(2)]


def _pack_op(op, a, b):
    return pltpu.pack_elementwise([op(a[0], b[0]), op(a[1], b[1])], packed_dtype=bf16)


class _Phase:
    def __init__(self, n, gen):
        self.n, self.gen = n, gen


def _chain(*phases):
    def gen():
        for p in phases:
            yield from p.gen
    return _Phase(sum(p.n for p in phases), gen())


def _mix(a, b):
    def gen():
        done = 0
        for i in range(a.n):
            yield next(a.gen)
            while done < (i + 1) * b.n // a.n:
                yield next(b.gen)
                done += 1
    return _Phase(a.n + b.n, gen())


class _Schedule:
    def __init__(self, zero_ref):
        self.zero_ref = zero_ref
        self.results = []
        self.token = None
        self.due = None
        self.carry = {}
        self.lag = 3

    def gate(self, *xs):
        if self.token is None:
            return list(xs)
        zero = pltpu.bitcast(self.token, u32) & self.zero_ref[...]
        out = []
        for x in xs:
            u = pltpu.bitcast(x, u32)
            out.append(pltpu.bitcast(u | jnp.tile(zero, (u.shape[0] // 8, u.shape[1] // 128)), x.dtype))
        return out

    def hold(self, lhs):
        if self.due is None:
            return lhs
        n = min(lhs.shape[1], 512)
        head = [lhs[:8, c:c + 128] | self.due for c in range(0, n, 128)]
        if lhs.shape[1] > n:
            head.append(lhs[:8, n:])
        self.due = None
        return jnp.concatenate([jnp.concatenate(head, axis=1), lhs[8:]], axis=0)

    def run(self, main, *side, lead=1, lag=None):
        lag = self.lag if lag is None else lag
        side = _chain(*side)
        slots = max(main.n - lead, 1)
        dues, done = dict(self.carry), 0
        self.carry = {}
        for i in range(main.n):
            self.results = []
            self.due = dues.pop(i, None)
            next(main.gen)
            tokens = [(y, r) for y in self.results for r in range(0, y.shape[0], 8)]
            want = min(side.n, -(-side.n * (i + 1) // slots))
            finished = None
            for j in range(want - done):
                y, r = tokens[j * len(tokens) // (want - done)]
                self.token = y[r:r + 8]
                last = next(side.gen)
                if last is not None:
                    last = pltpu.bitcast(last, u32)[:8, :128]
                    finished = last if finished is None else finished & last
            if finished is not None:
                dues[i + lag] = finished & self.zero_ref[...]
            done = want
        self.token = self.due = None
        self.carry = {i - main.n: z for i, z in dues.items()}
        for p in (main, side):
            assert next(p.gen, _Schedule) is _Schedule, "wrong piece count"

    def solo(self, *phases):
        self.due = self.carry.pop(0, None)
        self.carry = {}
        for p in phases:
            for _ in p.gen:
                pass
        self.due = None

    def barrier(self):
        self.carry = {}


def _kernel(x_hbm, wqkv_hbm, wo_hbm, w1_hbm, b1_ref, w2_hbm, b2_ref, o_hbm,
            xb, wqkv_raw, wo_raw, w1_raw, w2_raw, w_tmp, wo_tmp,
            wq7, wk7, wv7, wo7, w17, w27, bias,
            xa7, xb7, xf7, oa7, ob7, h7, sa, sb, sf, soa, sob, sh,
            stage, stage_inv, h_stage, h_inv, h_ss,
            qa, qb, kk, vv, pp, zero_ref, sem_x, sem_w, sem_o):
    def x_copy(t):
        return pltpu.make_async_copy(x_hbm.at[pl.ds(t * T, T)], xb.at[pl.ds(t * T, T)], sem_x.at[t])

    def o_copy(t):
        return pltpu.make_async_copy(xb.at[pl.ds(t * T, T)], o_hbm.at[pl.ds(t * T, T)], sem_o.at[t])

    def wqkv_copy(i):
        return pltpu.make_async_copy(wqkv_hbm.at[:, pl.ds(i * D, D)], wqkv_raw.at[i], sem_w.at[i])

    wo_copy = pltpu.make_async_copy(wo_hbm, wo_raw, sem_w.at[3])
    w1_copy = pltpu.make_async_copy(w1_hbm, w1_raw, sem_w.at[4])
    w2_copy = pltpu.make_async_copy(w2_hbm, w2_raw, sem_w.at[5])

    for copy in (x_copy(0), wqkv_copy(0), x_copy(1), wqkv_copy(1), wqkv_copy(2), wo_copy, x_copy(2),
                 w1_copy, x_copy(3), w2_copy, *[x_copy(t) for t in range(4, NT)]):
        copy.start()

    bias[0:NF, :] = b1_ref[...].astype(f32)
    bias[32:32 + NC, :] = b2_ref[...].astype(f32)
    zero_ref[...] = jnp.zeros((8, 128), u32)

    sched = _Schedule(zero_ref)
    gate, run, solo = sched.gate, sched.run, sched.solo

    def wait(copy):
        sched.barrier()
        copy.wait()

    def store_b7(dst, row, col, u11, u12, u21, u22):
        b11, b12, b21, b22 = (_halves(u) for u in (u11, u12, u21, u22))
        at = (pl.ds(row, u11.shape[0]), pl.ds(col, 128))
        dst[(0,) + at] = _pack_op(lax.add, b11, b22)
        dst[(1,) + at] = u11
        dst[(2,) + at] = _pack_op(lax.sub, b12, b22)
        dst[(3,) + at] = _pack_op(lax.sub, b21, b11)
        dst[(4,) + at] = u22
        dst[(5,) + at] = _pack_op(lax.add, b11, b12)
        last = _pack_op(lax.add, b21, b22)
        dst[(6,) + at] = last
        return last

    def a7_pieces(src, inv, dst):
        nk = src.shape[0] // 2
        for r in range(0, TH, 16):
            top, bot = inv[r:r + 16, :], inv[TH + r:TH + r + 16, :]
            for j in range(nk):
                top, bot = gate(top, bot)
                a11, a12, a21, a22 = (src[c, r0:r0 + 16, :] * scale
                                      for r0, scale in ((r, top), (TH + r, bot)) for c in (j, nk + j))
                at = (slice(r // 2, r // 2 + 8), slice(j * 128, (j + 1) * 128))
                dst[(0,) + at] = _pack_rows(a11 + a22)
                dst[(1,) + at] = _pack_rows(a21 + a22)
                dst[(2,) + at] = _pack_rows(a11)
                dst[(3,) + at] = _pack_rows(a22)
                dst[(4,) + at] = _pack_rows(a11 + a12)
                dst[(5,) + at] = _pack_rows(a21 - a11)
                last = _pack_rows(a12 - a22)
                dst[(6,) + at] = last
                yield last

    def matmul(a7, b7, emit):
        kh, nh = a7.shape[2], b7.shape[2] // 128

        def product(i, j):
            y = None
            for k in range(0, kh, 512):
                ke = min(k + 512, kh)
                yk = lax.dot_general(_as_bf16(sched.hold(a7[i, :, k:ke])),
                                     _as_bf16(b7[i, k // 2:ke // 2, j * 128:(j + 1) * 128]),
                                     (((1,), (0,)), ((), ())), preferred_element_type=f32)
                sched.results.append(yk)
                y = yk if y is None else y + yk
            return y

        def gen():
            for j in range(nh):
                m1 = product(0, j)
                m2 = product(1, j)
                c22 = m1 - m2
                m4 = product(3, j)
                emit(1, j, m2 + m4)
                c11 = m1 + m4
                c11 = c11 + product(6, j)
                m5 = product(4, j)
                emit(0, j, c11 - m5)
                m3 = product(2, j)
                emit(0, nh + j, m3 + m5)
                c22 = c22 + m3
                emit(1, nh + j, c22 + product(5, j))
                yield
        return _Phase(nh, gen())

    def store_row_norm(ss, inv_ref, s_ref, r):
        ss = ss + TINY
        inv = lax.rsqrt(ss)
        shape = (ss.shape[0], 128)
        inv_ref[r:r + shape[0], :] = jnp.broadcast_to(inv, shape)
        norm = jnp.broadcast_to(ss * inv, shape)
        s_ref[r:r + shape[0], :] = norm
        return norm

    def qkv_skew(i):
        def gen(group=4):
            lane = lax.broadcasted_iota(jnp.int32, (8, 128), 1)
            bits = [(lane & (1 << b)) != 0 for b in range(3)]
            for g0 in range(0, D // 16, group):
                xs = [[None] * NC for _ in range(group)]
                for c in range(NC):
                    for g in range(group):
                        rows = slice((g0 + g) * 16, (g0 + g + 1) * 16)
                        u, = gate(pltpu.bitcast(wqkv_raw[i, rows, c * 128:(c + 1) * 128], u32))
                        xs[g][c] = pltpu.roll(u, c, 1) if c else u
                for g in range(group):
                    ws = [xs[g][(-c) % NC] for c in range(NC)]
                    for b in range(3):
                        ws = [jnp.where(bits[b], ws[(c - (1 << b)) % NC], ws[c]) for c in range(NC)]
                    for c in range(NC):
                        w_tmp[c, (g0 + g) * 8:(g0 + g + 1) * 8, :] = ws[c]
                yield ws[0]
        return _Phase(D // 64, gen())

    def qkv_finish(dst, j0, j1):
        def gen():
            lane = lax.broadcasted_iota(jnp.int32, (64, 128), 1)
            base = (lane & 3) * 32 + (lane >> 5) * 8 + ((lane >> 2) & 7)
            for j in range(j0, j1):
                left, right = j, NC // 2 + j
                for c in (left, right):
                    for r in range(0, D // 2, 64):
                        u, = gate(w_tmp[c, r:r + 64, :])
                        u = jnp.take_along_axis(u, (base + c) & 127, axis=1)
                        w_tmp[c, r:r + 64, :] = u
                    yield u
                for r in range(0, D // 4, 16):
                    top, bot = slice(r, r + 16), slice(D // 4 + r, D // 4 + r + 16)
                    last = store_b7(dst, r, j * 128, w_tmp[left, top, :], w_tmp[right, top, :],
                                    w_tmp[left, bot, :], w_tmp[right, bot, :])
                yield last
        return _Phase(3 * (j1 - j0), gen())

    def wo_stage():
        def gen():
            for n in range(NC):
                u, = gate(pltpu.bitcast(wo_raw[:, n * 128:(n + 1) * 128], u32))
                for g in range(D // 64):
                    wo_tmp[n, pl.ds(PAD * g, 32), :] = u[32 * g:32 * (g + 1)]
                yield u
        return _Phase(NC, gen())

    def wo_finish():
        def rows16(n, cp, a):
            start = PAD * 8 * (a % 2) + 4 * (a // 2) + cp
            lo = wo_tmp[n, pl.ds(start, 8, stride=PAD), :]
            hi = wo_tmp[n, pl.ds(start + 16, 8, stride=PAD), :]
            return (lo & u32(0xFFFF)) | (hi << 16), (lo >> 16) | (hi & u32(0xFFFF0000))

        def gen():
            for j in range(NC // 2):
                for cp in range(NC // 4):
                    for a in range(8):
                        u11, u12 = rows16(j, cp, a), rows16(NC // 2 + j, cp, a)
                        u21, u22 = rows16(j, NC // 4 + cp, a), rows16(NC // 2 + j, NC // 4 + cp, a)
                        u11, u22 = gate(*u11), gate(*u22)
                        for odd in range(2):
                            last = store_b7(wo7, (2 * cp + odd) * 64 + 8 * a, j * 128,
                                            u11[odd], u12[odd], u21[odd], u22[odd])
                        if a % 2:
                            yield last
        return _Phase(NC * NC // 2, gen())

    def ffn_prepare(raw, dst, j0, j1, rows=64):
        kh, nh = raw.shape[0] // 2, raw.shape[1] // 2

        def gen():
            for c in range(j0 * 128, j1 * 128, 128):
                for r in range(0, kh, rows):
                    q = [pltpu.bitcast(raw[r0:r0 + rows, c0:c0 + 128], u32)
                         for r0 in (r, kh + r) for c0 in (c, nh + c)]
                    q[0], q[3] = gate(q[0], q[3])
                    yield store_b7(dst, r // 2, c, *q)
        return _Phase((j1 - j0) * kh // rows, gen())

    def layernorm(t, a7, s_ref):
        def gen():
            for r in range(0, T, 16):
                rows = pl.ds(pl.multiple_of(t * T + r, 16), 16)
                acc = None
                for c in range(NC):
                    x = xb[rows, c * 128:(c + 1) * 128]
                    if c == 0:
                        x, = gate(x)
                    acc = x.astype(f32) if acc is None else acc + x.astype(f32)
                mean = jnp.broadcast_to(jnp.sum(acc, axis=-1, keepdims=True) * (1.0 / D), (16, 128))
                yield mean
                mean, = gate(mean)
                acc = None
                for c in range(NC):
                    xc = xb[rows, c * 128:(c + 1) * 128].astype(f32) - mean
                    stage[c, r:r + 16, :] = xc
                    acc = xc * xc if acc is None else acc + xc * xc
                var = jnp.sum(acc, axis=-1, keepdims=True) * (1.0 / D)
                inv = lax.rsqrt(var + TINY)
                stage_inv[r:r + 16, :] = jnp.broadcast_to(inv, (16, 128))
                scale = jnp.broadcast_to((var + TINY) * inv * lax.rsqrt(var + EPS), (16, 128))
                s_ref[r:r + 16, :] = scale
                yield scale
            yield from a7_pieces(stage, stage_inv, a7)
        return _Phase(2 * T // 16 + TH // 16 * NC // 2, gen())

    def project(a7, s_ref, b7, dst, row0):
        def emit(half, c, y):
            dst[c, pl.ds(row0 + half * TH, TH), :] = y * s_ref[half * TH:(half + 1) * TH, :]
        return matmul(a7, b7, emit)

    def attn_scores(q, row0, first, r0, r1, chunks):
        def gen():
            for r in range(r0, r1, 8):
                ls = [None] * W
                for c in range(NC):
                    qv, = gate(q[c, r:r + 8, :])
                    for w in range(W):
                        t = qv * kk[c, pl.ds(HALO + row0 + r - DIL * w, 8), :]
                        ls[w] = t if ls[w] is None else ls[w] + t
                    if c % chunks == chunks - 1 and c != NC - 1:
                        yield None
                for w in range(W):
                    t = ls[w] + pltpu.roll(ls[w], 64, 1)
                    t = t + pltpu.roll(t, 32, 1)
                    if first is not None and r < DIL * w:
                        row = lax.broadcasted_iota(jnp.int32, (8, 128), 0) + r
                        t = jnp.where(row < first * (DIL * w), MASKED / SCALE, t)
                    ls[w] = t
                m = ls[0]
                for w in range(1, W):
                    m = jnp.maximum(m, ls[w])
                es = [jnp.exp2((t - m) * (SCALE * LOG2E)) for t in ls]
                total = es[0]
                for w in range(1, W):
                    total = total + es[w]
                inv = 1.0 / total
                for w in range(W):
                    pp[w, r:r + 8, :] = es[w] * inv
                yield inv
        return _Phase((r1 - r0) // 8 * (NC // chunks), gen())

    def attn_mix(row0, o7, s_ref, r0, r1, chunks):
        def gen():
            for r in range(r0, r1, 8):
                ps = [pp[w, r:r + 8, :] for w in range(W)]
                ss = None
                for c in range(NC):
                    if c % chunks == 0:
                        ps = gate(*ps)
                    acc = None
                    for w in range(W):
                        t = ps[w] * vv[c, pl.ds(HALO + row0 + r - DIL * w, 8), :]
                        acc = t if acc is None else acc + t
                    stage[c, r:r + 8, :] = acc
                    ss = acc * acc if ss is None else ss + acc * acc
                    if c % chunks == chunks - 1 and c != NC - 1:
                        yield None
                yield store_row_norm(jnp.sum(ss, axis=-1, keepdims=True), stage_inv, s_ref, r)
            if r1 == T:
                yield from a7_pieces(stage, stage_inv, o7)
        return _Phase((r1 - r0) // 8 * (NC // chunks) + (TH // 16 * NC // 2 if r1 == T else 0), gen())

    def add_residual(t, a7, s_ref, b7, bias_row):
        def emit(half, c, y):
            rows = pl.ds(pl.multiple_of(t * T + half * TH, TH), TH)
            cols = slice(c * 128, (c + 1) * 128)
            z = y * s_ref[half * TH:(half + 1) * TH, :]
            if bias_row is not None:
                z = z + bias[bias_row + c:bias_row + c + 1, :]
            xb[rows, cols] = (xb[rows, cols].astype(f32) + z).astype(bf16)
        return matmul(a7, b7, emit)

    def attn_out(t, o7, s_ref):
        return add_residual(t, o7, s_ref, wo7, None)

    def ffn_up():
        started = [False, False]

        def emit(half, c, y):
            rows = slice(half * TH, (half + 1) * TH)
            z = jnp.maximum(y * sf[rows, :] + bias[c:c + 1, :], 0.0)
            z = z * z
            h_stage[c, rows, :] = z
            h_ss[rows, :] = h_ss[rows, :] + z * z if started[half] else z * z
            started[half] = True
        return matmul(xf7, w17, emit)

    def ffn_mid():
        def gen():
            for r in range(0, T, 32):
                ss, = gate(h_ss[r:r + 32, :])
                yield store_row_norm(jnp.sum(ss, axis=-1, keepdims=True), h_inv, sh, r)
            yield from a7_pieces(h_stage, h_inv, h7)
        return _Phase(T // 32 + TH // 16 * NF // 2, gen())

    def ffn_down(t):
        return add_residual(t, h7, sh, w27, 32)

    def move_halo(ref, src, dst):
        for c in range(NC):
            ref[c, pl.ds(dst, HALO), :] = ref[c, pl.ds(src, HALO), :]

    k0, k1, k2 = HALO, HALO + T, HALO + 2 * T
    wait(x_copy(0))
    solo(layernorm(0, xa7, sa))
    wait(wqkv_copy(0))
    solo(qkv_skew(0))
    wait(x_copy(1))
    solo(qkv_finish(wq7, 0, 1))
    run(project(xa7, sa, wq7, qa, 0), _mix(qkv_finish(wq7, 1, 4), layernorm(1, xb7, sb)), lag=1)
    wait(wqkv_copy(1))
    run(project(xb7, sb, wq7, qb, 0), qkv_skew(1), qkv_finish(wk7, 0, 2))
    wait(wqkv_copy(2))
    run(_chain(project(xa7, sa, wk7, kk, k0), project(xb7, sb, wk7, kk, k1)),
        qkv_finish(wk7, 2, 4), qkv_skew(2), qkv_finish(wv7, 0, 4), lag=1)
    for c in range(NC):
        kk[c, 0:HALO, :] = jnp.zeros((HALO, 128), f32)
    wait(wo_copy)
    run(project(xa7, sa, wv7, vv, k0), attn_scores(qa, 0, 1, 0, T, NC), wo_stage())
    for c in range(NC):
        vv[c, 0:HALO, :] = jnp.broadcast_to(vv[c, HALO:HALO + 1, :], (HALO, 128))
    wait(x_copy(2))
    run(project(xb7, sb, wv7, vv, k1), layernorm(2, xa7, sa), lead=0)
    run(project(xa7, sa, wq7, qa, 0), wo_finish(), attn_mix(0, oa7, soa, 0, TH, NC), lead=0)
    run(project(xa7, sa, wk7, kk, k2), attn_mix(0, oa7, soa, TH, T, NC), attn_scores(qb, T, None, 0, TH, NC), lead=0)
    wait(w1_copy)
    run(project(xa7, sa, wv7, vv, k2), attn_scores(qb, T, None, TH, T, NC), attn_mix(T, ob7, sob, 0, 64, NC),
        ffn_prepare(w1_raw, w17, 0, 5), lead=0)
    run(attn_out(0, oa7, soa), attn_mix(T, ob7, sob, 64, T, NC))
    wait(x_copy(3))
    run(attn_out(1, ob7, sob), layernorm(0, xf7, sf), ffn_prepare(w1_raw, w17, 5, NF // 2), lead=0, lag=1)
    run(ffn_up(), attn_scores(qa, 2 * T, None, 0, T, NC), attn_mix(2 * T, oa7, soa, 0, T, NC),
        layernorm(3, xa7, sa))
    move_halo(kk, 3 * T, T)
    move_halo(vv, 3 * T, T)
    wait(w2_copy)
    run(attn_out(2, oa7, soa), ffn_prepare(w2_raw, w27, 0, NC // 2), lead=0)

    sched.barrier()
    sched.lag = 2

    def step(i, _):
        t_attn = (i + SKEW) % NT
        first = (t_attn == 0).astype(jnp.int32)

        @pl.when(i + SKEW + 1 < NT)
        def _():
            x_copy(i + SKEW + 1).wait()

        move_halo(kk, T, 0)
        move_halo(vv, T, 0)
        run(_chain(project(xa7, sa, wq7, qa, 0), project(xa7, sa, wk7, kk, k0)),
            layernorm((i + 1) % NT, xf7, sf), ffn_mid())
        run(project(xa7, sa, wv7, vv, k0), attn_scores(qa, 0, first, 0, 112, 4))
        for c in range(NC):
            v0 = jnp.broadcast_to(vv[c, HALO:HALO + 1, :], (HALO, 128))
            vv[c, 0:HALO, :] = jnp.where(t_attn == 0, v0, vv[c, 0:HALO, :])
        run(ffn_down(i % NT), attn_scores(qa, 0, first, 112, T, 4), attn_mix(0, oa7, soa, 0, T, 4))
        solo(attn_out(t_attn, oa7, soa))
        run(ffn_up(), layernorm((i + SKEW + 1) % NT, xa7, sa), lead=2)
        sched.barrier()

        @pl.when(i >= NT)
        def _():
            o_copy(i - NT).start()
        return 0

    lax.fori_loop(0, 2 * NT - SKEW, step, 0)

    def drain(t, _):
        solo(ffn_mid())
        run(ffn_down(t), layernorm((t + 1) % NT, xf7, sf), lead=2)
        sched.barrier()
        o_copy(t).start()

        @pl.when(t < NT - 1)
        def _():
            solo(ffn_up())
        return 0

    lax.fori_loop(NT - SKEW, NT, drain, 0)
    for t in range(NT):
        o_copy(t).wait()


def _scratch_shapes():
    vmem = pltpu.VMEM
    lhs = vmem((7, T // 4, D // 2), u32)
    square = vmem((7, D // 4, D // 2), u32)
    per_row = vmem((T, 128), f32)
    chunks = vmem((NC, T, 128), f32)
    window = vmem((NC, HALO + 3 * T, 128), f32)
    return [
        vmem((S, D), bf16),
        vmem((3, D, D), bf16), vmem((D, D), bf16),
        vmem((D, F), bf16), vmem((F, D), bf16),
        vmem((NC, D // 2, 128), u32),
        vmem((NC, PAD * D // 64, 128), u32),
        square, square, square, square,
        vmem((7, D // 4, F // 2), u32), vmem((7, F // 4, D // 2), u32),
        vmem((40, 128), f32),
        lhs, lhs, lhs, lhs, lhs, vmem((7, T // 4, F // 2), u32),
        per_row, per_row, per_row, per_row, per_row, per_row,
        chunks, per_row, vmem((NF, T, 128), f32), per_row, per_row,
        chunks, chunks, window, window, vmem((W, T, 128), f32),
        vmem((8, 128), u32),
        pltpu.SemaphoreType.DMA((NT,)), pltpu.SemaphoreType.DMA((6,)), pltpu.SemaphoreType.DMA((NT,)),
    ]


@jax.jit
def pallas_interleave_layers__sliding_local_dilated__dense_activation_squared_relu__prompt_kernel(
    A_x: jax.Array,
    A_wqkv: jax.Array,
    A_wo: jax.Array,
    B_x: jax.Array,
    B_w1: jax.Array,
    B_b1: jax.Array,
    B_w2: jax.Array,
    B_b2: jax.Array,
):
    del B_x
    hbm = pl.BlockSpec(memory_space=pl.ANY)
    vmem = pl.BlockSpec(memory_space=pltpu.VMEM)
    out = pl.pallas_call(
        _kernel,
        in_specs=[hbm, hbm, hbm, hbm, vmem, hbm, vmem],
        out_specs=hbm,
        out_shape=jax.ShapeDtypeStruct((S, D), bf16),
        scratch_shapes=_scratch_shapes(),
        compiler_params=pltpu.CompilerParams(vmem_limit_bytes=110 * 2 ** 20),
    )(A_x.reshape(S, D), A_wqkv, A_wo, B_w1, B_b1.reshape(NF, 128), B_w2, B_b2.reshape(NC, 128))
    return out.reshape(1, S, D)
```

```python
import jax
import jax.numpy as jnp
from jax import lax
from jax.experimental import pallas as pl
from jax.experimental.pallas import tpu as pltpu

S, D, F = 2048, 1024, 3584
DH, W, DIL = 32, 8, 2
EPS = 1e-5
SCALE = DH ** -0.5
MASKED = -1e9
LOG2E = 1.4426950408889634
TINY = 1e-36

T = 256
TH = T // 2
NT = S // T
HALO = 16
NC = D // 128
NF = F // 128
SKEW = 3
PAD = DH + 1

f32 = jnp.float32
bf16 = jnp.bfloat16
u32 = jnp.uint32


def _pack_rows(x):
    return pltpu.bitcast(x.astype(bf16), u32)


def _as_bf16(u):
    return pltpu.bitcast(u, bf16)


def _halves(u):
    return [pltpu.unpack_elementwise(u, index=i, packed_dtype=bf16, unpacked_dtype=f32) for i in range(2)]


def _pack_op(op, a, b):
    return pltpu.pack_elementwise([op(a[0], b[0]), op(a[1], b[1])], packed_dtype=bf16)


class _Phase:
    def __init__(self, n, gen):
        self.n, self.gen = n, gen


def _chain(*phases):
    def gen():
        for p in phases:
            yield from p.gen
    return _Phase(sum(p.n for p in phases), gen())


def _take(phase, n):
    return _Phase(n, (next(phase.gen) for _ in range(n)))


def _mix(a, b):
    def gen():
        done = 0
        for i in range(a.n):
            yield next(a.gen)
            while done < (i + 1) * b.n // a.n:
                yield next(b.gen)
                done += 1
    return _Phase(a.n + b.n, gen())


class _Schedule:
    def __init__(self, zero_ref):
        self.zero_ref = zero_ref
        self.results = []
        self.token = None
        self.due = None
        self.carry = {}
        self.lag = 3

    def gate(self, *xs):
        if self.token is None:
            return list(xs)
        zero = pltpu.bitcast(self.token, u32) & self.zero_ref[...]
        out = []
        for x in xs:
            u = pltpu.bitcast(x, u32)
            out.append(pltpu.bitcast(u | jnp.tile(zero, (u.shape[0] // 8, u.shape[1] // 128)), x.dtype))
        return out

    def hold(self, lhs):
        if self.due is None:
            return lhs
        n = min(lhs.shape[1], 512)
        head = [lhs[:8, c:c + 128] | self.due for c in range(0, n, 128)]
        if lhs.shape[1] > n:
            head.append(lhs[:8, n:])
        self.due = None
        return jnp.concatenate([jnp.concatenate(head, axis=1), lhs[8:]], axis=0)

    def run(self, main, *side, lead=1, lag=None):
        lag = self.lag if lag is None else lag
        side = _chain(*side)
        slots = max(main.n - lead, 1)
        dues, done = dict(self.carry), 0
        self.carry = {}
        for i in range(main.n):
            self.results = []
            self.due = dues.pop(i, None)
            next(main.gen)
            tokens = [(y, r) for y in self.results for r in range(0, y.shape[0], 8)]
            want = min(side.n, -(-side.n * (i + 1) // slots))
            finished = None
            for j in range(want - done):
                y, r = tokens[j * len(tokens) // (want - done)]
                self.token = y[r:r + 8]
                last = next(side.gen)
                if last is not None:
                    last = pltpu.bitcast(last, u32)[:8, :128]
                    finished = last if finished is None else finished & last
            if finished is not None:
                dues[i + lag] = finished & self.zero_ref[...]
            done = want
        self.token = self.due = None
        self.carry = {i - main.n: z for i, z in dues.items()}
        for p in (main, side):
            assert next(p.gen, _Schedule) is _Schedule, "wrong piece count"

    def solo(self, *phases):
        self.due = self.carry.pop(0, None)
        self.carry = {}
        for p in phases:
            for _ in p.gen:
                pass
        self.due = None

    def barrier(self):
        self.carry = {}


def _kernel(x_hbm, wqkv_hbm, wo_hbm, w1_hbm, b1_ref, w2_hbm, b2_ref, o_hbm,
            xb, wqkv_raw, wo_raw, w1_raw, w2_raw, w_tmp, wo_tmp,
            wq7, wk7, wv7, wo7, w17, w27, bias,
            xa7, xb7, xf7, oa7, ob7, ha7, hb7, sa, sb, sf, soa, sob, sh,
            stage, stage_inv, h_stage, h_inv, h_ss,
            qa, qb, kk, vv, pp, zero_ref, sem_x, sem_w, sem_o):
    def x_copy(t):
        return pltpu.make_async_copy(x_hbm.at[pl.ds(t * T, T)], xb.at[pl.ds(t * T, T)], sem_x.at[t])

    def o_copy(t):
        return pltpu.make_async_copy(xb.at[pl.ds(t * T, T)], o_hbm.at[pl.ds(t * T, T)], sem_o.at[t])

    def wq_copy(half):
        rows = pl.ds(half * (D // 2), D // 2)
        return pltpu.make_async_copy(wqkv_hbm.at[rows, pl.ds(0, D)], wqkv_raw.at[0, rows], sem_w.at[half])

    def wkv_copy(i):
        return pltpu.make_async_copy(wqkv_hbm.at[:, pl.ds(i * D, D)], wqkv_raw.at[i], sem_w.at[1 + i])

    wo_copy = pltpu.make_async_copy(wo_hbm, wo_raw, sem_w.at[4])
    w1_copy = pltpu.make_async_copy(w1_hbm, w1_raw, sem_w.at[5])
    w2_copy = pltpu.make_async_copy(w2_hbm, w2_raw, sem_w.at[6])

    for copy in (x_copy(0), wq_copy(0), wq_copy(1), x_copy(1), wkv_copy(1), x_copy(2), wkv_copy(2), wo_copy,
                 x_copy(3), w1_copy, w2_copy, *[x_copy(t) for t in range(4, NT)]):
        copy.start()

    bias[0:NF, :] = b1_ref[...].astype(f32)
    bias[32:32 + NC, :] = b2_ref[...].astype(f32)
    zero_ref[...] = jnp.zeros((8, 128), u32)

    sched = _Schedule(zero_ref)
    tuning = [512, 0]
    gate, run, solo = sched.gate, sched.run, sched.solo

    def wait(copy):
        sched.barrier()
        copy.wait()

    def store_b7(dst, row, col, u11, u12, u21, u22):
        b11, b12, b21, b22 = (_halves(u) for u in (u11, u12, u21, u22))
        at = (pl.ds(row, u11.shape[0]), pl.ds(col, 128))
        dst[(0,) + at] = _pack_op(lax.add, b11, b22)
        dst[(1,) + at] = u11
        dst[(2,) + at] = _pack_op(lax.sub, b12, b22)
        dst[(3,) + at] = _pack_op(lax.sub, b21, b11)
        dst[(4,) + at] = u22
        dst[(5,) + at] = _pack_op(lax.add, b11, b12)
        last = _pack_op(lax.add, b21, b22)
        dst[(6,) + at] = last
        return last

    def a7_pieces(src, inv, dst):
        nk = src.shape[0] // 2
        for r in range(0, TH, 16):
            top, bot = inv[r:r + 16, :], inv[TH + r:TH + r + 16, :]
            for j in range(nk):
                top, bot = gate(top, bot)
                a11, a12, a21, a22 = (src[c, r0:r0 + 16, :] * scale
                                      for r0, scale in ((r, top), (TH + r, bot)) for c in (j, nk + j))
                at = (slice(r // 2, r // 2 + 8), slice(j * 128, (j + 1) * 128))
                dst[(0,) + at] = _pack_rows(a11 + a22)
                dst[(1,) + at] = _pack_rows(a21 + a22)
                dst[(2,) + at] = _pack_rows(a11)
                dst[(3,) + at] = _pack_rows(a22)
                dst[(4,) + at] = _pack_rows(a11 + a12)
                dst[(5,) + at] = _pack_rows(a21 - a11)
                last = _pack_rows(a12 - a22)
                dst[(6,) + at] = last
                yield last

    def matmul(a7, b7, emit):
        kh, nh = a7.shape[2], b7.shape[2] // 128
        k_step, order = tuning

        def product(i, j):
            y = None
            for k in range(0, kh, k_step):
                ke = min(k + k_step, kh)
                yk = lax.dot_general(_as_bf16(sched.hold(a7[i, :, k:ke])),
                                     _as_bf16(b7[i, k // 2:ke // 2, j * 128:(j + 1) * 128]),
                                     (((1,), (0,)), ((), ())), preferred_element_type=f32)
                sched.results.append(yk)
                y = yk if y is None else y + yk
            return y

        def gen():
            for j in range(nh):
                if order == 0:
                    m1, m2 = product(0, j), product(1, j)
                    c22 = m1 - m2
                    m4 = product(3, j)
                    emit(1, j, m2 + m4)
                    c11 = m1 + m4
                    c11 = c11 + product(6, j)
                    m5 = product(4, j)
                    emit(0, j, c11 - m5)
                    m3 = product(2, j)
                    emit(0, nh + j, m3 + m5)
                    c22 = c22 + m3
                    emit(1, nh + j, c22 + product(5, j))
                else:
                    m6, m2 = product(5, j), product(1, j)
                    c22 = m6 - m2
                    m3 = product(2, j)
                    c22 = c22 + m3
                    m1 = product(0, j)
                    emit(1, nh + j, c22 + m1)
                    m5 = product(4, j)
                    emit(0, nh + j, m3 + m5)
                    c11 = m1 - m5
                    m4 = product(3, j)
                    emit(1, j, m2 + m4)
                    c11 = c11 + m4
                    emit(0, j, c11 + product(6, j))
                yield
        return _Phase(nh, gen())

    def store_row_norm(ss, inv_ref, s_ref, r):
        ss = ss + TINY
        inv = lax.rsqrt(ss)
        shape = (ss.shape[0], 128)
        inv_ref[r:r + shape[0], :] = jnp.broadcast_to(inv, shape)
        norm = jnp.broadcast_to(ss * inv, shape)
        s_ref[r:r + shape[0], :] = norm
        return norm

    def qkv_skew(i, r0=0, r1=D):
        def gen(group=4):
            lane = lax.broadcasted_iota(jnp.int32, (8, 128), 1)
            bits = [(lane & (1 << b)) != 0 for b in range(3)]
            for g0 in range(r0 // 16, r1 // 16, group):
                xs = [[None] * NC for _ in range(group)]
                for c in range(NC):
                    for g in range(group):
                        rows = slice((g0 + g) * 16, (g0 + g + 1) * 16)
                        u, = gate(pltpu.bitcast(wqkv_raw[i, rows, c * 128:(c + 1) * 128], u32))
                        xs[g][c] = pltpu.roll(u, c, 1) if c else u
                for g in range(group):
                    ws = [xs[g][(-c) % NC] for c in range(NC)]
                    for b in range(3):
                        ws = [jnp.where(bits[b], ws[(c - (1 << b)) % NC], ws[c]) for c in range(NC)]
                    for c in range(NC):
                        w_tmp[c, (g0 + g) * 8:(g0 + g + 1) * 8, :] = ws[c]
                yield ws[0]
        return _Phase((r1 - r0) // 64, gen())

    def gather_lanes(c, r0):
        lane = lax.broadcasted_iota(jnp.int32, (64, 128), 1)
        base = (lane & 3) * 32 + (lane >> 5) * 8 + ((lane >> 2) & 7)
        for r in range(r0 // 2, r0 // 2 + D // 4, 64):
            u, = gate(w_tmp[c, r:r + 64, :])
            u = jnp.take_along_axis(u, (base + c) & 127, axis=1)
            w_tmp[c, r:r + 64, :] = u
        return u

    def qkv_finish(dst, j0, j1, top_done=False):
        def gen():
            for j in range(j0, j1):
                left, right = j, NC // 2 + j
                for c in (left, right):
                    if not top_done:
                        gather_lanes(c, 0)
                    yield gather_lanes(c, D // 2)
                for r in range(0, D // 4, 16):
                    top, bot = slice(r, r + 16), slice(D // 4 + r, D // 4 + r + 16)
                    last = store_b7(dst, r, j * 128, w_tmp[left, top, :], w_tmp[right, top, :],
                                    w_tmp[left, bot, :], w_tmp[right, bot, :])
                yield last
        return _Phase(3 * (j1 - j0), gen())

    def wo_stage():
        def gen():
            for n in range(NC):
                u, = gate(pltpu.bitcast(wo_raw[:, n * 128:(n + 1) * 128], u32))
                for g in range(D // 64):
                    wo_tmp[n, pl.ds(PAD * g, 32), :] = u[32 * g:32 * (g + 1)]
                yield u
        return _Phase(NC, gen())

    def wo_finish():
        def rows16(n, cp, a):
            start = PAD * 8 * (a % 2) + 4 * (a // 2) + cp
            lo = wo_tmp[n, pl.ds(start, 8, stride=PAD), :]
            hi = wo_tmp[n, pl.ds(start + 16, 8, stride=PAD), :]
            return (lo & u32(0xFFFF)) | (hi << 16), (lo >> 16) | (hi & u32(0xFFFF0000))

        def gen():
            for j in range(NC // 2):
                for cp in range(NC // 4):
                    for a in range(8):
                        u11, u12 = rows16(j, cp, a), rows16(NC // 2 + j, cp, a)
                        u21, u22 = rows16(j, NC // 4 + cp, a), rows16(NC // 2 + j, NC // 4 + cp, a)
                        u11, u22 = gate(*u11), gate(*u22)
                        for odd in range(2):
                            last = store_b7(wo7, (2 * cp + odd) * 64 + 8 * a, j * 128,
                                            u11[odd], u12[odd], u21[odd], u22[odd])
                        if a % 2:
                            yield last
        return _Phase(NC * NC // 2, gen())

    def ffn_prepare(raw, dst, j0, j1, rows=64):
        kh, nh = raw.shape[0] // 2, raw.shape[1] // 2

        def gen():
            for c in range(j0 * 128, j1 * 128, 128):
                for r in range(0, kh, rows):
                    q = [pltpu.bitcast(raw[r0:r0 + rows, c0:c0 + 128], u32)
                         for r0 in (r, kh + r) for c0 in (c, nh + c)]
                    q[0], q[3] = gate(q[0], q[3])
                    yield store_b7(dst, r // 2, c, *q)
        return _Phase((j1 - j0) * kh // rows, gen())

    def layernorm(t, a7, s_ref):
        def gen():
            for r in range(0, T, 16):
                rows = pl.ds(pl.multiple_of(t * T + r, 16), 16)
                acc = None
                for c in range(NC):
                    x = xb[rows, c * 128:(c + 1) * 128]
                    if c == 0:
                        x, = gate(x)
                    acc = x.astype(f32) if acc is None else acc + x.astype(f32)
                mean = jnp.broadcast_to(jnp.sum(acc, axis=-1, keepdims=True) * (1.0 / D), (16, 128))
                yield mean
                mean, = gate(mean)
                acc = None
                for c in range(NC):
                    xc = xb[rows, c * 128:(c + 1) * 128].astype(f32) - mean
                    stage[c, r:r + 16, :] = xc
                    acc = xc * xc if acc is None else acc + xc * xc
                var = jnp.sum(acc, axis=-1, keepdims=True) * (1.0 / D)
                inv = lax.rsqrt(var + TINY)
                stage_inv[r:r + 16, :] = jnp.broadcast_to(inv, (16, 128))
                scale = jnp.broadcast_to((var + TINY) * inv * lax.rsqrt(var + EPS), (16, 128))
                s_ref[r:r + 16, :] = scale
                yield scale
            yield from a7_pieces(stage, stage_inv, a7)
        return _Phase(2 * T // 16 + TH // 16 * NC // 2, gen())

    def project(a7, s_ref, b7, dst, row0):
        def emit(half, c, y):
            dst[c, pl.ds(row0 + half * TH, TH), :] = y * s_ref[half * TH:(half + 1) * TH, :]
        return matmul(a7, b7, emit)

    def attn_scores(q, row0, first, r0, r1, chunks):
        def gen():
            for r in range(r0, r1, 8):
                ls = [None] * W
                for c in range(NC):
                    qv, = gate(q[c, r:r + 8, :])
                    for w in range(W):
                        t = qv * kk[c, pl.ds(HALO + row0 + r - DIL * w, 8), :]
                        ls[w] = t if ls[w] is None else ls[w] + t
                    if c % chunks == chunks - 1 and c != NC - 1:
                        yield None
                for w in range(W):
                    t = ls[w] + pltpu.roll(ls[w], 64, 1)
                    t = t + pltpu.roll(t, 32, 1)
                    if first is not None and r < DIL * w:
                        row = lax.broadcasted_iota(jnp.int32, (8, 128), 0) + r
                        t = jnp.where(row < first * (DIL * w), MASKED / SCALE, t)
                    ls[w] = t
                m = ls[0]
                for w in range(1, W):
                    m = jnp.maximum(m, ls[w])
                es = [jnp.exp2((t - m) * (SCALE * LOG2E)) for t in ls]
                total = es[0]
                for w in range(1, W):
                    total = total + es[w]
                inv = 1.0 / total
                for w in range(W):
                    pp[w, r:r + 8, :] = es[w] * inv
                yield inv
        return _Phase((r1 - r0) // 8 * (NC // chunks), gen())

    def attn_mix(row0, o7, s_ref, r0, r1, chunks):
        def gen():
            for r in range(r0, r1, 8):
                ps = [pp[w, r:r + 8, :] for w in range(W)]
                ss = None
                for c in range(NC):
                    if c % chunks == 0:
                        ps = gate(*ps)
                    acc = None
                    for w in range(W):
                        t = ps[w] * vv[c, pl.ds(HALO + row0 + r - DIL * w, 8), :]
                        acc = t if acc is None else acc + t
                    stage[c, r:r + 8, :] = acc
                    ss = acc * acc if ss is None else ss + acc * acc
                    if c % chunks == chunks - 1 and c != NC - 1:
                        yield None
                yield store_row_norm(jnp.sum(ss, axis=-1, keepdims=True), stage_inv, s_ref, r)
            if r1 == T:
                yield from a7_pieces(stage, stage_inv, o7)
        return _Phase((r1 - r0) // 8 * (NC // chunks) + (TH // 16 * NC // 2 if r1 == T else 0), gen())

    def add_residual(t, a7, s_ref, b7, bias_row):
        def emit(half, c, y):
            rows = pl.ds(pl.multiple_of(t * T + half * TH, TH), TH)
            cols = slice(c * 128, (c + 1) * 128)
            z = y * s_ref[half * TH:(half + 1) * TH, :]
            if bias_row is not None:
                z = z + bias[bias_row + c:bias_row + c + 1, :]
            xb[rows, cols] = (xb[rows, cols].astype(f32) + z).astype(bf16)
        return matmul(a7, b7, emit)

    def attn_out(t, o7, s_ref):
        return add_residual(t, o7, s_ref, wo7, None)

    def ffn_up(a7=xf7, s_ref=sf):
        started = [False, False]

        def emit(half, c, y):
            rows = slice(half * TH, (half + 1) * TH)
            z = jnp.maximum(y * s_ref[rows, :] + bias[c:c + 1, :], 0.0)
            z = z * z
            h_stage[c, rows, :] = z
            h_ss[rows, :] = h_ss[rows, :] + z * z if started[half] else z * z
            started[half] = True
        return matmul(a7, w17, emit)

    def ffn_mid(h7=ha7, s_ref=sh):
        def gen():
            for r in range(0, T, 32):
                ss, = gate(h_ss[r:r + 32, :])
                yield store_row_norm(jnp.sum(ss, axis=-1, keepdims=True), h_inv, s_ref, r)
            yield from a7_pieces(h_stage, h_inv, h7)
        return _Phase(T // 32 + TH // 16 * NF // 2, gen())

    def ffn_down(t, h7=ha7, s_ref=sh):
        return add_residual(t, h7, s_ref, w27, 32)

    def move_halo(ref, src, dst):
        for c in range(NC):
            ref[c, pl.ds(dst, HALO), :] = ref[c, pl.ds(src, HALO), :]

    k0, k1, k2 = HALO, HALO + T, HALO + 2 * T
    wait(x_copy(0))
    solo(layernorm(0, xa7, sa))
    wait(wq_copy(0))
    solo(qkv_skew(0, 0, D // 2))
    for c in range(NC):
        gather_lanes(c, 0)
    wait(wq_copy(1))
    solo(qkv_skew(0, D // 2, D), qkv_finish(wq7, 0, 3, True))
    wait(x_copy(1))
    run(project(xa7, sa, wq7, qa, 0), qkv_finish(wq7, 3, 4, True), layernorm(1, xb7, sb))
    wait(wkv_copy(1))
    run(project(xb7, sb, wq7, qb, 0), qkv_skew(1), qkv_finish(wk7, 0, 3), lag=9)
    run(project(xa7, sa, wk7, kk, k0), qkv_finish(wk7, 3, 4), lead=2, lag=1)
    for c in range(NC):
        kk[c, 0:HALO, :] = jnp.zeros((HALO, 128), f32)
    wait(x_copy(2))
    run(project(xb7, sb, wk7, kk, k1), layernorm(2, xf7, sf), attn_scores(qa, 0, 1, 0, 160, 4), lead=0)
    wait(wkv_copy(2))
    run(project(xf7, sf, wk7, kk, k2), qkv_skew(2), qkv_finish(wv7, 0, 2))
    wait(wo_copy)
    run(project(xa7, sa, wv7, vv, k0), qkv_finish(wv7, 2, 4), attn_scores(qa, 0, 1, 160, T, 4), wo_stage(), lead=0)
    for c in range(NC):
        vv[c, 0:HALO, :] = jnp.broadcast_to(vv[c, HALO:HALO + 1, :], (HALO, 128))
    wait(x_copy(3))
    run(project(xb7, sb, wv7, vv, k1), wo_finish(), attn_mix(0, oa7, soa, 0, 160, 4), lead=0)
    run(project(xf7, sf, wq7, qa, 0), attn_mix(0, oa7, soa, 160, T, 4), attn_scores(qb, T, None, 0, 192, 4), lead=0)
    wait(w1_copy)
    run(project(xf7, sf, wv7, vv, k2), attn_scores(qb, T, None, 192, T, 4), attn_mix(T, ob7, sob, 0, 96, 4),
        ffn_prepare(w1_raw, w17, 0, 4), lead=0)
    run(attn_out(0, oa7, soa), attn_mix(T, ob7, sob, 96, T, 4), ffn_prepare(w1_raw, w17, 4, 8))
    run(attn_out(1, ob7, sob), _mix(layernorm(0, xa7, sa), ffn_prepare(w1_raw, w17, 8, 10)), lag=2)
    run(ffn_up(xa7, sa), ffn_prepare(w1_raw, w17, 10, NF // 2), attn_scores(qa, 2 * T, None, 0, T, 8),
        attn_mix(2 * T, oa7, soa, 0, T, 8), lead=3)
    move_halo(kk, 3 * T, T)
    move_halo(vv, 3 * T, T)
    wait(w2_copy)
    run(attn_out(2, oa7, soa), ffn_prepare(w2_raw, w27, 0, NC // 2, 32), layernorm(3, xa7, sa), lead=0, lag=9)

    sched.barrier()
    tuning[:] = 1024, 1

    def step(i, _):
        t_attn = (i + SKEW) % NT
        first = (t_attn == 0).astype(jnp.int32)

        @pl.when(i + SKEW + 1 < NT)
        def _():
            x_copy(i + SKEW + 1).wait()

        move_halo(kk, T, 0)
        move_halo(vv, T, 0)
        run(_chain(project(xa7, sa, wq7, qa, 0), project(xa7, sa, wk7, kk, k0)),
            layernorm((i + 1) % NT, xf7, sf), ffn_mid(), lag=2)
        run(project(xa7, sa, wv7, vv, k0), attn_scores(qa, 0, first, 0, 112, 8), lead=0, lag=2)
        for c in range(NC):
            v0 = jnp.broadcast_to(vv[c, HALO:HALO + 1, :], (HALO, 128))
            vv[c, 0:HALO, :] = jnp.where(t_attn == 0, v0, vv[c, 0:HALO, :])
        run(ffn_down(i % NT), attn_scores(qa, 0, first, 112, T, 4), attn_mix(0, oa7, soa, 0, T, 4), lag=2)
        solo(attn_out(t_attn, oa7, soa))
        run(ffn_up(), layernorm((i + SKEW + 1) % NT, xa7, sa), lead=5)
        sched.barrier()

        @pl.when(i >= NT)
        def _():
            o_copy(i - NT).start()
        return 0

    lax.fori_loop(0, 2 * NT - SKEW, step, 0)

    down_a, down_b = ffn_down(NT - 3), ffn_down(NT - 2, hb7, sob)
    solo(ffn_mid())
    run(_take(down_a, 2), layernorm(NT - 2, xf7, sf), lead=0)
    run(ffn_up(), layernorm(NT - 1, xa7, sa), lead=6)
    run(_chain(_take(down_a, 2), _take(down_b, 1)), ffn_mid(hb7, sob), lead=2)
    solo(ffn_up(xa7, sa))
    run(_take(down_b, 3), ffn_mid(), lead=0)
    sched.barrier()
    o_copy(NT - 3).start()
    o_copy(NT - 2).start()
    solo(ffn_down(NT - 1))
    o_copy(NT - 1).start()
    for t in range(NT):
        o_copy(t).wait()


def _scratch_shapes():
    vmem = pltpu.VMEM
    lhs = vmem((7, T // 4, D // 2), u32)
    square = vmem((7, D // 4, D // 2), u32)
    per_row = vmem((T, 128), f32)
    chunks = vmem((NC, T, 128), f32)
    window = vmem((NC, HALO + 3 * T, 128), f32)
    return [
        vmem((S, D), bf16),
        vmem((3, D, D), bf16), vmem((D, D), bf16),
        vmem((D, F), bf16), vmem((F, D), bf16),
        vmem((NC, D // 2, 128), u32),
        vmem((NC, PAD * D // 64, 128), u32),
        square, square, square, square,
        vmem((7, D // 4, F // 2), u32), vmem((7, F // 4, D // 2), u32),
        vmem((40, 128), f32),
        lhs, lhs, lhs, lhs, lhs,
        vmem((7, T // 4, F // 2), u32), vmem((7, T // 4, F // 2), u32),
        per_row, per_row, per_row, per_row, per_row, per_row,
        chunks, per_row, vmem((NF, T, 128), f32), per_row, per_row,
        chunks, chunks, window, window, vmem((W, T, 128), f32),
        vmem((8, 128), u32),
        pltpu.SemaphoreType.DMA((NT,)), pltpu.SemaphoreType.DMA((7,)), pltpu.SemaphoreType.DMA((NT,)),
    ]


@jax.jit
def pallas_interleave_layers__sliding_local_dilated__dense_activation_squared_relu__prompt_kernel(
    A_x: jax.Array,
    A_wqkv: jax.Array,
    A_wo: jax.Array,
    B_x: jax.Array,
    B_w1: jax.Array,
    B_b1: jax.Array,
    B_w2: jax.Array,
    B_b2: jax.Array,
):
    del B_x
    hbm = pl.BlockSpec(memory_space=pl.ANY)
    vmem = pl.BlockSpec(memory_space=pltpu.VMEM)
    out = pl.pallas_call(
        _kernel,
        in_specs=[hbm, hbm, hbm, hbm, vmem, hbm, vmem],
        out_specs=hbm,
        out_shape=jax.ShapeDtypeStruct((S, D), bf16),
        scratch_shapes=_scratch_shapes(),
        compiler_params=pltpu.CompilerParams(vmem_limit_bytes=110 * 2 ** 20),
    )(A_x.reshape(S, D), A_wqkv, A_wo, B_w1, B_b1.reshape(NF, 128), B_w2, B_b2.reshape(NC, 128))
    return out.reshape(1, S, D)
```

```python
import jax
import jax.numpy as jnp
from jax import lax
from jax.experimental import pallas as pl
from jax.experimental.pallas import tpu as pltpu

S, D, F = 2048, 1024, 3584
DH, W, DIL = 32, 8, 2
EPS = 1e-5
SCALE = DH ** -0.5
MASKED = -1e9
LOG2E = 1.4426950408889634
TINY = 1e-36

T = 256
TH = T // 2
NT = S // T
HALO = 16
NC = D // 128
NF = F // 128
SKEW = 3
UP_SPLIT = 13
PAD = DH + 1

f32 = jnp.float32
bf16 = jnp.bfloat16
u32 = jnp.uint32


def _pack_rows(x):
    return pltpu.bitcast(x.astype(bf16), u32)


def _as_bf16(u):
    return pltpu.bitcast(u, bf16)


class _Phase:
    def __init__(self, n, gen):
        self.n, self.gen = n, gen


def _chain(*phases):
    def gen():
        for p in phases:
            yield from p.gen
    return _Phase(sum(p.n for p in phases), gen())


def _take(phase, n):
    return _Phase(n, (next(phase.gen) for _ in range(n)))


def _mix(a, b):
    def gen():
        done = 0
        for i in range(a.n):
            yield next(a.gen)
            while done < (i + 1) * b.n // a.n:
                yield next(b.gen)
                done += 1
    return _Phase(a.n + b.n, gen())


class _Schedule:
    def __init__(self, zero_ref):
        self.zero_ref = zero_ref
        self.results = []
        self.token = None
        self.due = None
        self.carry = {}
        self.lag = 3

    def gate(self, *xs):
        if self.token is None:
            return list(xs)
        zero = pltpu.bitcast(self.token, u32) & self.zero_ref[...]
        out = []
        for x in xs:
            u = pltpu.bitcast(x, u32)
            out.append(pltpu.bitcast(u | jnp.tile(zero, (u.shape[0] // 8, u.shape[1] // 128)), x.dtype))
        return out

    def hold(self, lhs):
        if self.due is None:
            return lhs
        n = min(lhs.shape[1], 512)
        head = [lhs[:8, c:c + 128] | self.due for c in range(0, n, 128)]
        if lhs.shape[1] > n:
            head.append(lhs[:8, n:])
        self.due = None
        return jnp.concatenate([jnp.concatenate(head, axis=1), lhs[8:]], axis=0)

    def run(self, main, *side, lead=1, lag=None):
        lag = self.lag if lag is None else lag
        side = _chain(*side)
        slots = max(main.n - lead, 1)
        dues, done = dict(self.carry), 0
        self.carry = {}
        for i in range(main.n):
            self.results = []
            self.due = dues.pop(i, None)
            next(main.gen)
            tokens = [(y, r) for y in self.results for r in range(0, y.shape[0], 8)]
            want = min(side.n, -(-side.n * (i + 1) // slots))
            finished = None
            for j in range(want - done):
                y, r = tokens[j * len(tokens) // (want - done)]
                self.token = y[r:r + 8]
                last = next(side.gen)
                if last is not None:
                    last = pltpu.bitcast(last, u32)[:8, :128]
                    finished = last if finished is None else finished & last
            if finished is not None:
                dues[i + lag] = finished & self.zero_ref[...]
            done = want
        self.token = self.due = None
        self.carry = {i - main.n: z for i, z in dues.items()}
        for p in (main, side):
            assert next(p.gen, _Schedule) is _Schedule, "wrong piece count"

    def solo(self, *phases):
        self.due = self.carry.pop(0, None)
        self.carry = {}
        for p in phases:
            for _ in p.gen:
                pass
        self.due = None

    def barrier(self):
        self.carry = {}


def _kernel(x_hbm, wqkv_hbm, wo_hbm, w1_hbm, b1_ref, w2_hbm, b2_ref, o_hbm,
            xb, wqkv_raw, wo_raw, w1_raw, w2_raw, w_tmp, wo_tmp,
            wq7, wk7, wv7, wo7, w17, w27, bias,
            xa7, xb7, xf7, oa7, ob7, ha7, hb7, sa, sb, sf, soa, sob, sh,
            stage, stage_inv, h_stage, h_inv, h_ss,
            qa, qb, kk, vv, pp, zero_ref, sem_x, sem_w, sem_o):
    def x_copy(t):
        return pltpu.make_async_copy(x_hbm.at[pl.ds(t * T, T)], xb.at[pl.ds(t * T, T)], sem_x.at[t])

    def o_copy(t):
        return pltpu.make_async_copy(xb.at[pl.ds(t * T, T)], o_hbm.at[pl.ds(t * T, T)], sem_o.at[t])

    def wq_copy(half):
        rows = pl.ds(half * (D // 2), D // 2)
        return pltpu.make_async_copy(wqkv_hbm.at[rows, pl.ds(0, D)], wqkv_raw.at[0, rows], sem_w.at[half])

    def wkv_copy(i):
        return pltpu.make_async_copy(wqkv_hbm.at[:, pl.ds(i * D, D)], wqkv_raw.at[i], sem_w.at[1 + i])

    wo_copy = pltpu.make_async_copy(wo_hbm, wo_raw, sem_w.at[4])
    w1_copy = pltpu.make_async_copy(w1_hbm, w1_raw, sem_w.at[5])
    w2_copy = pltpu.make_async_copy(w2_hbm, w2_raw, sem_w.at[6])

    for copy in (x_copy(0), wq_copy(0), wq_copy(1), x_copy(1), wkv_copy(1), x_copy(2), wkv_copy(2), wo_copy,
                 x_copy(3), w1_copy, w2_copy, *[x_copy(t) for t in range(4, NT)]):
        copy.start()

    bias[0:NF, :] = b1_ref[...].astype(f32)
    bias[32:32 + NC, :] = b2_ref[...].astype(f32)
    zero_ref[...] = jnp.zeros((8, 128), u32)

    sched = _Schedule(zero_ref)
    tuning = [512, 0]
    gate, run, solo = sched.gate, sched.run, sched.solo

    def wait(copy):
        sched.barrier()
        copy.wait()

    def store_b7(dst, row, col, u11, u12, u21, u22):
        b11, b12, b21, b22 = (_as_bf16(u).astype(f32) for u in (u11, u12, u21, u22))
        at = (pl.ds(row, u11.shape[0]), pl.ds(col, 128))
        dst[(0,) + at] = _pack_rows(b11 + b22)
        dst[(1,) + at] = u11
        dst[(2,) + at] = _pack_rows(b12 - b22)
        dst[(3,) + at] = _pack_rows(b21 - b11)
        dst[(4,) + at] = u22
        dst[(5,) + at] = _pack_rows(b11 + b12)
        last = _pack_rows(b21 + b22)
        dst[(6,) + at] = last
        return last

    def a7_pieces(src, inv, dst):
        nk = src.shape[0] // 2
        for r in range(0, TH, 16):
            top, bot = inv[r:r + 16, :], inv[TH + r:TH + r + 16, :]
            for j in range(nk):
                top, bot = gate(top, bot)
                a11, a12, a21, a22 = (src[c, r0:r0 + 16, :] * scale
                                      for r0, scale in ((r, top), (TH + r, bot)) for c in (j, nk + j))
                at = (slice(r // 2, r // 2 + 8), slice(j * 128, (j + 1) * 128))
                dst[(0,) + at] = _pack_rows(a11 + a22)
                dst[(1,) + at] = _pack_rows(a21 + a22)
                dst[(2,) + at] = _pack_rows(a11)
                dst[(3,) + at] = _pack_rows(a22)
                dst[(4,) + at] = _pack_rows(a11 + a12)
                dst[(5,) + at] = _pack_rows(a21 - a11)
                last = _pack_rows(a12 - a22)
                dst[(6,) + at] = last
                yield last

    def matmul(a7, b7, emit, j0=0, j1=None):
        kh, nh = a7.shape[2], b7.shape[2] // 128
        k_step, order = tuning
        j1 = nh if j1 is None else j1

        def product(i, j):
            y = None
            for k in range(0, kh, k_step):
                ke = min(k + k_step, kh)
                yk = lax.dot_general(_as_bf16(sched.hold(a7[i, :, k:ke])),
                                     _as_bf16(b7[i, k // 2:ke // 2, j * 128:(j + 1) * 128]),
                                     (((1,), (0,)), ((), ())), preferred_element_type=f32)
                sched.results.append(yk)
                y = yk if y is None else y + yk
            return y

        def gen():
            for j in range(j0, j1):
                if order == 0:
                    m1, m2 = product(0, j), product(1, j)
                    c22 = m1 - m2
                    m4 = product(3, j)
                    emit(1, j, m2 + m4)
                    c11 = m1 + m4
                    c11 = c11 + product(6, j)
                    m5 = product(4, j)
                    emit(0, j, c11 - m5)
                    m3 = product(2, j)
                    emit(0, nh + j, m3 + m5)
                    c22 = c22 + m3
                    emit(1, nh + j, c22 + product(5, j))
                else:
                    m6, m2 = product(5, j), product(1, j)
                    c22 = m6 - m2
                    m3 = product(2, j)
                    c22 = c22 + m3
                    m1 = product(0, j)
                    emit(1, nh + j, c22 + m1)
                    m5 = product(4, j)
                    emit(0, nh + j, m3 + m5)
                    c11 = m1 - m5
                    m4 = product(3, j)
                    emit(1, j, m2 + m4)
                    c11 = c11 + m4
                    emit(0, j, c11 + product(6, j))
                yield
        return _Phase(j1 - j0, gen())

    def store_row_norm(ss, inv_ref, s_ref, r):
        ss = ss + TINY
        inv = lax.rsqrt(ss)
        shape = (ss.shape[0], 128)
        inv_ref[r:r + shape[0], :] = jnp.broadcast_to(inv, shape)
        norm = jnp.broadcast_to(ss * inv, shape)
        s_ref[r:r + shape[0], :] = norm
        return norm

    def qkv_skew(i, r0=0, r1=D):
        def gen(group=4):
            lane = lax.broadcasted_iota(jnp.int32, (8, 128), 1)
            bits = [(lane & (1 << b)) != 0 for b in range(3)]
            for g0 in range(r0 // 16, r1 // 16, group):
                xs = [[None] * NC for _ in range(group)]
                for c in range(NC):
                    for g in range(group):
                        rows = slice((g0 + g) * 16, (g0 + g + 1) * 16)
                        u, = gate(pltpu.bitcast(wqkv_raw[i, rows, c * 128:(c + 1) * 128], u32))
                        xs[g][c] = pltpu.roll(u, c, 1) if c else u
                for g in range(group):
                    ws = [xs[g][(-c) % NC] for c in range(NC)]
                    for b in range(3):
                        ws = [jnp.where(bits[b], ws[(c - (1 << b)) % NC], ws[c]) for c in range(NC)]
                    for c in range(NC):
                        w_tmp[c, (g0 + g) * 8:(g0 + g + 1) * 8, :] = ws[c]
                yield ws[0]
        return _Phase((r1 - r0) // 64, gen())

    def gather_lanes(c, r0):
        lane = lax.broadcasted_iota(jnp.int32, (64, 128), 1)
        base = (lane & 3) * 32 + (lane >> 5) * 8 + ((lane >> 2) & 7)
        for r in range(r0 // 2, r0 // 2 + D // 4, 64):
            u, = gate(w_tmp[c, r:r + 64, :])
            u = jnp.take_along_axis(u, (base + c) & 127, axis=1)
            w_tmp[c, r:r + 64, :] = u
        return u

    def qkv_finish(dst, j0, j1, top_done=False):
        def gen():
            for j in range(j0, j1):
                left, right = j, NC // 2 + j
                for c in (left, right):
                    if not top_done:
                        gather_lanes(c, 0)
                    yield gather_lanes(c, D // 2)
                for r in range(0, D // 4, 16):
                    top, bot = slice(r, r + 16), slice(D // 4 + r, D // 4 + r + 16)
                    last = store_b7(dst, r, j * 128, w_tmp[left, top, :], w_tmp[right, top, :],
                                    w_tmp[left, bot, :], w_tmp[right, bot, :])
                yield last
        return _Phase(3 * (j1 - j0), gen())

    def wo_stage():
        def gen():
            for n in range(NC):
                u, = gate(pltpu.bitcast(wo_raw[:, n * 128:(n + 1) * 128], u32))
                for g in range(D // 64):
                    wo_tmp[n, pl.ds(PAD * g, 32), :] = u[32 * g:32 * (g + 1)]
                yield u
        return _Phase(NC, gen())

    def wo_finish():
        def rows16(n, cp, a):
            start = PAD * 8 * (a % 2) + 4 * (a // 2) + cp
            lo = wo_tmp[n, pl.ds(start, 8, stride=PAD), :]
            hi = wo_tmp[n, pl.ds(start + 16, 8, stride=PAD), :]
            return (lo & u32(0xFFFF)) | (hi << 16), (lo >> 16) | (hi & u32(0xFFFF0000))

        def gen():
            for j in range(NC // 2):
                for cp in range(NC // 4):
                    for a in range(8):
                        u11, u12 = rows16(j, cp, a), rows16(NC // 2 + j, cp, a)
                        u21, u22 = rows16(j, NC // 4 + cp, a), rows16(NC // 2 + j, NC // 4 + cp, a)
                        u11, u22 = gate(*u11), gate(*u22)
                        for odd in range(2):
                            last = store_b7(wo7, (2 * cp + odd) * 64 + 8 * a, j * 128,
                                            u11[odd], u12[odd], u21[odd], u22[odd])
                        if a % 2:
                            yield last
        return _Phase(NC * NC // 2, gen())

    def ffn_prepare(raw, dst, j0, j1, rows=64):
        kh, nh = raw.shape[0] // 2, raw.shape[1] // 2

        def gen():
            for c in range(j0 * 128, j1 * 128, 128):
                for r in range(0, kh, rows):
                    q = [pltpu.bitcast(raw[r0:r0 + rows, c0:c0 + 128], u32)
                         for r0 in (r, kh + r) for c0 in (c, nh + c)]
                    q[0], q[3] = gate(q[0], q[3])
                    yield store_b7(dst, r // 2, c, *q)
        return _Phase((j1 - j0) * kh // rows, gen())

    def layernorm(t, a7, s_ref):
        def gen():
            for r in range(0, T, 16):
                rows = pl.ds(pl.multiple_of(t * T + r, 16), 16)
                acc = None
                for c in range(NC):
                    x = xb[rows, c * 128:(c + 1) * 128]
                    if c == 0:
                        x, = gate(x)
                    acc = x.astype(f32) if acc is None else acc + x.astype(f32)
                mean = jnp.broadcast_to(jnp.sum(acc, axis=-1, keepdims=True) * (1.0 / D), (16, 128))
                yield mean
                mean, = gate(mean)
                acc = None
                for c in range(NC):
                    xc = xb[rows, c * 128:(c + 1) * 128].astype(f32) - mean
                    stage[c, r:r + 16, :] = xc
                    acc = xc * xc if acc is None else acc + xc * xc
                var = jnp.sum(acc, axis=-1, keepdims=True) * (1.0 / D)
                inv = lax.rsqrt(var + TINY)
                stage_inv[r:r + 16, :] = jnp.broadcast_to(inv, (16, 128))
                scale = jnp.broadcast_to((var + TINY) * inv * lax.rsqrt(var + EPS), (16, 128))
                s_ref[r:r + 16, :] = scale
                yield scale
            yield from a7_pieces(stage, stage_inv, a7)
        return _Phase(2 * T // 16 + TH // 16 * NC // 2, gen())

    def project(a7, s_ref, b7, dst, row0):
        def emit(half, c, y):
            dst[c, pl.ds(row0 + half * TH, TH), :] = y * s_ref[half * TH:(half + 1) * TH, :]
        return matmul(a7, b7, emit)

    def attn_scores(q, row0, first, r0, r1, chunks):
        def gen():
            for r in range(r0, r1, 8):
                ls = [None] * W
                for c in range(NC):
                    qv, = gate(q[c, r:r + 8, :])
                    for w in range(W):
                        t = qv * kk[c, pl.ds(HALO + row0 + r - DIL * w, 8), :]
                        ls[w] = t if ls[w] is None else ls[w] + t
                    if c % chunks == chunks - 1 and c != NC - 1:
                        yield None
                for w in range(W):
                    t = ls[w] + pltpu.roll(ls[w], 64, 1)
                    t = t + pltpu.roll(t, 32, 1)
                    if first is not None and r < DIL * w:
                        row = lax.broadcasted_iota(jnp.int32, (8, 128), 0) + r
                        t = jnp.where(row < first * (DIL * w), MASKED / SCALE, t)
                    ls[w] = t
                m = ls[0]
                for w in range(1, W):
                    m = jnp.maximum(m, ls[w])
                es = [jnp.exp2((t - m) * (SCALE * LOG2E)) for t in ls]
                total = es[0]
                for w in range(1, W):
                    total = total + es[w]
                inv = 1.0 / total
                for w in range(W):
                    pp[w, r:r + 8, :] = es[w] * inv
                yield inv
        return _Phase((r1 - r0) // 8 * (NC // chunks), gen())

    def attn_mix(row0, o7, s_ref, r0, r1, chunks):
        def gen():
            for r in range(r0, r1, 8):
                ps = [pp[w, r:r + 8, :] for w in range(W)]
                ss = None
                for c in range(NC):
                    if c % chunks == 0:
                        ps = gate(*ps)
                    acc = None
                    for w in range(W):
                        t = ps[w] * vv[c, pl.ds(HALO + row0 + r - DIL * w, 8), :]
                        acc = t if acc is None else acc + t
                    stage[c, r:r + 8, :] = acc
                    ss = acc * acc if ss is None else ss + acc * acc
                    if c % chunks == chunks - 1 and c != NC - 1:
                        yield None
                yield store_row_norm(jnp.sum(ss, axis=-1, keepdims=True), stage_inv, s_ref, r)
            if r1 == T:
                yield from a7_pieces(stage, stage_inv, o7)
        return _Phase((r1 - r0) // 8 * (NC // chunks) + (TH // 16 * NC // 2 if r1 == T else 0), gen())

    def add_residual(t, a7, s_ref, b7, bias_row):
        def emit(half, c, y):
            rows = pl.ds(pl.multiple_of(t * T + half * TH, TH), TH)
            cols = slice(c * 128, (c + 1) * 128)
            z = y * s_ref[half * TH:(half + 1) * TH, :]
            if bias_row is not None:
                z = z + bias[bias_row + c:bias_row + c + 1, :]
            xb[rows, cols] = (xb[rows, cols].astype(f32) + z).astype(bf16)
        return matmul(a7, b7, emit)

    def attn_out(t, o7, s_ref):
        return add_residual(t, o7, s_ref, wo7, None)

    def ffn_up(j0=0, j1=NF // 2, a7=xf7, s_ref=sf):
        started = [j0 > 0, j0 > 0]

        def emit(half, c, y):
            rows = slice(half * TH, (half + 1) * TH)
            z = jnp.maximum(y * s_ref[rows, :] + bias[c:c + 1, :], 0.0)
            z = z * z
            h_stage[c, rows, :] = z
            h_ss[rows, :] = h_ss[rows, :] + z * z if started[half] else z * z
            started[half] = True
        return matmul(a7, w17, emit, j0, j1)

    def ffn_mid(h7=ha7, s_ref=sh):
        def gen():
            for r in range(0, T, 32):
                ss, = gate(h_ss[r:r + 32, :])
                yield store_row_norm(jnp.sum(ss, axis=-1, keepdims=True), h_inv, s_ref, r)
            yield from a7_pieces(h_stage, h_inv, h7)
        return _Phase(T // 32 + TH // 16 * NF // 2, gen())

    def ffn_down(t, h7=ha7, s_ref=sh):
        return add_residual(t, h7, s_ref, w27, 32)

    def move_halo(ref, src, dst):
        for c in range(NC):
            ref[c, pl.ds(dst, HALO), :] = ref[c, pl.ds(src, HALO), :]

    k0, k1, k2 = HALO, HALO + T, HALO + 2 * T
    wait(x_copy(0))
    solo(layernorm(0, xa7, sa))
    wait(wq_copy(0))
    solo(qkv_skew(0, 0, D // 2))
    for c in range(NC):
        gather_lanes(c, 0)
    wait(wq_copy(1))
    solo(qkv_skew(0, D // 2, D), qkv_finish(wq7, 0, 3, True))
    wait(x_copy(1))
    run(project(xa7, sa, wq7, qa, 0), qkv_finish(wq7, 3, 4, True), layernorm(1, xb7, sb))
    wait(wkv_copy(1))
    run(project(xb7, sb, wq7, qb, 0), qkv_skew(1), qkv_finish(wk7, 0, 3), lag=9)
    run(project(xa7, sa, wk7, kk, k0), qkv_finish(wk7, 3, 4), lead=2, lag=1)
    for c in range(NC):
        kk[c, 0:HALO, :] = jnp.zeros((HALO, 128), f32)
    wait(x_copy(2))
    run(project(xb7, sb, wk7, kk, k1), layernorm(2, xf7, sf), attn_scores(qa, 0, 1, 0, 160, 4), lead=0, lag=9)
    wait(wkv_copy(2))
    run(project(xf7, sf, wk7, kk, k2), qkv_skew(2), qkv_finish(wv7, 0, 2))
    wait(wo_copy)
    run(project(xa7, sa, wv7, vv, k0), qkv_finish(wv7, 2, 4), attn_scores(qa, 0, 1, 160, T, 4), wo_stage(), lead=0)
    for c in range(NC):
        vv[c, 0:HALO, :] = jnp.broadcast_to(vv[c, HALO:HALO + 1, :], (HALO, 128))
    wait(x_copy(3))
    run(project(xb7, sb, wv7, vv, k1), wo_finish(), attn_mix(0, oa7, soa, 0, 160, 4), lead=0, lag=9)
    run(project(xf7, sf, wq7, qa, 0), attn_mix(0, oa7, soa, 160, T, 4), attn_scores(qb, T, None, 0, 192, 4),
        lead=0, lag=9)
    wait(w1_copy)
    run(project(xf7, sf, wv7, vv, k2), attn_scores(qb, T, None, 192, T, 4), attn_mix(T, ob7, sob, 0, 128, 4),
        ffn_prepare(w1_raw, w17, 0, 4), lead=0)
    run(attn_out(0, oa7, soa), attn_mix(T, ob7, sob, 128, T, 4), ffn_prepare(w1_raw, w17, 4, 6), lead=0)
    run(attn_out(1, ob7, sob), _mix(layernorm(0, xf7, sf), ffn_prepare(w1_raw, w17, 6, 8)), lead=0, lag=2)
    run(ffn_up(0, 6), ffn_prepare(w1_raw, w17, 8, NF // 2), attn_scores(qa, 2 * T, None, 0, T, 8),
        attn_mix(2 * T, oa7, soa, 0, 192, 8), lead=0)
    move_halo(kk, 3 * T, T)
    wait(w2_copy)
    run(ffn_up(6, UP_SPLIT), attn_mix(2 * T, oa7, soa, 192, T, 8), layernorm(3, xa7, sa),
        ffn_prepare(w2_raw, w27, 0, 2, 32), lead=0)
    move_halo(vv, 3 * T, T)
    run(attn_out(2, oa7, soa), ffn_prepare(w2_raw, w27, 2, NC // 2, 32), lead=0, lag=9)

    sched.barrier()
    tuning[:] = 1024, 1

    def step(i, _):
        t_attn = (i + SKEW) % NT
        first = (t_attn == 0).astype(jnp.int32)

        @pl.when(i + SKEW + 1 < NT)
        def _():
            x_copy(i + SKEW + 1).wait()

        move_halo(kk, T, 0)
        move_halo(vv, T, 0)
        solo(ffn_up(UP_SPLIT))
        run(_chain(project(xa7, sa, wq7, qa, 0), project(xa7, sa, wk7, kk, k0)),
            layernorm((i + 1) % NT, xf7, sf), ffn_mid(), lag=2)
        run(project(xa7, sa, wv7, vv, k0), attn_scores(qa, 0, first, 0, 112, 8), lead=0, lag=2)
        for c in range(NC):
            v0 = jnp.broadcast_to(vv[c, HALO:HALO + 1, :], (HALO, 128))
            vv[c, 0:HALO, :] = jnp.where(t_attn == 0, v0, vv[c, 0:HALO, :])
        run(ffn_down(i % NT), attn_scores(qa, 0, first, 112, T, 4), attn_mix(0, oa7, soa, 0, T, 4), lag=2)
        solo(attn_out(t_attn, oa7, soa))
        run(ffn_up(0, UP_SPLIT), layernorm((i + SKEW + 1) % NT, xa7, sa), lead=4)
        sched.barrier()

        @pl.when(i >= NT)
        def _():
            o_copy(i - NT).start()
        return 0

    lax.fori_loop(0, 2 * NT - SKEW, step, 0)

    down_a, down_b = ffn_down(NT - 3), ffn_down(NT - 2, hb7, sob)
    solo(ffn_up(UP_SPLIT), ffn_mid())
    run(_take(down_a, 2), layernorm(NT - 2, xf7, sf), lead=0)
    run(ffn_up(), layernorm(NT - 1, xa7, sa), lead=6)
    run(_chain(_take(down_a, 2), _take(down_b, 1)), ffn_mid(hb7, sob), lead=2)
    solo(ffn_up(a7=xa7, s_ref=sa))
    run(_take(down_b, 3), ffn_mid(), lead=0)
    sched.barrier()
    o_copy(NT - 3).start()
    o_copy(NT - 2).start()
    solo(ffn_down(NT - 1))
    o_copy(NT - 1).start()
    for t in range(NT):
        o_copy(t).wait()


def _scratch_shapes():
    vmem = pltpu.VMEM
    lhs = vmem((7, T // 4, D // 2), u32)
    square = vmem((7, D // 4, D // 2), u32)
    per_row = vmem((T, 128), f32)
    chunks = vmem((NC, T, 128), f32)
    window = vmem((NC, HALO + 3 * T, 128), f32)
    return [
        vmem((S, D), bf16),
        vmem((3, D, D), bf16), vmem((D, D), bf16),
        vmem((D, F), bf16), vmem((F, D), bf16),
        vmem((NC, D // 2, 128), u32),
        vmem((NC, PAD * D // 64, 128), u32),
        square, square, square, square,
        vmem((7, D // 4, F // 2), u32), vmem((7, F // 4, D // 2), u32),
        vmem((40, 128), f32),
        lhs, lhs, lhs, lhs, lhs,
        vmem((7, T // 4, F // 2), u32), vmem((7, T // 4, F // 2), u32),
        per_row, per_row, per_row, per_row, per_row, per_row,
        chunks, per_row, vmem((NF, T, 128), f32), per_row, per_row,
        chunks, chunks, window, window, vmem((W, T, 128), f32),
        vmem((8, 128), u32),
        pltpu.SemaphoreType.DMA((NT,)), pltpu.SemaphoreType.DMA((7,)), pltpu.SemaphoreType.DMA((NT,)),
    ]


@jax.jit
def pallas_interleave_layers__sliding_local_dilated__dense_activation_squared_relu__prompt_kernel(
    A_x: jax.Array,
    A_wqkv: jax.Array,
    A_wo: jax.Array,
    B_x: jax.Array,
    B_w1: jax.Array,
    B_b1: jax.Array,
    B_w2: jax.Array,
    B_b2: jax.Array,
):
    del B_x
    hbm = pl.BlockSpec(memory_space=pl.ANY)
    vmem = pl.BlockSpec(memory_space=pltpu.VMEM)
    out = pl.pallas_call(
        _kernel,
        in_specs=[hbm, hbm, hbm, hbm, vmem, hbm, vmem],
        out_specs=hbm,
        out_shape=jax.ShapeDtypeStruct((S, D), bf16),
        scratch_shapes=_scratch_shapes(),
        compiler_params=pltpu.CompilerParams(vmem_limit_bytes=110 * 2 ** 20),
    )(A_x.reshape(S, D), A_wqkv, A_wo, B_w1, B_b1.reshape(NF, 128), B_w2, B_b2.reshape(NC, 128))
    return out.reshape(1, S, D)
```

```python
import jax
import jax.numpy as jnp
from jax import lax
from jax.experimental import pallas as pl
from jax.experimental.pallas import tpu as pltpu

S, D, F = 2048, 1024, 3584
DH, W, DIL = 32, 8, 2
EPS = 1e-5
SCALE = DH ** -0.5
MASKED = -1e9
LOG2E = 1.4426950408889634
TINY = 1e-36

T = 256
TH = T // 2
NT = S // T
HALO = 16
NC = D // 128
NF = F // 128
SKEW = 3
UP_SPLIT = 13
PAD = DH + 1

f32 = jnp.float32
bf16 = jnp.bfloat16
u32 = jnp.uint32


def _pack_rows(x):
    return pltpu.bitcast(x.astype(bf16), u32)


def _as_bf16(u):
    return pltpu.bitcast(u, bf16)


class _Phase:
    def __init__(self, n, gen):
        self.n, self.gen = n, gen


def _chain(*phases):
    def gen():
        for p in phases:
            yield from p.gen
    return _Phase(sum(p.n for p in phases), gen())


def _take(phase, n):
    return _Phase(n, (next(phase.gen) for _ in range(n)))


def _mix(a, b):
    def gen():
        done = 0
        for i in range(a.n):
            yield next(a.gen)
            while done < (i + 1) * b.n // a.n:
                yield next(b.gen)
                done += 1
    return _Phase(a.n + b.n, gen())


class _Schedule:
    def __init__(self, zero_ref):
        self.zero_ref = zero_ref
        self.results = []
        self.token = None
        self.due = None
        self.carry = {}
        self.lag = 3

    def gate(self, *xs):
        if self.token is None:
            return list(xs)
        zero = pltpu.bitcast(self.token, u32) & self.zero_ref[...]
        out = []
        for x in xs:
            u = pltpu.bitcast(x, u32)
            out.append(pltpu.bitcast(u | jnp.tile(zero, (u.shape[0] // 8, u.shape[1] // 128)), x.dtype))
        return out

    def hold(self, lhs):
        if self.due is None:
            return lhs
        n = min(lhs.shape[1], 512)
        head = [lhs[:8, c:c + 128] | self.due for c in range(0, n, 128)]
        if lhs.shape[1] > n:
            head.append(lhs[:8, n:])
        self.due = None
        return jnp.concatenate([jnp.concatenate(head, axis=1), lhs[8:]], axis=0)

    def run(self, main, *side, lead=1, lag=None):
        lag = self.lag if lag is None else lag
        side = _chain(*side)
        slots = max(main.n - lead, 1)
        dues, done = dict(self.carry), 0
        self.carry = {}
        for i in range(main.n):
            self.results = []
            self.due = dues.pop(i, None)
            next(main.gen)
            tokens = [(y, r) for y in self.results for r in range(0, y.shape[0], 8)]
            want = min(side.n, -(-side.n * (i + 1) // slots))
            finished = None
            for j in range(want - done):
                y, r = tokens[j * len(tokens) // (want - done)]
                self.token = y[r:r + 8]
                last = next(side.gen)
                if last is not None:
                    last = pltpu.bitcast(last, u32)[:8, :128]
                    finished = last if finished is None else finished & last
            if finished is not None:
                dues[i + lag] = finished & self.zero_ref[...]
            done = want
        self.token = self.due = None
        self.carry = {i - main.n: z for i, z in dues.items()}
        for p in (main, side):
            assert next(p.gen, _Schedule) is _Schedule, "wrong piece count"

    def solo(self, *phases):
        self.due = self.carry.pop(0, None)
        self.carry = {}
        for p in phases:
            for _ in p.gen:
                pass
        self.due = None

    def barrier(self):
        self.carry = {}


def _kernel(x_hbm, wqkv_hbm, wo_hbm, w1_hbm, b1_ref, w2_hbm, b2_ref, o_hbm,
            xb, wqkv_raw, wo_raw, w1_raw, w2_raw, w_tmp, wo_tmp,
            wq7, wk7, wv7, wo7, w17, w27, bias,
            xa7, xb7, xf7, oa7, ob7, ha7, hb7, sa, sb, sf, soa, sob, sh,
            stage, stage_inv, h_stage, h_inv, h_ss,
            qa, qb, kk, vv, pp, zero_ref, sem_x, sem_w, sem_o):
    def x_copy(t):
        return pltpu.make_async_copy(x_hbm.at[pl.ds(t * T, T)], xb.at[pl.ds(t * T, T)], sem_x.at[t])

    def o_copy(t):
        return pltpu.make_async_copy(xb.at[pl.ds(t * T, T)], o_hbm.at[pl.ds(t * T, T)], sem_o.at[t])

    def wq_copy(half):
        rows = pl.ds(half * (D // 2), D // 2)
        return pltpu.make_async_copy(wqkv_hbm.at[rows, pl.ds(0, D)], wqkv_raw.at[0, rows], sem_w.at[half])

    def wkv_copy(i):
        return pltpu.make_async_copy(wqkv_hbm.at[:, pl.ds(i * D, D)], wqkv_raw.at[i], sem_w.at[1 + i])

    wo_copy = pltpu.make_async_copy(wo_hbm, wo_raw, sem_w.at[4])
    w1_copy = pltpu.make_async_copy(w1_hbm, w1_raw, sem_w.at[5])
    w2_copy = pltpu.make_async_copy(w2_hbm, w2_raw, sem_w.at[6])

    for copy in (x_copy(0), wq_copy(0), wq_copy(1), x_copy(1), wkv_copy(1), x_copy(2), wkv_copy(2), wo_copy,
                 x_copy(3), w1_copy, w2_copy, *[x_copy(t) for t in range(4, NT)]):
        copy.start()

    bias[0:NF, :] = b1_ref[...].astype(f32)
    bias[32:32 + NC, :] = b2_ref[...].astype(f32)
    zero_ref[...] = jnp.zeros((8, 128), u32)

    sched = _Schedule(zero_ref)
    tuning = [512, 0]
    gate, run, solo = sched.gate, sched.run, sched.solo

    def wait(copy):
        sched.barrier()
        copy.wait()

    def store_b7(dst, row, col, u11, u12, u21, u22):
        b11, b12, b21, b22 = (_as_bf16(u).astype(f32) for u in (u11, u12, u21, u22))
        at = (pl.ds(row, u11.shape[0]), pl.ds(col, u11.shape[1]))
        dst[(0,) + at] = _pack_rows(b11 + b22)
        dst[(1,) + at] = u11
        dst[(2,) + at] = _pack_rows(b12 - b22)
        dst[(3,) + at] = _pack_rows(b21 - b11)
        dst[(4,) + at] = u22
        dst[(5,) + at] = _pack_rows(b11 + b12)
        last = _pack_rows(b21 + b22)
        dst[(6,) + at] = last
        return last

    def a7_pieces(src, inv, dst):
        nk = src.shape[0] // 2
        for r in range(0, TH, 16):
            top, bot = inv[r:r + 16, :], inv[TH + r:TH + r + 16, :]
            for j in range(nk):
                top, bot = gate(top, bot)
                a11, a12, a21, a22 = (src[c, r0:r0 + 16, :] * scale
                                      for r0, scale in ((r, top), (TH + r, bot)) for c in (j, nk + j))
                at = (slice(r // 2, r // 2 + 8), slice(j * 128, (j + 1) * 128))
                dst[(0,) + at] = _pack_rows(a11 + a22)
                dst[(1,) + at] = _pack_rows(a21 + a22)
                dst[(2,) + at] = _pack_rows(a11)
                dst[(3,) + at] = _pack_rows(a22)
                dst[(4,) + at] = _pack_rows(a11 + a12)
                dst[(5,) + at] = _pack_rows(a21 - a11)
                last = _pack_rows(a12 - a22)
                dst[(6,) + at] = last
                yield last

    def matmul(a7, b7, emit, j0=0, j1=None):
        kh, nh = a7.shape[2], b7.shape[2] // 128
        k_step, order = tuning
        j1 = nh if j1 is None else j1

        def product(i, j):
            y = None
            for k in range(0, kh, k_step):
                ke = min(k + k_step, kh)
                yk = lax.dot_general(_as_bf16(sched.hold(a7[i, :, k:ke])),
                                     _as_bf16(b7[i, k // 2:ke // 2, j * 128:(j + 1) * 128]),
                                     (((1,), (0,)), ((), ())), preferred_element_type=f32)
                sched.results.append(yk)
                y = yk if y is None else y + yk
            return y

        def gen():
            for j in range(j0, j1):
                if order == 0:
                    m1, m2 = product(0, j), product(1, j)
                    c22 = m1 - m2
                    m4 = product(3, j)
                    emit(1, j, m2 + m4)
                    c11 = m1 + m4
                    c11 = c11 + product(6, j)
                    m5 = product(4, j)
                    emit(0, j, c11 - m5)
                    m3 = product(2, j)
                    emit(0, nh + j, m3 + m5)
                    c22 = c22 + m3
                    emit(1, nh + j, c22 + product(5, j))
                else:
                    m6, m2 = product(5, j), product(1, j)
                    c22 = m6 - m2
                    m3 = product(2, j)
                    c22 = c22 + m3
                    m1 = product(0, j)
                    emit(1, nh + j, c22 + m1)
                    m5 = product(4, j)
                    emit(0, nh + j, m3 + m5)
                    c11 = m1 - m5
                    m4 = product(3, j)
                    emit(1, j, m2 + m4)
                    c11 = c11 + m4
                    emit(0, j, c11 + product(6, j))
                yield
        return _Phase(j1 - j0, gen())

    def store_row_norm(ss, inv_ref, s_ref, r):
        ss = ss + TINY
        inv = lax.rsqrt(ss)
        shape = (ss.shape[0], 128)
        inv_ref[r:r + shape[0], :] = jnp.broadcast_to(inv, shape)
        norm = jnp.broadcast_to(ss * inv, shape)
        s_ref[r:r + shape[0], :] = norm
        return norm

    def qkv_skew(i, r0=0, r1=D):
        def gen(group=4):
            lane = lax.broadcasted_iota(jnp.int32, (8, 128), 1)
            bits = [(lane & (1 << b)) != 0 for b in range(3)]
            for g0 in range(r0 // 16, r1 // 16, group):
                xs = [[None] * NC for _ in range(group)]
                for c in range(NC):
                    for g in range(group):
                        rows = slice((g0 + g) * 16, (g0 + g + 1) * 16)
                        u, = gate(pltpu.bitcast(wqkv_raw[i, rows, c * 128:(c + 1) * 128], u32))
                        xs[g][c] = pltpu.roll(u, c, 1) if c else u
                for g in range(group):
                    ws = [xs[g][(-c) % NC] for c in range(NC)]
                    for b in range(3):
                        ws = [jnp.where(bits[b], ws[(c - (1 << b)) % NC], ws[c]) for c in range(NC)]
                    for c in range(NC):
                        w_tmp[c, (g0 + g) * 8:(g0 + g + 1) * 8, :] = ws[c]
                yield ws[0]
        return _Phase((r1 - r0) // 64, gen())

    def gather_lanes(c, r0):
        lane = lax.broadcasted_iota(jnp.int32, (64, 128), 1)
        base = (lane & 3) * 32 + (lane >> 5) * 8 + ((lane >> 2) & 7)
        for r in range(r0 // 2, r0 // 2 + D // 4, 64):
            u, = gate(w_tmp[c, r:r + 64, :])
            u = jnp.take_along_axis(u, (base + c) & 127, axis=1)
            w_tmp[c, r:r + 64, :] = u
        return u

    def qkv_finish(dst, j0, j1, top_done=False):
        def gen():
            for j in range(j0, j1):
                left, right = j, NC // 2 + j
                for c in (left, right):
                    if not top_done:
                        gather_lanes(c, 0)
                    yield gather_lanes(c, D // 2)
                for r in range(0, D // 4, 16):
                    top, bot = slice(r, r + 16), slice(D // 4 + r, D // 4 + r + 16)
                    last = store_b7(dst, r, j * 128, w_tmp[left, top, :], w_tmp[right, top, :],
                                    w_tmp[left, bot, :], w_tmp[right, bot, :])
                yield last
        return _Phase(3 * (j1 - j0), gen())

    def wo_stage():
        def gen():
            for n in range(NC):
                u, = gate(pltpu.bitcast(wo_raw[:, n * 128:(n + 1) * 128], u32))
                for g in range(D // 64):
                    wo_tmp[n, pl.ds(PAD * g, 32), :] = u[32 * g:32 * (g + 1)]
                yield u
        return _Phase(NC, gen())

    def wo_finish():
        def rows16(n, cp, a):
            start = PAD * 8 * (a % 2) + 4 * (a // 2) + cp
            lo = wo_tmp[n, pl.ds(start, 8, stride=PAD), :]
            hi = wo_tmp[n, pl.ds(start + 16, 8, stride=PAD), :]
            return (lo & u32(0xFFFF)) | (hi << 16), (lo >> 16) | (hi & u32(0xFFFF0000))

        def gen():
            for j in range(NC // 2):
                for cp in range(NC // 4):
                    for a in range(8):
                        u11, u12 = rows16(j, cp, a), rows16(NC // 2 + j, cp, a)
                        u21, u22 = rows16(j, NC // 4 + cp, a), rows16(NC // 2 + j, NC // 4 + cp, a)
                        u11, u22 = gate(*u11), gate(*u22)
                        for odd in range(2):
                            last = store_b7(wo7, (2 * cp + odd) * 64 + 8 * a, j * 128,
                                            u11[odd], u12[odd], u21[odd], u22[odd])
                        if a % 2:
                            yield last
        return _Phase(NC * NC // 2, gen())

    def ffn_prepare(raw, dst, j0, j1, rows=32):
        kh, nh = raw.shape[0] // 2, raw.shape[1] // 2

        def gen():
            for c in range(j0 * 128, j1 * 128, 256):
                for r in range(0, kh, rows):
                    q = [pltpu.bitcast(raw[r0:r0 + rows, c0:c0 + 256], u32)
                         for r0 in (r, kh + r) for c0 in (c, nh + c)]
                    q[0], q[3] = gate(q[0], q[3])
                    yield store_b7(dst, r // 2, c, *q)
        return _Phase((j1 - j0) // 2 * kh // rows, gen())

    def layernorm(t, a7, s_ref):
        def gen():
            for r in range(0, T, 16):
                rows = pl.ds(pl.multiple_of(t * T + r, 16), 16)
                acc = None
                for c in range(NC):
                    x = xb[rows, c * 128:(c + 1) * 128]
                    if c == 0:
                        x, = gate(x)
                    acc = x.astype(f32) if acc is None else acc + x.astype(f32)
                mean = jnp.broadcast_to(jnp.sum(acc, axis=-1, keepdims=True) * (1.0 / D), (16, 128))
                yield mean
                mean, = gate(mean)
                acc = None
                for c in range(NC):
                    xc = xb[rows, c * 128:(c + 1) * 128].astype(f32) - mean
                    stage[c, r:r + 16, :] = xc
                    acc = xc * xc if acc is None else acc + xc * xc
                var = jnp.sum(acc, axis=-1, keepdims=True) * (1.0 / D)
                inv = lax.rsqrt(var + TINY)
                stage_inv[r:r + 16, :] = jnp.broadcast_to(inv, (16, 128))
                scale = jnp.broadcast_to((var + TINY) * inv * lax.rsqrt(var + EPS), (16, 128))
                s_ref[r:r + 16, :] = scale
                yield scale
            yield from a7_pieces(stage, stage_inv, a7)
        return _Phase(2 * T // 16 + TH // 16 * NC // 2, gen())

    def project(a7, s_ref, b7, dst, row0):
        def emit(half, c, y):
            dst[c, pl.ds(row0 + half * TH, TH), :] = y * s_ref[half * TH:(half + 1) * TH, :]
        return matmul(a7, b7, emit)

    def attn_scores(q, row0, first, r0, r1, chunks):
        def gen():
            for r in range(r0, r1, 8):
                ls = [None] * W
                for c in range(NC):
                    qv, = gate(q[c, r:r + 8, :])
                    for w in range(W):
                        t = qv * kk[c, pl.ds(HALO + row0 + r - DIL * w, 8), :]
                        ls[w] = t if ls[w] is None else ls[w] + t
                    if c % chunks == chunks - 1 and c != NC - 1:
                        yield None
                for w in range(W):
                    t = ls[w] + pltpu.roll(ls[w], 64, 1)
                    t = t + pltpu.roll(t, 32, 1)
                    if first is not None and r < DIL * w:
                        row = lax.broadcasted_iota(jnp.int32, (8, 128), 0) + r
                        t = jnp.where(row < first * (DIL * w), MASKED / SCALE, t)
                    ls[w] = t
                m = ls[0]
                for w in range(1, W):
                    m = jnp.maximum(m, ls[w])
                es = [jnp.exp2((t - m) * (SCALE * LOG2E)) for t in ls]
                total = es[0]
                for w in range(1, W):
                    total = total + es[w]
                inv = 1.0 / total
                for w in range(W):
                    pp[w, r:r + 8, :] = es[w] * inv
                yield inv
        return _Phase((r1 - r0) // 8 * (NC // chunks), gen())

    def attn_mix(row0, o7, s_ref, r0, r1, chunks):
        def gen():
            for r in range(r0, r1, 8):
                ps = [pp[w, r:r + 8, :] for w in range(W)]
                ss = None
                for c in range(NC):
                    if c % chunks == 0:
                        ps = gate(*ps)
                    acc = None
                    for w in range(W):
                        t = ps[w] * vv[c, pl.ds(HALO + row0 + r - DIL * w, 8), :]
                        acc = t if acc is None else acc + t
                    stage[c, r:r + 8, :] = acc
                    ss = acc * acc if ss is None else ss + acc * acc
                    if c % chunks == chunks - 1 and c != NC - 1:
                        yield None
                yield store_row_norm(jnp.sum(ss, axis=-1, keepdims=True), stage_inv, s_ref, r)
            if r1 == T:
                yield from a7_pieces(stage, stage_inv, o7)
        return _Phase((r1 - r0) // 8 * (NC // chunks) + (TH // 16 * NC // 2 if r1 == T else 0), gen())

    def add_residual(t, a7, s_ref, b7, bias_row):
        def emit(half, c, y):
            rows = pl.ds(pl.multiple_of(t * T + half * TH, TH), TH)
            cols = slice(c * 128, (c + 1) * 128)
            z = y * s_ref[half * TH:(half + 1) * TH, :]
            if bias_row is not None:
                z = z + bias[bias_row + c:bias_row + c + 1, :]
            xb[rows, cols] = (xb[rows, cols].astype(f32) + z).astype(bf16)
        return matmul(a7, b7, emit)

    def attn_out(t, o7, s_ref):
        return add_residual(t, o7, s_ref, wo7, None)

    def ffn_up(j0=0, j1=NF // 2, a7=xf7, s_ref=sf):
        started = [j0 > 0, j0 > 0]

        def emit(half, c, y):
            rows = slice(half * TH, (half + 1) * TH)
            z = jnp.maximum(y * s_ref[rows, :] + bias[c:c + 1, :], 0.0)
            z = z * z
            h_stage[c, rows, :] = z
            h_ss[rows, :] = h_ss[rows, :] + z * z if started[half] else z * z
            started[half] = True
        return matmul(a7, w17, emit, j0, j1)

    def ffn_mid(h7=ha7, s_ref=sh):
        def gen():
            for r in range(0, T, 32):
                ss, = gate(h_ss[r:r + 32, :])
                yield store_row_norm(jnp.sum(ss, axis=-1, keepdims=True), h_inv, s_ref, r)
            yield from a7_pieces(h_stage, h_inv, h7)
        return _Phase(T // 32 + TH // 16 * NF // 2, gen())

    def ffn_down(t, h7=ha7, s_ref=sh):
        return add_residual(t, h7, s_ref, w27, 32)

    def move_halo(ref, src, dst):
        for c in range(NC):
            ref[c, pl.ds(dst, HALO), :] = ref[c, pl.ds(src, HALO), :]

    k0, k1, k2 = HALO, HALO + T, HALO + 2 * T
    wait(x_copy(0))
    solo(layernorm(0, xa7, sa))
    wait(wq_copy(0))
    solo(qkv_skew(0, 0, D // 2))
    for c in range(NC):
        gather_lanes(c, 0)
    wait(wq_copy(1))
    solo(qkv_skew(0, D // 2, D), qkv_finish(wq7, 0, 3, True))
    wait(x_copy(1))
    run(project(xa7, sa, wq7, qa, 0), qkv_finish(wq7, 3, 4, True), layernorm(1, xb7, sb))
    wait(wkv_copy(1))
    run(project(xb7, sb, wq7, qb, 0), qkv_skew(1), qkv_finish(wk7, 0, 3), lag=9)
    run(project(xa7, sa, wk7, kk, k0), qkv_finish(wk7, 3, 4), lead=2, lag=1)
    for c in range(NC):
        kk[c, 0:HALO, :] = jnp.zeros((HALO, 128), f32)
    wait(x_copy(2))
    run(project(xb7, sb, wk7, kk, k1), layernorm(2, xf7, sf), attn_scores(qa, 0, 1, 0, 160, 4), lead=0, lag=9)
    wait(wkv_copy(2))
    run(project(xf7, sf, wk7, kk, k2), qkv_skew(2), qkv_finish(wv7, 0, 2))
    wait(wo_copy)
    run(project(xa7, sa, wv7, vv, k0), qkv_finish(wv7, 2, 4), attn_scores(qa, 0, 1, 160, T, 4), wo_stage(), lead=0)
    for c in range(NC):
        vv[c, 0:HALO, :] = jnp.broadcast_to(vv[c, HALO:HALO + 1, :], (HALO, 128))
    wait(x_copy(3))
    run(project(xb7, sb, wv7, vv, k1), wo_finish(), attn_mix(0, oa7, soa, 0, 160, 4), lead=0, lag=9)
    run(project(xf7, sf, wq7, qa, 0), attn_mix(0, oa7, soa, 160, T, 4), attn_scores(qb, T, None, 0, 192, 4),
        lead=0, lag=9)
    wait(w1_copy)
    run(project(xf7, sf, wv7, vv, k2), attn_scores(qb, T, None, 192, T, 4), attn_mix(T, ob7, sob, 0, 128, 4),
        ffn_prepare(w1_raw, w17, 0, 4), lead=0)
    run(attn_out(0, oa7, soa), attn_mix(T, ob7, sob, 128, T, 4), ffn_prepare(w1_raw, w17, 4, 6), lead=0)
    run(attn_out(1, ob7, sob), _mix(layernorm(0, xf7, sf), ffn_prepare(w1_raw, w17, 6, 8)), lead=0, lag=2)
    run(ffn_up(0, 6), ffn_prepare(w1_raw, w17, 8, NF // 2), attn_scores(qa, 2 * T, None, 0, T, 8),
        attn_mix(2 * T, oa7, soa, 0, 192, 8), lead=0)
    move_halo(kk, 3 * T, T)
    wait(w2_copy)
    run(ffn_up(6, UP_SPLIT), attn_mix(2 * T, oa7, soa, 192, T, 8), layernorm(3, xa7, sa),
        ffn_prepare(w2_raw, w27, 0, 2, 16), lead=0)
    move_halo(vv, 3 * T, T)
    run(attn_out(2, oa7, soa), ffn_prepare(w2_raw, w27, 2, NC // 2, 16), lead=0, lag=9)

    sched.barrier()
    tuning[:] = 1024, 1

    def step(i, _):
        t_attn = (i + SKEW) % NT
        first = (t_attn == 0).astype(jnp.int32)

        @pl.when(i + SKEW + 1 < NT)
        def _():
            x_copy(i + SKEW + 1).wait()

        move_halo(kk, T, 0)
        move_halo(vv, T, 0)
        solo(ffn_up(UP_SPLIT))
        run(_chain(project(xa7, sa, wq7, qa, 0), project(xa7, sa, wk7, kk, k0)),
            layernorm((i + 1) % NT, xf7, sf), ffn_mid(), lag=2)
        run(project(xa7, sa, wv7, vv, k0), attn_scores(qa, 0, first, 0, 112, 8), lead=0, lag=2)
        for c in range(NC):
            v0 = jnp.broadcast_to(vv[c, HALO:HALO + 1, :], (HALO, 128))
            vv[c, 0:HALO, :] = jnp.where(t_attn == 0, v0, vv[c, 0:HALO, :])
        run(ffn_down(i % NT), attn_scores(qa, 0, first, 112, T, 4), attn_mix(0, oa7, soa, 0, T, 4), lag=2)
        solo(attn_out(t_attn, oa7, soa))
        run(ffn_up(0, UP_SPLIT), layernorm((i + SKEW + 1) % NT, xa7, sa), lead=4)
        sched.barrier()

        @pl.when(i >= NT)
        def _():
            o_copy(i - NT).start()
        return 0

    lax.fori_loop(0, 2 * NT - SKEW, step, 0)

    down_a, down_b = ffn_down(NT - 3), ffn_down(NT - 2, hb7, sob)
    solo(ffn_up(UP_SPLIT), ffn_mid())
    run(_take(down_a, 2), layernorm(NT - 2, xf7, sf), lead=0)
    run(ffn_up(), layernorm(NT - 1, xa7, sa), lead=6)
    run(_chain(_take(down_a, 2), _take(down_b, 1)), ffn_mid(hb7, sob), lead=2)
    solo(ffn_up(a7=xa7, s_ref=sa))
    run(_take(down_b, 3), ffn_mid(), lead=0)
    sched.barrier()
    o_copy(NT - 3).start()
    o_copy(NT - 2).start()
    solo(ffn_down(NT - 1))
    o_copy(NT - 1).start()
    for t in range(NT):
        o_copy(t).wait()


def _scratch_shapes():
    vmem = pltpu.VMEM
    lhs = vmem((7, T // 4, D // 2), u32)
    square = vmem((7, D // 4, D // 2), u32)
    per_row = vmem((T, 128), f32)
    chunks = vmem((NC, T, 128), f32)
    window = vmem((NC, HALO + 3 * T, 128), f32)
    return [
        vmem((S, D), bf16),
        vmem((3, D, D), bf16), vmem((D, D), bf16),
        vmem((D, F), bf16), vmem((F, D), bf16),
        vmem((NC, D // 2, 128), u32),
        vmem((NC, PAD * D // 64, 128), u32),
        square, square, square, square,
        vmem((7, D // 4, F // 2), u32), vmem((7, F // 4, D // 2), u32),
        vmem((40, 128), f32),
        lhs, lhs, lhs, lhs, lhs,
        vmem((7, T // 4, F // 2), u32), vmem((7, T // 4, F // 2), u32),
        per_row, per_row, per_row, per_row, per_row, per_row,
        chunks, per_row, vmem((NF, T, 128), f32), per_row, per_row,
        chunks, chunks, window, window, vmem((W, T, 128), f32),
        vmem((8, 128), u32),
        pltpu.SemaphoreType.DMA((NT,)), pltpu.SemaphoreType.DMA((7,)), pltpu.SemaphoreType.DMA((NT,)),
    ]


@jax.jit
def pallas_interleave_layers__sliding_local_dilated__dense_activation_squared_relu__prompt_kernel(
    A_x: jax.Array,
    A_wqkv: jax.Array,
    A_wo: jax.Array,
    B_x: jax.Array,
    B_w1: jax.Array,
    B_b1: jax.Array,
    B_w2: jax.Array,
    B_b2: jax.Array,
):
    del B_x
    hbm = pl.BlockSpec(memory_space=pl.ANY)
    vmem = pl.BlockSpec(memory_space=pltpu.VMEM)
    out = pl.pallas_call(
        _kernel,
        in_specs=[hbm, hbm, hbm, hbm, vmem, hbm, vmem],
        out_specs=hbm,
        out_shape=jax.ShapeDtypeStruct((S, D), bf16),
        scratch_shapes=_scratch_shapes(),
        compiler_params=pltpu.CompilerParams(vmem_limit_bytes=110 * 2 ** 20),
    )(A_x.reshape(S, D), A_wqkv, A_wo, B_w1, B_b1.reshape(NF, 128), B_w2, B_b2.reshape(NC, 128))
    return out.reshape(1, S, D)
```

```python
import jax
import jax.numpy as jnp
from jax import lax
from jax.experimental import pallas as pl
from jax.experimental.pallas import tpu as pltpu

S, D, F = 2048, 1024, 3584
DH, W, DIL = 32, 8, 2
EPS = 1e-5
SCALE = DH ** -0.5
MASKED = -1e9
LOG2E = 1.4426950408889634
TINY = 1e-36

T = 256
TH = T // 2
NT = S // T
HALO = 16
NC = D // 128
NF = F // 128
SKEW = 3
UP_SPLIT = 13
PAD = DH + 1

f32 = jnp.float32
bf16 = jnp.bfloat16
u32 = jnp.uint32


def _pack_rows(x):
    return pltpu.bitcast(x.astype(bf16), u32)


def _as_bf16(u):
    return pltpu.bitcast(u, bf16)


class _Phase:
    def __init__(self, n, gen):
        self.n, self.gen = n, gen


def _chain(*phases):
    def gen():
        for p in phases:
            yield from p.gen
    return _Phase(sum(p.n for p in phases), gen())


def _take(phase, n):
    return _Phase(n, (next(phase.gen) for _ in range(n)))


def _mix(a, b):
    def gen():
        done = 0
        for i in range(a.n):
            yield next(a.gen)
            while done < (i + 1) * b.n // a.n:
                yield next(b.gen)
                done += 1
    return _Phase(a.n + b.n, gen())


class _Schedule:
    def __init__(self, zero_ref):
        self.zero_ref = zero_ref
        self.results = []
        self.token = None
        self.due = None
        self.carry = {}
        self.lag = 3

    def gate(self, *xs):
        if self.token is None:
            return list(xs)
        zero = pltpu.bitcast(self.token, u32) & self.zero_ref[...]
        out = []
        for x in xs:
            u = pltpu.bitcast(x, u32)
            out.append(pltpu.bitcast(u | jnp.tile(zero, (u.shape[0] // 8, u.shape[1] // 128)), x.dtype))
        return out

    def hold(self, lhs):
        if self.due is None:
            return lhs
        n = min(lhs.shape[1], 512)
        head = [lhs[:8, c:c + 128] | self.due for c in range(0, n, 128)]
        if lhs.shape[1] > n:
            head.append(lhs[:8, n:])
        self.due = None
        return jnp.concatenate([jnp.concatenate(head, axis=1), lhs[8:]], axis=0)

    def run(self, main, *side, lead=1, lag=None):
        lag = self.lag if lag is None else lag
        side = _chain(*side)
        slots = max(main.n - lead, 1)
        dues, done = dict(self.carry), 0
        self.carry = {}
        for i in range(main.n):
            self.results = []
            self.due = dues.pop(i, None)
            next(main.gen)
            tokens = [(y, r) for y in self.results for r in range(0, y.shape[0], 8)]
            want = min(side.n, -(-side.n * (i + 1) // slots))
            finished = None
            for j in range(want - done):
                y, r = tokens[j * len(tokens) // (want - done)]
                self.token = y[r:r + 8]
                last = next(side.gen)
                if last is not None:
                    last = pltpu.bitcast(last, u32)[:8, :128]
                    finished = last if finished is None else finished & last
            if finished is not None:
                dues[i + lag] = finished & self.zero_ref[...]
            done = want
        self.token = self.due = None
        self.carry = {i - main.n: z for i, z in dues.items()}
        for p in (main, side):
            assert next(p.gen, _Schedule) is _Schedule, "wrong piece count"

    def solo(self, *phases):
        self.due = self.carry.pop(0, None)
        self.carry = {}
        for p in phases:
            for _ in p.gen:
                pass
        self.due = None

    def barrier(self):
        self.carry = {}


def _kernel(x_hbm, wqkv_hbm, wo_hbm, w1_hbm, b1_ref, w2_hbm, b2_ref, o_hbm,
            xb, wqkv_raw, wo_raw, w1_raw, w2_raw, w_tmp, wo_tmp,
            wq7, wk7, wv7, wo7, w17, w27, bias,
            xa7, xb7, xf7, oa7, ob7, ha7, hb7, sa, sb, sf, soa, sob, sh,
            stage, stage_inv, h_stage, h_inv, h_ss,
            qa, qb, kk, vv, pp, zero_ref, sem_x, sem_w, sem_o):
    def x_copy(t):
        return pltpu.make_async_copy(x_hbm.at[pl.ds(t * T, T)], xb.at[pl.ds(t * T, T)], sem_x.at[t])

    def o_copy(t):
        return pltpu.make_async_copy(xb.at[pl.ds(t * T, T)], o_hbm.at[pl.ds(t * T, T)], sem_o.at[t])

    def wq_copy(half):
        rows = pl.ds(half * (D // 2), D // 2)
        return pltpu.make_async_copy(wqkv_hbm.at[rows, pl.ds(0, D)], wqkv_raw.at[0, rows], sem_w.at[half])

    def wkv_copy(i):
        return pltpu.make_async_copy(wqkv_hbm.at[:, pl.ds(i * D, D)], wqkv_raw.at[i], sem_w.at[1 + i])

    wo_copy = pltpu.make_async_copy(wo_hbm, wo_raw, sem_w.at[4])
    w1_copy = pltpu.make_async_copy(w1_hbm, w1_raw, sem_w.at[5])
    w2_copy = pltpu.make_async_copy(w2_hbm, w2_raw, sem_w.at[6])

    for copy in (x_copy(0), wq_copy(0), wq_copy(1), x_copy(1), wkv_copy(1), x_copy(2), wkv_copy(2), wo_copy,
                 x_copy(3), w1_copy, w2_copy, *[x_copy(t) for t in range(4, NT)]):
        copy.start()

    bias[0:NF, :] = b1_ref[...].astype(f32)
    bias[32:32 + NC, :] = b2_ref[...].astype(f32)
    zero_ref[...] = jnp.zeros((8, 128), u32)

    sched = _Schedule(zero_ref)
    tuning = [512, 0]
    gate, run, solo = sched.gate, sched.run, sched.solo

    def wait(copy):
        sched.barrier()
        copy.wait()

    def store_b7(dst, row, col, u11, u12, u21, u22):
        b11, b12, b21, b22 = ((_as_bf16(u) if u.dtype == u32 else u).astype(f32) for u in (u11, u12, u21, u22))
        at = (pl.ds(row, u11.shape[0]), pl.ds(col, u11.shape[1]))
        dst[(0,) + at] = _pack_rows(b11 + b22)
        dst[(1,) + at] = u11
        dst[(2,) + at] = _pack_rows(b12 - b22)
        dst[(3,) + at] = _pack_rows(b21 - b11)
        dst[(4,) + at] = u22
        dst[(5,) + at] = _pack_rows(b11 + b12)
        last = _pack_rows(b21 + b22)
        dst[(6,) + at] = last
        return last

    def a7_pieces(src, inv, dst):
        nk = src.shape[0] // 2
        for r in range(0, TH, 16):
            top, bot = inv[r:r + 16, :], inv[TH + r:TH + r + 16, :]
            for j in range(nk):
                top, bot = gate(top, bot)
                a11, a12, a21, a22 = (src[c, r0:r0 + 16, :] * scale
                                      for r0, scale in ((r, top), (TH + r, bot)) for c in (j, nk + j))
                at = (slice(r // 2, r // 2 + 8), slice(j * 128, (j + 1) * 128))
                dst[(0,) + at] = _pack_rows(a11 + a22)
                dst[(1,) + at] = _pack_rows(a21 + a22)
                dst[(2,) + at] = _pack_rows(a11)
                dst[(3,) + at] = _pack_rows(a22)
                dst[(4,) + at] = _pack_rows(a11 + a12)
                dst[(5,) + at] = _pack_rows(a21 - a11)
                last = _pack_rows(a12 - a22)
                dst[(6,) + at] = last
                yield last

    def matmul(a7, b7, emit, j0=0, j1=None):
        kh, nh = a7.shape[2], b7.shape[2] // 128
        k_step, order = tuning
        j1 = nh if j1 is None else j1

        def product(i, j):
            y = None
            for k in range(0, kh, k_step):
                ke = min(k + k_step, kh)
                yk = lax.dot_general(_as_bf16(sched.hold(a7[i, :, k:ke])),
                                     _as_bf16(b7[i, k // 2:ke // 2, j * 128:(j + 1) * 128]),
                                     (((1,), (0,)), ((), ())), preferred_element_type=f32)
                sched.results.append(yk)
                y = yk if y is None else y + yk
            return y

        def gen():
            for j in range(j0, j1):
                if order == 0:
                    m1, m2 = product(0, j), product(1, j)
                    c22 = m1 - m2
                    m4 = product(3, j)
                    emit(1, j, m2 + m4)
                    c11 = m1 + m4
                    c11 = c11 + product(6, j)
                    m5 = product(4, j)
                    emit(0, j, c11 - m5)
                    m3 = product(2, j)
                    emit(0, nh + j, m3 + m5)
                    c22 = c22 + m3
                    emit(1, nh + j, c22 + product(5, j))
                else:
                    m6, m2 = product(5, j), product(1, j)
                    c22 = m6 - m2
                    m3 = product(2, j)
                    c22 = c22 + m3
                    m1 = product(0, j)
                    emit(1, nh + j, c22 + m1)
                    m5 = product(4, j)
                    emit(0, nh + j, m3 + m5)
                    c11 = m1 - m5
                    m4 = product(3, j)
                    emit(1, j, m2 + m4)
                    c11 = c11 + m4
                    emit(0, j, c11 + product(6, j))
                yield
        return _Phase(j1 - j0, gen())

    def store_row_norm(ss, inv_ref, s_ref, r):
        ss = ss + TINY
        inv = lax.rsqrt(ss)
        shape = (ss.shape[0], 128)
        inv_ref[r:r + shape[0], :] = jnp.broadcast_to(inv, shape)
        norm = jnp.broadcast_to(ss * inv, shape)
        s_ref[r:r + shape[0], :] = norm
        return norm

    def qkv_skew(i, r0=0, r1=D):
        def gen(group=4):
            lane = lax.broadcasted_iota(jnp.int32, (8, 128), 1)
            bits = [(lane & (1 << b)) != 0 for b in range(3)]
            for g0 in range(r0 // 16, r1 // 16, group):
                xs = [[None] * NC for _ in range(group)]
                for c in range(NC):
                    for g in range(group):
                        rows = slice((g0 + g) * 16, (g0 + g + 1) * 16)
                        u, = gate(pltpu.bitcast(wqkv_raw[i, rows, c * 128:(c + 1) * 128], u32))
                        xs[g][c] = pltpu.roll(u, c, 1) if c else u
                for g in range(group):
                    ws = [xs[g][(-c) % NC] for c in range(NC)]
                    for b in range(3):
                        ws = [jnp.where(bits[b], ws[(c - (1 << b)) % NC], ws[c]) for c in range(NC)]
                    for c in range(NC):
                        w_tmp[c, (g0 + g) * 8:(g0 + g + 1) * 8, :] = ws[c]
                yield ws[0]
        return _Phase((r1 - r0) // 64, gen())

    def gather_lanes(c, r0):
        lane = lax.broadcasted_iota(jnp.int32, (64, 128), 1)
        base = (lane & 3) * 32 + (lane >> 5) * 8 + ((lane >> 2) & 7)
        for r in range(r0 // 2, r0 // 2 + D // 4, 64):
            u, = gate(w_tmp[c, r:r + 64, :])
            u = jnp.take_along_axis(u, (base + c) & 127, axis=1)
            w_tmp[c, r:r + 64, :] = u
        return u

    def qkv_finish(dst, j0, j1, top_done=False):
        def gen():
            for j in range(j0, j1):
                left, right = j, NC // 2 + j
                for c in (left, right):
                    if not top_done:
                        gather_lanes(c, 0)
                    yield gather_lanes(c, D // 2)
                for r in range(0, D // 4, 16):
                    top, bot = slice(r, r + 16), slice(D // 4 + r, D // 4 + r + 16)
                    last = store_b7(dst, r, j * 128, w_tmp[left, top, :], w_tmp[right, top, :],
                                    w_tmp[left, bot, :], w_tmp[right, bot, :])
                yield last
        return _Phase(3 * (j1 - j0), gen())

    def wo_stage():
        def gen():
            for n in range(NC):
                u, = gate(pltpu.bitcast(wo_raw[:, n * 128:(n + 1) * 128], u32))
                for g in range(D // 64):
                    wo_tmp[n, pl.ds(PAD * g, 32), :] = u[32 * g:32 * (g + 1)]
                yield u
        return _Phase(NC, gen())

    def wo_finish():
        def rows16(n, cp, a):
            start = PAD * 8 * (a % 2) + 4 * (a // 2) + cp
            lo = wo_tmp[n, pl.ds(start, 8, stride=PAD), :]
            hi = wo_tmp[n, pl.ds(start + 16, 8, stride=PAD), :]
            return (lo & u32(0xFFFF)) | (hi << 16), (lo >> 16) | (hi & u32(0xFFFF0000))

        def gen():
            for j in range(NC // 2):
                for cp in range(NC // 4):
                    for a in range(8):
                        u11, u12 = rows16(j, cp, a), rows16(NC // 2 + j, cp, a)
                        u21, u22 = rows16(j, NC // 4 + cp, a), rows16(NC // 2 + j, NC // 4 + cp, a)
                        u11, u22 = gate(*u11), gate(*u22)
                        for odd in range(2):
                            last = store_b7(wo7, (2 * cp + odd) * 64 + 8 * a, j * 128,
                                            u11[odd], u12[odd], u21[odd], u22[odd])
                        if a % 2:
                            yield last
        return _Phase(NC * NC // 2, gen())

    def ffn_prepare(raw, dst, j0, j1, rows=32):
        kh, nh = raw.shape[0] // 2, raw.shape[1] // 2

        def gen():
            for c in range(j0 * 128, j1 * 128, 256):
                for r in range(0, kh, rows):
                    q = [raw[r0:r0 + rows, c0:c0 + 256] for r0 in (r, kh + r) for c0 in (c, nh + c)]
                    q[0], q[3] = gate(pltpu.bitcast(q[0], u32), pltpu.bitcast(q[3], u32))
                    yield store_b7(dst, r // 2, c, *q)
        return _Phase((j1 - j0) // 2 * kh // rows, gen())

    def layernorm(t, a7, s_ref):
        def gen():
            for r in range(0, T, 16):
                rows = pl.ds(pl.multiple_of(t * T + r, 16), 16)
                acc = None
                for c in range(NC):
                    x = xb[rows, c * 128:(c + 1) * 128]
                    if c == 0:
                        x, = gate(x)
                    acc = x.astype(f32) if acc is None else acc + x.astype(f32)
                mean = jnp.broadcast_to(jnp.sum(acc, axis=-1, keepdims=True) * (1.0 / D), (16, 128))
                yield mean
                mean, = gate(mean)
                acc = None
                for c in range(NC):
                    xc = xb[rows, c * 128:(c + 1) * 128].astype(f32) - mean
                    stage[c, r:r + 16, :] = xc
                    acc = xc * xc if acc is None else acc + xc * xc
                var = jnp.sum(acc, axis=-1, keepdims=True) * (1.0 / D)
                inv = lax.rsqrt(var + TINY)
                stage_inv[r:r + 16, :] = jnp.broadcast_to(inv, (16, 128))
                scale = jnp.broadcast_to((var + TINY) * inv * lax.rsqrt(var + EPS), (16, 128))
                s_ref[r:r + 16, :] = scale
                yield scale
            yield from a7_pieces(stage, stage_inv, a7)
        return _Phase(2 * T // 16 + TH // 16 * NC // 2, gen())

    def project(a7, s_ref, b7, dst, row0):
        def emit(half, c, y):
            dst[c, pl.ds(row0 + half * TH, TH), :] = y * s_ref[half * TH:(half + 1) * TH, :]
        return matmul(a7, b7, emit)

    def attn_scores(q, row0, first, r0, r1, chunks):
        def gen():
            for r in range(r0, r1, 8):
                ls = [None] * W
                for c in range(NC):
                    qv, = gate(q[c, r:r + 8, :])
                    for w in range(W):
                        t = qv * kk[c, pl.ds(HALO + row0 + r - DIL * w, 8), :]
                        ls[w] = t if ls[w] is None else ls[w] + t
                    if c % chunks == chunks - 1 and c != NC - 1:
                        yield None
                for w in range(W):
                    t = ls[w] + pltpu.roll(ls[w], 64, 1)
                    t = t + pltpu.roll(t, 32, 1)
                    if first is not None and r < DIL * w:
                        row = lax.broadcasted_iota(jnp.int32, (8, 128), 0) + r
                        t = jnp.where(row < first * (DIL * w), MASKED / SCALE, t)
                    ls[w] = t
                m = ls[0]
                for w in range(1, W):
                    m = jnp.maximum(m, ls[w])
                es = [jnp.exp2((t - m) * (SCALE * LOG2E)) for t in ls]
                total = es[0]
                for w in range(1, W):
                    total = total + es[w]
                inv = 1.0 / total
                for w in range(W):
                    pp[w, r:r + 8, :] = es[w] * inv
                yield inv
        return _Phase((r1 - r0) // 8 * (NC // chunks), gen())

    def attn_mix(row0, o7, s_ref, r0, r1, chunks):
        def gen():
            for r in range(r0, r1, 8):
                ps = [pp[w, r:r + 8, :] for w in range(W)]
                ss = None
                for c in range(NC):
                    if c % chunks == 0:
                        ps = gate(*ps)
                    acc = None
                    for w in range(W):
                        t = ps[w] * vv[c, pl.ds(HALO + row0 + r - DIL * w, 8), :]
                        acc = t if acc is None else acc + t
                    stage[c, r:r + 8, :] = acc
                    ss = acc * acc if ss is None else ss + acc * acc
                    if c % chunks == chunks - 1 and c != NC - 1:
                        yield None
                yield store_row_norm(jnp.sum(ss, axis=-1, keepdims=True), stage_inv, s_ref, r)
            if r1 == T:
                yield from a7_pieces(stage, stage_inv, o7)
        return _Phase((r1 - r0) // 8 * (NC // chunks) + (TH // 16 * NC // 2 if r1 == T else 0), gen())

    def add_residual(t, a7, s_ref, b7, bias_row):
        def emit(half, c, y):
            rows = pl.ds(pl.multiple_of(t * T + half * TH, TH), TH)
            cols = slice(c * 128, (c + 1) * 128)
            z = y * s_ref[half * TH:(half + 1) * TH, :]
            if bias_row is not None:
                z = z + bias[bias_row + c:bias_row + c + 1, :]
            xb[rows, cols] = (xb[rows, cols].astype(f32) + z).astype(bf16)
        return matmul(a7, b7, emit)

    def attn_out(t, o7, s_ref):
        return add_residual(t, o7, s_ref, wo7, None)

    def ffn_up(j0=0, j1=NF // 2, a7=xf7, s_ref=sf):
        started = [j0 > 0, j0 > 0]

        def emit(half, c, y):
            rows = slice(half * TH, (half + 1) * TH)
            z = jnp.maximum(y * s_ref[rows, :] + bias[c:c + 1, :], 0.0)
            z = z * z
            h_stage[c, rows, :] = z
            h_ss[rows, :] = h_ss[rows, :] + z * z if started[half] else z * z
            started[half] = True
        return matmul(a7, w17, emit, j0, j1)

    def ffn_mid(h7=ha7, s_ref=sh):
        def gen():
            for r in range(0, T, 32):
                ss, = gate(h_ss[r:r + 32, :])
                yield store_row_norm(jnp.sum(ss, axis=-1, keepdims=True), h_inv, s_ref, r)
            yield from a7_pieces(h_stage, h_inv, h7)
        return _Phase(T // 32 + TH // 16 * NF // 2, gen())

    def ffn_down(t, h7=ha7, s_ref=sh):
        return add_residual(t, h7, s_ref, w27, 32)

    def move_halo(ref, src, dst):
        for c in range(NC):
            ref[c, pl.ds(dst, HALO), :] = ref[c, pl.ds(src, HALO), :]

    k0, k1, k2 = HALO, HALO + T, HALO + 2 * T
    wait(x_copy(0))
    solo(layernorm(0, xa7, sa))
    wait(wq_copy(0))
    solo(qkv_skew(0, 0, D // 2))
    for c in range(NC):
        gather_lanes(c, 0)
    wait(wq_copy(1))
    solo(qkv_skew(0, D // 2, D), qkv_finish(wq7, 0, 3, True))
    wait(x_copy(1))
    run(project(xa7, sa, wq7, qa, 0), qkv_finish(wq7, 3, 4, True), layernorm(1, xb7, sb))
    wait(wkv_copy(1))
    run(project(xb7, sb, wq7, qb, 0), qkv_skew(1), qkv_finish(wk7, 0, 3), lag=9)
    run(project(xa7, sa, wk7, kk, k0), qkv_finish(wk7, 3, 4), lead=2, lag=1)
    for c in range(NC):
        kk[c, 0:HALO, :] = jnp.zeros((HALO, 128), f32)
    wait(x_copy(2))
    run(project(xb7, sb, wk7, kk, k1), layernorm(2, xf7, sf), attn_scores(qa, 0, 1, 0, 160, 4), lead=0, lag=9)
    wait(wkv_copy(2))
    run(project(xf7, sf, wk7, kk, k2), qkv_skew(2), qkv_finish(wv7, 0, 2))
    wait(wo_copy)
    run(project(xa7, sa, wv7, vv, k0), qkv_finish(wv7, 2, 4), attn_scores(qa, 0, 1, 160, T, 4), wo_stage(), lead=0)
    for c in range(NC):
        vv[c, 0:HALO, :] = jnp.broadcast_to(vv[c, HALO:HALO + 1, :], (HALO, 128))
    wait(x_copy(3))
    run(project(xb7, sb, wv7, vv, k1), wo_finish(), attn_mix(0, oa7, soa, 0, 160, 4), lead=0, lag=9)
    run(project(xf7, sf, wq7, qa, 0), attn_mix(0, oa7, soa, 160, T, 4), attn_scores(qb, T, None, 0, 192, 4),
        lead=0, lag=9)
    wait(w1_copy)
    run(project(xf7, sf, wv7, vv, k2), attn_scores(qb, T, None, 192, T, 4), attn_mix(T, ob7, sob, 0, 128, 4),
        ffn_prepare(w1_raw, w17, 0, 4), lead=0)
    run(attn_out(0, oa7, soa), attn_mix(T, ob7, sob, 128, T, 4), ffn_prepare(w1_raw, w17, 4, 6), lead=0)
    run(attn_out(1, ob7, sob), _mix(layernorm(0, xf7, sf), ffn_prepare(w1_raw, w17, 6, 8)), lead=0, lag=2)
    run(ffn_up(0, 6), ffn_prepare(w1_raw, w17, 8, NF // 2), attn_scores(qa, 2 * T, None, 0, T, 8),
        attn_mix(2 * T, oa7, soa, 0, 192, 8), lead=0)
    move_halo(kk, 3 * T, T)
    wait(w2_copy)
    run(ffn_up(6, UP_SPLIT), attn_mix(2 * T, oa7, soa, 192, T, 8), layernorm(3, xa7, sa),
        ffn_prepare(w2_raw, w27, 0, 2, 16), lead=0)
    move_halo(vv, 3 * T, T)
    run(attn_out(2, oa7, soa), ffn_prepare(w2_raw, w27, 2, NC // 2, 16), lead=0, lag=9)

    sched.barrier()
    tuning[:] = 1024, 1

    def step(i, _):
        t_attn = (i + SKEW) % NT
        first = (t_attn == 0).astype(jnp.int32)

        @pl.when(i + SKEW + 1 < NT)
        def _():
            x_copy(i + SKEW + 1).wait()

        move_halo(kk, T, 0)
        move_halo(vv, T, 0)
        solo(ffn_up(UP_SPLIT))
        run(_chain(project(xa7, sa, wq7, qa, 0), project(xa7, sa, wk7, kk, k0)),
            layernorm((i + 1) % NT, xf7, sf), ffn_mid(), lag=2)
        run(project(xa7, sa, wv7, vv, k0), attn_scores(qa, 0, first, 0, 112, 8), lead=0, lag=2)
        for c in range(NC):
            v0 = jnp.broadcast_to(vv[c, HALO:HALO + 1, :], (HALO, 128))
            vv[c, 0:HALO, :] = jnp.where(t_attn == 0, v0, vv[c, 0:HALO, :])
        run(ffn_down(i % NT), attn_scores(qa, 0, first, 112, T, 4), attn_mix(0, oa7, soa, 0, T, 4), lag=2)
        solo(attn_out(t_attn, oa7, soa))
        run(ffn_up(0, UP_SPLIT), layernorm((i + SKEW + 1) % NT, xa7, sa), lead=4)
        sched.barrier()

        @pl.when(i >= NT)
        def _():
            o_copy(i - NT).start()
        return 0

    lax.fori_loop(0, 2 * NT - SKEW, step, 0)

    down_a, down_b = ffn_down(NT - 3), ffn_down(NT - 2, hb7, sob)
    solo(ffn_up(UP_SPLIT), ffn_mid())
    run(_take(down_a, 2), layernorm(NT - 2, xf7, sf), lead=0)
    run(ffn_up(), layernorm(NT - 1, xa7, sa), lead=6)
    run(_chain(_take(down_a, 2), _take(down_b, 1)), ffn_mid(hb7, sob), lead=2)
    solo(ffn_up(a7=xa7, s_ref=sa))
    run(_take(down_b, 3), ffn_mid(), lead=0)
    sched.barrier()
    o_copy(NT - 3).start()
    o_copy(NT - 2).start()
    down_c = ffn_down(NT - 1)
    last = []
    for j in range(NC // 2):
        solo(_take(down_c, 1))
        for c in (j, NC // 2 + j):
            at = (pl.ds((NT - 1) * T, T), pl.ds(c * 128, 128))
            last.append(pltpu.make_async_copy(xb.at[at], o_hbm.at[at], sem_o.at[NT - 1 + c]))
            last[-1].start()
    for copy in [o_copy(t) for t in range(NT - 1)] + last:
        copy.wait()


def _scratch_shapes():
    vmem = pltpu.VMEM
    lhs = vmem((7, T // 4, D // 2), u32)
    square = vmem((7, D // 4, D // 2), u32)
    per_row = vmem((T, 128), f32)
    chunks = vmem((NC, T, 128), f32)
    window = vmem((NC, HALO + 3 * T, 128), f32)
    return [
        vmem((S, D), bf16),
        vmem((3, D, D), bf16), vmem((D, D), bf16),
        vmem((D, F), bf16), vmem((F, D), bf16),
        vmem((NC, D // 2, 128), u32),
        vmem((NC, PAD * D // 64, 128), u32),
        square, square, square, square,
        vmem((7, D // 4, F // 2), u32), vmem((7, F // 4, D // 2), u32),
        vmem((40, 128), f32),
        lhs, lhs, lhs, lhs, lhs,
        vmem((7, T // 4, F // 2), u32), vmem((7, T // 4, F // 2), u32),
        per_row, per_row, per_row, per_row, per_row, per_row,
        chunks, per_row, vmem((NF, T, 128), f32), per_row, per_row,
        chunks, chunks, window, window, vmem((W, T, 128), f32),
        vmem((8, 128), u32),
        pltpu.SemaphoreType.DMA((NT,)), pltpu.SemaphoreType.DMA((7,)), pltpu.SemaphoreType.DMA((NT + NC,)),
    ]


@jax.jit
def pallas_interleave_layers__sliding_local_dilated__dense_activation_squared_relu__prompt_kernel(
    A_x: jax.Array,
    A_wqkv: jax.Array,
    A_wo: jax.Array,
    B_x: jax.Array,
    B_w1: jax.Array,
    B_b1: jax.Array,
    B_w2: jax.Array,
    B_b2: jax.Array,
):
    del B_x
    hbm = pl.BlockSpec(memory_space=pl.ANY)
    vmem = pl.BlockSpec(memory_space=pltpu.VMEM)
    out = pl.pallas_call(
        _kernel,
        in_specs=[hbm, hbm, hbm, hbm, vmem, hbm, vmem],
        out_specs=hbm,
        out_shape=jax.ShapeDtypeStruct((S, D), bf16),
        scratch_shapes=_scratch_shapes(),
        compiler_params=pltpu.CompilerParams(vmem_limit_bytes=110 * 2 ** 20),
    )(A_x.reshape(S, D), A_wqkv, A_wo, B_w1, B_b1.reshape(NF, 128), B_w2, B_b2.reshape(NC, 128))
    return out.reshape(1, S, D)
```

```python
import jax
import jax.numpy as jnp
from jax import lax
from jax.experimental import pallas as pl
from jax.experimental.pallas import tpu as pltpu

S, D, F = 2048, 1024, 3584
DH, W, DIL = 32, 8, 2
EPS = 1e-5
SCALE = DH ** -0.5
MASKED = -1e9
LOG2E = 1.4426950408889634
TINY = 1e-36

T = 256
TH = T // 2
NT = S // T
HALO = 16
NC = D // 128
NF = F // 128
SKEW = 3
UP_SPLIT = 13
PAD = DH + 1

f32 = jnp.float32
bf16 = jnp.bfloat16
u32 = jnp.uint32


def _pack_rows(x):
    return pltpu.bitcast(x.astype(bf16), u32)


def _as_bf16(u):
    return pltpu.bitcast(u, bf16)


class _Phase:
    def __init__(self, n, gen):
        self.n, self.gen = n, gen


def _chain(*phases):
    def gen():
        for p in phases:
            yield from p.gen
    return _Phase(sum(p.n for p in phases), gen())


def _take(phase, n):
    return _Phase(n, (next(phase.gen) for _ in range(n)))


def _mix(a, b):
    def gen():
        done = 0
        for i in range(a.n):
            yield next(a.gen)
            while done < (i + 1) * b.n // a.n:
                yield next(b.gen)
                done += 1
    return _Phase(a.n + b.n, gen())


class _Schedule:
    def __init__(self, zero_ref):
        self.zero_ref = zero_ref
        self.results = []
        self.token = None
        self.due = None
        self.carry = {}
        self.lag = 3

    def gate(self, *xs):
        if self.token is None:
            return list(xs)
        zero = pltpu.bitcast(self.token, u32) & self.zero_ref[...]
        out = []
        for x in xs:
            u = pltpu.bitcast(x, u32)
            out.append(pltpu.bitcast(u | jnp.tile(zero, (u.shape[0] // 8, u.shape[1] // 128)), x.dtype))
        return out

    def hold(self, lhs):
        if self.due is None:
            return lhs
        n = min(lhs.shape[1], 512)
        head = [lhs[:8, c:c + 128] | self.due for c in range(0, n, 128)]
        if lhs.shape[1] > n:
            head.append(lhs[:8, n:])
        self.due = None
        return jnp.concatenate([jnp.concatenate(head, axis=1), lhs[8:]], axis=0)

    def run(self, main, *side, lead=1, lag=None):
        lag = self.lag if lag is None else lag
        side = _chain(*side)
        slots = max(main.n - lead, 1)
        dues, done = dict(self.carry), 0
        self.carry = {}
        for i in range(main.n):
            self.results = []
            self.due = dues.pop(i, None)
            next(main.gen)
            tokens = [(y, r) for y in self.results for r in range(0, y.shape[0], 8)]
            want = min(side.n, -(-side.n * (i + 1) // slots))
            finished = None
            for j in range(want - done):
                y, r = tokens[j * len(tokens) // (want - done)]
                self.token = y[r:r + 8]
                last = next(side.gen)
                if last is not None:
                    last = pltpu.bitcast(last, u32)[:8, :128]
                    finished = last if finished is None else finished & last
            if finished is not None:
                dues[i + lag] = finished & self.zero_ref[...]
            done = want
        self.token = self.due = None
        self.carry = {i - main.n: z for i, z in dues.items()}
        for p in (main, side):
            assert next(p.gen, _Schedule) is _Schedule, "wrong piece count"

    def solo(self, *phases):
        self.due = self.carry.pop(0, None)
        self.carry = {}
        for p in phases:
            for _ in p.gen:
                pass
        self.due = None

    def barrier(self):
        self.carry = {}


def _kernel(x_hbm, wqkv_hbm, wo_hbm, w1_hbm, b1_ref, w2_hbm, b2_ref, o_hbm,
            xb, wqkv_raw, wo_raw, w1_raw, w2_raw, w_tmp, wo_tmp,
            wq7, wk7, wv7, wo7, w17, w27, bias,
            xa7, xb7, xf7, oa7, ob7, ha7, hb7, sa, sb, sf, soa, sob, sh,
            stage, stage_inv, h_stage, h_inv, h_ss,
            qa, qb, kk, vv, pp, zero_ref, sem_x, sem_w, sem_o):
    def x_copy(t):
        return pltpu.make_async_copy(x_hbm.at[pl.ds(t * T, T)], xb.at[pl.ds(t * T, T)], sem_x.at[t])

    def o_copy(t):
        return pltpu.make_async_copy(xb.at[pl.ds(t * T, T)], o_hbm.at[pl.ds(t * T, T)], sem_o.at[t])

    def wq_copy(half):
        rows = pl.ds(half * (D // 2), D // 2)
        return pltpu.make_async_copy(wqkv_hbm.at[rows, pl.ds(0, D)], wqkv_raw.at[0, rows], sem_w.at[half])

    def wkv_copy(i):
        return pltpu.make_async_copy(wqkv_hbm.at[:, pl.ds(i * D, D)], wqkv_raw.at[i], sem_w.at[1 + i])

    wo_copy = pltpu.make_async_copy(wo_hbm, wo_raw, sem_w.at[4])
    w1_copy = pltpu.make_async_copy(w1_hbm, w1_raw, sem_w.at[5])
    w2_copy = pltpu.make_async_copy(w2_hbm, w2_raw, sem_w.at[6])

    for copy in (x_copy(0), wq_copy(0), wq_copy(1), x_copy(1), wkv_copy(1), x_copy(2), wkv_copy(2), wo_copy,
                 x_copy(3), w1_copy, w2_copy, *[x_copy(t) for t in range(4, NT)]):
        copy.start()

    bias[0:NF, :] = b1_ref[...].astype(f32)
    bias[32:32 + NC, :] = b2_ref[...].astype(f32)
    zero_ref[...] = jnp.zeros((8, 128), u32)

    sched = _Schedule(zero_ref)
    tuning = [512, 0]
    gate, run, solo = sched.gate, sched.run, sched.solo

    def wait(copy):
        sched.barrier()
        copy.wait()

    def store_b7(dst, row, col, u11, u12, u21, u22):
        b11, b12, b21, b22 = ((_as_bf16(u) if u.dtype == u32 else u).astype(f32) for u in (u11, u12, u21, u22))
        at = (pl.ds(row, u11.shape[0]), pl.ds(col, u11.shape[1]))
        dst[(0,) + at] = _pack_rows(b11 + b22)
        dst[(1,) + at] = u11
        dst[(2,) + at] = _pack_rows(b12 - b22)
        dst[(3,) + at] = _pack_rows(b21 - b11)
        dst[(4,) + at] = u22
        dst[(5,) + at] = _pack_rows(b11 + b12)
        last = _pack_rows(b21 + b22)
        dst[(6,) + at] = last
        return last

    def a7_pieces(src, inv, dst):
        nk = src.shape[0] // 2
        for r in range(0, TH, 16):
            top, bot = inv[r:r + 16, :], inv[TH + r:TH + r + 16, :]
            for j in range(nk):
                top, bot = gate(top, bot)
                a11, a12, a21, a22 = (src[c, r0:r0 + 16, :] * scale
                                      for r0, scale in ((r, top), (TH + r, bot)) for c in (j, nk + j))
                at = (slice(r // 2, r // 2 + 8), slice(j * 128, (j + 1) * 128))
                dst[(0,) + at] = _pack_rows(a11 + a22)
                dst[(1,) + at] = _pack_rows(a21 + a22)
                dst[(2,) + at] = _pack_rows(a11)
                dst[(3,) + at] = _pack_rows(a22)
                dst[(4,) + at] = _pack_rows(a11 + a12)
                dst[(5,) + at] = _pack_rows(a21 - a11)
                last = _pack_rows(a12 - a22)
                dst[(6,) + at] = last
                yield last

    def matmul(a7, b7, emit, j0=0, j1=None):
        kh, nh = a7.shape[2], b7.shape[2] // 128
        k_step, order = tuning
        j1 = nh if j1 is None else j1

        def product(i, j):
            y = None
            for k in range(0, kh, k_step):
                ke = min(k + k_step, kh)
                yk = lax.dot_general(_as_bf16(sched.hold(a7[i, :, k:ke])),
                                     _as_bf16(b7[i, k // 2:ke // 2, j * 128:(j + 1) * 128]),
                                     (((1,), (0,)), ((), ())), preferred_element_type=f32)
                sched.results.append(yk)
                y = yk if y is None else y + yk
            return y

        def gen():
            for j in range(j0, j1):
                if order == 0:
                    m1, m2 = product(0, j), product(1, j)
                    c22 = m1 - m2
                    m4 = product(3, j)
                    emit(1, j, m2 + m4)
                    c11 = m1 + m4
                    c11 = c11 + product(6, j)
                    m5 = product(4, j)
                    emit(0, j, c11 - m5)
                    m3 = product(2, j)
                    emit(0, nh + j, m3 + m5)
                    c22 = c22 + m3
                    emit(1, nh + j, c22 + product(5, j))
                else:
                    m6, m2 = product(5, j), product(1, j)
                    c22 = m6 - m2
                    m3 = product(2, j)
                    c22 = c22 + m3
                    m1 = product(0, j)
                    emit(1, nh + j, c22 + m1)
                    m5 = product(4, j)
                    emit(0, nh + j, m3 + m5)
                    c11 = m1 - m5
                    m4 = product(3, j)
                    emit(1, j, m2 + m4)
                    c11 = c11 + m4
                    emit(0, j, c11 + product(6, j))
                yield
        return _Phase(j1 - j0, gen())

    def store_row_norm(ss, inv_ref, s_ref, r):
        ss = ss + TINY
        inv = lax.rsqrt(ss)
        shape = (ss.shape[0], 128)
        inv_ref[r:r + shape[0], :] = jnp.broadcast_to(inv, shape)
        norm = jnp.broadcast_to(ss * inv, shape)
        s_ref[r:r + shape[0], :] = norm
        return norm

    def qkv_skew(i, r0=0, r1=D):
        def gen(group=4):
            lane = lax.broadcasted_iota(jnp.int32, (8, 128), 1)
            bits = [(lane & (1 << b)) != 0 for b in range(3)]
            for g0 in range(r0 // 16, r1 // 16, group):
                xs = [[None] * NC for _ in range(group)]
                for c in range(NC):
                    for g in range(group):
                        rows = slice((g0 + g) * 16, (g0 + g + 1) * 16)
                        u, = gate(pltpu.bitcast(wqkv_raw[i, rows, c * 128:(c + 1) * 128], u32))
                        xs[g][c] = pltpu.roll(u, c, 1) if c else u
                for g in range(group):
                    ws = [xs[g][(-c) % NC] for c in range(NC)]
                    for b in range(3):
                        ws = [jnp.where(bits[b], ws[(c - (1 << b)) % NC], ws[c]) for c in range(NC)]
                    for c in range(NC):
                        w_tmp[c, (g0 + g) * 8:(g0 + g + 1) * 8, :] = ws[c]
                yield ws[0]
        return _Phase((r1 - r0) // 64, gen())

    def gather_lanes(c, r0):
        lane = lax.broadcasted_iota(jnp.int32, (64, 128), 1)
        base = (lane & 3) * 32 + (lane >> 5) * 8 + ((lane >> 2) & 7)
        for r in range(r0 // 2, r0 // 2 + D // 4, 64):
            u, = gate(w_tmp[c, r:r + 64, :])
            u = jnp.take_along_axis(u, (base + c) & 127, axis=1)
            w_tmp[c, r:r + 64, :] = u
        return u

    def qkv_finish(dst, j0, j1):
        def gen():
            for j in range(j0, j1):
                left, right = j, NC // 2 + j
                for c in (left, right):
                    gather_lanes(c, 0)
                    yield gather_lanes(c, D // 2)
                for r in range(0, D // 4, 16):
                    top, bot = slice(r, r + 16), slice(D // 4 + r, D // 4 + r + 16)
                    last = store_b7(dst, r, j * 128, w_tmp[left, top, :], w_tmp[right, top, :],
                                    w_tmp[left, bot, :], w_tmp[right, bot, :])
                yield last
        return _Phase(3 * (j1 - j0), gen())

    def wo_stage():
        def gen():
            for n in range(NC):
                u, = gate(pltpu.bitcast(wo_raw[:, n * 128:(n + 1) * 128], u32))
                for g in range(D // 64):
                    wo_tmp[n, pl.ds(PAD * g, 32), :] = u[32 * g:32 * (g + 1)]
                yield u
        return _Phase(NC, gen())

    def wo_finish():
        def rows16(n, cp, a):
            start = PAD * 8 * (a % 2) + 4 * (a // 2) + cp
            lo = wo_tmp[n, pl.ds(start, 8, stride=PAD), :]
            hi = wo_tmp[n, pl.ds(start + 16, 8, stride=PAD), :]
            return (lo & u32(0xFFFF)) | (hi << 16), (lo >> 16) | (hi & u32(0xFFFF0000))

        def gen():
            for j in range(NC // 2):
                for cp in range(NC // 4):
                    for a in range(8):
                        u11, u12 = rows16(j, cp, a), rows16(NC // 2 + j, cp, a)
                        u21, u22 = rows16(j, NC // 4 + cp, a), rows16(NC // 2 + j, NC // 4 + cp, a)
                        u11, u22 = gate(*u11), gate(*u22)
                        for odd in range(2):
                            last = store_b7(wo7, (2 * cp + odd) * 64 + 8 * a, j * 128,
                                            u11[odd], u12[odd], u21[odd], u22[odd])
                        if a % 2:
                            yield last
        return _Phase(NC * NC // 2, gen())

    def ffn_prepare(raw, dst, j0, j1, rows=32):
        kh, nh = raw.shape[0] // 2, raw.shape[1] // 2

        def gen():
            for c in range(j0 * 128, j1 * 128, 256):
                for r in range(0, kh, rows):
                    q = [raw[r0:r0 + rows, c0:c0 + 256] for r0 in (r, kh + r) for c0 in (c, nh + c)]
                    q[0], q[3] = gate(pltpu.bitcast(q[0], u32), pltpu.bitcast(q[3], u32))
                    yield store_b7(dst, r // 2, c, *q)
        return _Phase((j1 - j0) // 2 * kh // rows, gen())

    def layernorm(t, a7, s_ref):
        def gen():
            for r in range(0, T, 16):
                rows = pl.ds(pl.multiple_of(t * T + r, 16), 16)
                acc = None
                for c in range(NC):
                    x = xb[rows, c * 128:(c + 1) * 128]
                    if c == 0:
                        x, = gate(x)
                    acc = x.astype(f32) if acc is None else acc + x.astype(f32)
                mean = jnp.broadcast_to(jnp.sum(acc, axis=-1, keepdims=True) * (1.0 / D), (16, 128))
                yield mean
                mean, = gate(mean)
                acc = None
                for c in range(NC):
                    xc = xb[rows, c * 128:(c + 1) * 128].astype(f32) - mean
                    stage[c, r:r + 16, :] = xc
                    acc = xc * xc if acc is None else acc + xc * xc
                var = jnp.sum(acc, axis=-1, keepdims=True) * (1.0 / D)
                inv = lax.rsqrt(var + TINY)
                stage_inv[r:r + 16, :] = jnp.broadcast_to(inv, (16, 128))
                scale = jnp.broadcast_to((var + TINY) * inv * lax.rsqrt(var + EPS), (16, 128))
                s_ref[r:r + 16, :] = scale
                yield scale
            yield from a7_pieces(stage, stage_inv, a7)
        return _Phase(2 * T // 16 + TH // 16 * NC // 2, gen())

    def project(a7, s_ref, b7, dst, row0):
        def emit(half, c, y):
            dst[c, pl.ds(row0 + half * TH, TH), :] = y * s_ref[half * TH:(half + 1) * TH, :]
        return matmul(a7, b7, emit)

    def plain_lhs():
        for r in range(0, TH, 16):
            for j in range(NC // 2):
                at = (slice(r // 2, r // 2 + 8), slice(j * 128, (j + 1) * 128))
                ob7[(0,) + at] = _pack_rows(stage[NC // 2 + j, r:r + 16, :] * stage_inv[r:r + 16, :])
                ob7[(1,) + at] = _pack_rows(stage[j, TH + r:TH + r + 16, :] * stage_inv[TH + r:TH + r + 16, :])

    def first_q(k_half):
        def gen():
            blocks = (ob7[0], xa7[3]) if k_half else (xa7[2], ob7[1])
            for c in range(NC):
                lhs = jnp.concatenate([sched.hold(blocks[0]), blocks[1]], axis=0)
                rhs = w_tmp[c, k_half * (D // 4):(k_half + 1) * (D // 4), :]
                y = lax.dot_general(_as_bf16(lhs), _as_bf16(rhs), (((1,), (0,)), ((), ())),
                                    preferred_element_type=f32)
                sched.results.append(y)
                qa[c] = (qa[c] + y) * sa[...] if k_half else y
                yield
        return _Phase(NC, gen())

    def gather_bottom(c0, c1):
        return _Phase(c1 - c0, (gather_lanes(c, D // 2) for c in range(c0, c1)))

    def qkv_combine(dst):
        def gen():
            for j in range(NC // 2):
                for r in range(0, D // 4, 16):
                    q = [w_tmp[c, r0:r0 + 16, :] for r0 in (r, D // 4 + r) for c in (j, NC // 2 + j)]
                    q[0], q[3] = gate(q[0], q[3])
                    last = store_b7(dst, r, j * 128, *q)
                    if r % 64 == 48:
                        yield last
        return _Phase(NC * 2, gen())

    def attn_scores(q, row0, first, r0, r1, chunks):
        def gen():
            for r in range(r0, r1, 8):
                ls = [None] * W
                for c in range(NC):
                    qv, = gate(q[c, r:r + 8, :])
                    for w in range(W):
                        t = qv * kk[c, pl.ds(HALO + row0 + r - DIL * w, 8), :]
                        ls[w] = t if ls[w] is None else ls[w] + t
                    if c % chunks == chunks - 1 and c != NC - 1:
                        yield None
                for w in range(W):
                    t = ls[w] + pltpu.roll(ls[w], 64, 1)
                    t = t + pltpu.roll(t, 32, 1)
                    if first is not None and r < DIL * w:
                        row = lax.broadcasted_iota(jnp.int32, (8, 128), 0) + r
                        t = jnp.where(row < first * (DIL * w), MASKED / SCALE, t)
                    ls[w] = t
                m = ls[0]
                for w in range(1, W):
                    m = jnp.maximum(m, ls[w])
                es = [jnp.exp2((t - m) * (SCALE * LOG2E)) for t in ls]
                total = es[0]
                for w in range(1, W):
                    total = total + es[w]
                inv = 1.0 / total
                for w in range(W):
                    pp[w, r:r + 8, :] = es[w] * inv
                yield inv
        return _Phase((r1 - r0) // 8 * (NC // chunks), gen())

    def attn_mix(row0, o7, s_ref, r0, r1, chunks):
        def gen():
            for r in range(r0, r1, 8):
                ps = [pp[w, r:r + 8, :] for w in range(W)]
                ss = None
                for c in range(NC):
                    if c % chunks == 0:
                        ps = gate(*ps)
                    acc = None
                    for w in range(W):
                        t = ps[w] * vv[c, pl.ds(HALO + row0 + r - DIL * w, 8), :]
                        acc = t if acc is None else acc + t
                    stage[c, r:r + 8, :] = acc
                    ss = acc * acc if ss is None else ss + acc * acc
                    if c % chunks == chunks - 1 and c != NC - 1:
                        yield None
                yield store_row_norm(jnp.sum(ss, axis=-1, keepdims=True), stage_inv, s_ref, r)
            if r1 == T:
                yield from a7_pieces(stage, stage_inv, o7)
        return _Phase((r1 - r0) // 8 * (NC // chunks) + (TH // 16 * NC // 2 if r1 == T else 0), gen())

    def add_residual(t, a7, s_ref, b7, bias_row):
        def emit(half, c, y):
            rows = pl.ds(pl.multiple_of(t * T + half * TH, TH), TH)
            cols = slice(c * 128, (c + 1) * 128)
            z = y * s_ref[half * TH:(half + 1) * TH, :]
            if bias_row is not None:
                z = z + bias[bias_row + c:bias_row + c + 1, :]
            xb[rows, cols] = (xb[rows, cols].astype(f32) + z).astype(bf16)
        return matmul(a7, b7, emit)

    def attn_out(t, o7, s_ref):
        return add_residual(t, o7, s_ref, wo7, None)

    def ffn_up(j0=0, j1=NF // 2, a7=xf7, s_ref=sf):
        started = [j0 > 0, j0 > 0]

        def emit(half, c, y):
            rows = slice(half * TH, (half + 1) * TH)
            z = jnp.maximum(y * s_ref[rows, :] + bias[c:c + 1, :], 0.0)
            z = z * z
            h_stage[c, rows, :] = z
            h_ss[rows, :] = h_ss[rows, :] + z * z if started[half] else z * z
            started[half] = True
        return matmul(a7, w17, emit, j0, j1)

    def ffn_mid(h7=ha7, s_ref=sh):
        def gen():
            for r in range(0, T, 32):
                ss, = gate(h_ss[r:r + 32, :])
                yield store_row_norm(jnp.sum(ss, axis=-1, keepdims=True), h_inv, s_ref, r)
            yield from a7_pieces(h_stage, h_inv, h7)
        return _Phase(T // 32 + TH // 16 * NF // 2, gen())

    def ffn_down(t, h7=ha7, s_ref=sh):
        return add_residual(t, h7, s_ref, w27, 32)

    def move_halo(ref, src, dst):
        for c in range(NC):
            ref[c, pl.ds(dst, HALO), :] = ref[c, pl.ds(src, HALO), :]

    k0, k1, k2 = HALO, HALO + T, HALO + 2 * T
    wait(x_copy(0))
    solo(layernorm(0, xa7, sa))
    plain_lhs()
    wait(wq_copy(0))
    solo(qkv_skew(0, 0, D // 2))
    for c in range(NC):
        gather_lanes(c, 0)
    solo(first_q(0))
    wait(wq_copy(1))
    solo(qkv_skew(0, D // 2, D), gather_bottom(0, 2))
    wait(x_copy(1))
    run(first_q(1), _mix(layernorm(1, xb7, sb), _chain(gather_bottom(2, NC), qkv_combine(wq7))), lead=0, lag=9)
    q1 = project(xb7, sb, wq7, qb, 0)
    solo(_take(q1, 1))
    wait(wkv_copy(1))
    run(_chain(_take(q1, 3), project(xa7, sa, wk7, kk, k0)), qkv_skew(1), qkv_finish(wk7, 0, 4), lead=3, lag=2)
    for c in range(NC):
        kk[c, 0:HALO, :] = jnp.zeros((HALO, 128), f32)
    wait(x_copy(2))
    run(project(xb7, sb, wk7, kk, k1), layernorm(2, xf7, sf), attn_scores(qa, 0, 1, 0, 160, 4), lead=0, lag=9)
    wait(wkv_copy(2))
    run(project(xf7, sf, wk7, kk, k2), qkv_skew(2), qkv_finish(wv7, 0, 2))
    wait(wo_copy)
    run(project(xa7, sa, wv7, vv, k0), qkv_finish(wv7, 2, 4), attn_scores(qa, 0, 1, 160, T, 4), wo_stage(), lead=0)
    for c in range(NC):
        vv[c, 0:HALO, :] = jnp.broadcast_to(vv[c, HALO:HALO + 1, :], (HALO, 128))
    wait(x_copy(3))
    run(project(xb7, sb, wv7, vv, k1), wo_finish(), attn_mix(0, oa7, soa, 0, 160, 4), lead=0, lag=9)
    run(project(xf7, sf, wq7, qa, 0), attn_mix(0, oa7, soa, 160, T, 4), attn_scores(qb, T, None, 0, 192, 4),
        lead=0, lag=9)
    wait(w1_copy)
    run(project(xf7, sf, wv7, vv, k2), attn_scores(qb, T, None, 192, T, 4), attn_mix(T, ob7, sob, 0, 128, 4),
        ffn_prepare(w1_raw, w17, 0, 4), lead=0)
    run(attn_out(0, oa7, soa), attn_mix(T, ob7, sob, 128, T, 4), ffn_prepare(w1_raw, w17, 4, 6), lead=0)
    run(attn_out(1, ob7, sob), _mix(layernorm(0, xf7, sf), ffn_prepare(w1_raw, w17, 6, 8)), lead=0, lag=2)
    run(ffn_up(0, 6), ffn_prepare(w1_raw, w17, 8, NF // 2), attn_scores(qa, 2 * T, None, 0, T, 8),
        attn_mix(2 * T, oa7, soa, 0, 192, 8), lead=0)
    move_halo(kk, 3 * T, T)
    wait(w2_copy)
    run(ffn_up(6, UP_SPLIT), attn_mix(2 * T, oa7, soa, 192, T, 8), layernorm(3, xa7, sa),
        ffn_prepare(w2_raw, w27, 0, 2, 16), lead=0)
    move_halo(vv, 3 * T, T)
    run(attn_out(2, oa7, soa), ffn_prepare(w2_raw, w27, 2, NC // 2, 16), lead=0, lag=9)

    sched.barrier()
    tuning[:] = 1024, 1

    def step(i, _):
        t_attn = (i + SKEW) % NT
        first = (t_attn == 0).astype(jnp.int32)

        @pl.when(i + SKEW + 1 < NT)
        def _():
            x_copy(i + SKEW + 1).wait()

        move_halo(kk, T, 0)
        move_halo(vv, T, 0)
        solo(ffn_up(UP_SPLIT))
        run(_chain(project(xa7, sa, wq7, qa, 0), project(xa7, sa, wk7, kk, k0)),
            layernorm((i + 1) % NT, xf7, sf), ffn_mid(), lag=2)
        run(project(xa7, sa, wv7, vv, k0), attn_scores(qa, 0, first, 0, 112, 8), lead=0, lag=2)
        for c in range(NC):
            v0 = jnp.broadcast_to(vv[c, HALO:HALO + 1, :], (HALO, 128))
            vv[c, 0:HALO, :] = jnp.where(t_attn == 0, v0, vv[c, 0:HALO, :])
        run(ffn_down(i % NT), attn_scores(qa, 0, first, 112, T, 4), attn_mix(0, oa7, soa, 0, T, 4), lag=2)
        solo(attn_out(t_attn, oa7, soa))
        run(ffn_up(0, UP_SPLIT), layernorm((i + SKEW + 1) % NT, xa7, sa), lead=4)
        sched.barrier()

        @pl.when(i >= NT)
        def _():
            o_copy(i - NT).start()
        return 0

    lax.fori_loop(0, 2 * NT - SKEW, step, 0)

    down_a, down_b = ffn_down(NT - 3), ffn_down(NT - 2, hb7, sob)
    solo(ffn_up(UP_SPLIT), ffn_mid())
    run(_take(down_a, 2), layernorm(NT - 2, xf7, sf), lead=0)
    run(ffn_up(), layernorm(NT - 1, xa7, sa), lead=6)
    run(_chain(_take(down_a, 2), _take(down_b, 1)), ffn_mid(hb7, sob), lead=2)
    solo(ffn_up(a7=xa7, s_ref=sa))
    run(_take(down_b, 3), ffn_mid(), lead=0)
    sched.barrier()
    o_copy(NT - 3).start()
    o_copy(NT - 2).start()
    down_c = ffn_down(NT - 1)
    last = []
    for j in range(NC // 2):
        solo(_take(down_c, 1))
        for c in (j, NC // 2 + j):
            at = (pl.ds((NT - 1) * T, T), pl.ds(c * 128, 128))
            last.append(pltpu.make_async_copy(xb.at[at], o_hbm.at[at], sem_o.at[NT - 1 + c]))
            last[-1].start()
    for copy in [o_copy(t) for t in range(NT - 1)] + last:
        copy.wait()


def _scratch_shapes():
    vmem = pltpu.VMEM
    lhs = vmem((7, T // 4, D // 2), u32)
    square = vmem((7, D // 4, D // 2), u32)
    per_row = vmem((T, 128), f32)
    chunks = vmem((NC, T, 128), f32)
    window = vmem((NC, HALO + 3 * T, 128), f32)
    return [
        vmem((S, D), bf16),
        vmem((3, D, D), bf16), vmem((D, D), bf16),
        vmem((D, F), bf16), vmem((F, D), bf16),
        vmem((NC, D // 2, 128), u32),
        vmem((NC, PAD * D // 64, 128), u32),
        square, square, square, square,
        vmem((7, D // 4, F // 2), u32), vmem((7, F // 4, D // 2), u32),
        vmem((40, 128), f32),
        lhs, lhs, lhs, lhs, lhs,
        vmem((7, T // 4, F // 2), u32), vmem((7, T // 4, F // 2), u32),
        per_row, per_row, per_row, per_row, per_row, per_row,
        chunks, per_row, vmem((NF, T, 128), f32), per_row, per_row,
        chunks, chunks, window, window, vmem((W, T, 128), f32),
        vmem((8, 128), u32),
        pltpu.SemaphoreType.DMA((NT,)), pltpu.SemaphoreType.DMA((7,)), pltpu.SemaphoreType.DMA((NT + NC,)),
    ]


@jax.jit
def pallas_interleave_layers__sliding_local_dilated__dense_activation_squared_relu__prompt_kernel(
    A_x: jax.Array,
    A_wqkv: jax.Array,
    A_wo: jax.Array,
    B_x: jax.Array,
    B_w1: jax.Array,
    B_b1: jax.Array,
    B_w2: jax.Array,
    B_b2: jax.Array,
):
    del B_x
    hbm = pl.BlockSpec(memory_space=pl.ANY)
    vmem = pl.BlockSpec(memory_space=pltpu.VMEM)
    out = pl.pallas_call(
        _kernel,
        in_specs=[hbm, hbm, hbm, hbm, vmem, hbm, vmem],
        out_specs=hbm,
        out_shape=jax.ShapeDtypeStruct((S, D), bf16),
        scratch_shapes=_scratch_shapes(),
        compiler_params=pltpu.CompilerParams(vmem_limit_bytes=110 * 2 ** 20),
    )(A_x.reshape(S, D), A_wqkv, A_wo, B_w1, B_b1.reshape(NF, 128), B_w2, B_b2.reshape(NC, 128))
    return out.reshape(1, S, D)
```

```python
import jax
import jax.numpy as jnp
from jax import lax
from jax.experimental import pallas as pl
from jax.experimental.pallas import tpu as pltpu

S, D, F = 2048, 1024, 3584
DH, W, DIL = 32, 8, 2
EPS = 1e-5
SCALE = DH ** -0.5
MASKED = -1e9
LOG2E = 1.4426950408889634
TINY = 1e-36

T = 256
TH = T // 2
NT = S // T
HALO = 16
NC = D // 128
NF = F // 128
SKEW = 3
UP_SPLIT = 13
PAD = DH + 1

f32 = jnp.float32
bf16 = jnp.bfloat16
u32 = jnp.uint32


def _pack_rows(x):
    return pltpu.bitcast(x.astype(bf16), u32)


def _as_bf16(u):
    return pltpu.bitcast(u, bf16)


class _Phase:
    def __init__(self, n, gen):
        self.n, self.gen = n, gen


def _chain(*phases):
    def gen():
        for p in phases:
            yield from p.gen
    return _Phase(sum(p.n for p in phases), gen())


def _take(phase, n):
    return _Phase(n, (next(phase.gen) for _ in range(n)))


def _mix(a, b):
    def gen():
        done = 0
        for i in range(a.n):
            yield next(a.gen)
            while done < (i + 1) * b.n // a.n:
                yield next(b.gen)
                done += 1
    return _Phase(a.n + b.n, gen())


class _Schedule:
    def __init__(self, zero_ref):
        self.zero_ref = zero_ref
        self.results = []
        self.token = None
        self.due = None
        self.carry = {}
        self.lag = 3

    def gate(self, *xs):
        if self.token is None:
            return list(xs)
        zero = pltpu.bitcast(self.token, u32) & self.zero_ref[...]
        out = []
        for x in xs:
            u = pltpu.bitcast(x, u32)
            out.append(pltpu.bitcast(u | jnp.tile(zero, (u.shape[0] // 8, u.shape[1] // 128)), x.dtype))
        return out

    def hold(self, lhs):
        if self.due is None:
            return lhs
        n = min(lhs.shape[1], 512)
        head = [lhs[:8, c:c + 128] | self.due for c in range(0, n, 128)]
        if lhs.shape[1] > n:
            head.append(lhs[:8, n:])
        self.due = None
        return jnp.concatenate([jnp.concatenate(head, axis=1), lhs[8:]], axis=0)

    def run(self, main, *side, lead=1, lag=None):
        lag = self.lag if lag is None else lag
        side = _chain(*side)
        slots = max(main.n - lead, 1)
        dues, done = dict(self.carry), 0
        self.carry = {}
        for i in range(main.n):
            self.results = []
            self.due = dues.pop(i, None)
            next(main.gen)
            tokens = [(y, r) for y in self.results for r in range(0, y.shape[0], 8)]
            want = min(side.n, -(-side.n * (i + 1) // slots))
            finished = None
            for j in range(want - done):
                y, r = tokens[j * len(tokens) // (want - done)]
                self.token = y[r:r + 8]
                last = next(side.gen)
                if last is not None:
                    last = pltpu.bitcast(last, u32)[:8, :128]
                    finished = last if finished is None else finished & last
            if finished is not None:
                dues[i + lag] = finished & self.zero_ref[...]
            done = want
        self.token = self.due = None
        self.carry = {i - main.n: z for i, z in dues.items()}
        for p in (main, side):
            assert next(p.gen, _Schedule) is _Schedule, "wrong piece count"

    def solo(self, *phases):
        self.due = self.carry.pop(0, None)
        self.carry = {}
        for p in phases:
            for _ in p.gen:
                pass
        self.due = None

    def barrier(self):
        self.carry = {}


def _kernel(x_hbm, wqkv_hbm, wo_hbm, w1_hbm, b1_ref, w2_hbm, b2_ref, o_hbm,
            xb, wqkv_raw, wo_raw, w1_raw, w2_raw, w_tmp, wo_tmp,
            wq7, wk7, wv7, wo7, w17, w27, bias,
            xa7, xb7, xf7, oa7, ob7, ha7, hb7, sa, sb, sf, soa, sob, sh,
            stage, stage_inv, h_stage, h_inv, h_ss,
            qa, qb, kk, vv, pp, zero_ref, sem_x, sem_w, sem_o):
    def x_copy(t):
        return pltpu.make_async_copy(x_hbm.at[pl.ds(t * T, T)], xb.at[pl.ds(t * T, T)], sem_x.at[t])

    def o_copy(t):
        return pltpu.make_async_copy(xb.at[pl.ds(t * T, T)], o_hbm.at[pl.ds(t * T, T)], sem_o.at[t])

    def wq_copy(half):
        rows = pl.ds(half * (D // 2), D // 2)
        return pltpu.make_async_copy(wqkv_hbm.at[rows, pl.ds(0, D)], wqkv_raw.at[0, rows], sem_w.at[half])

    def wkv_copy(i):
        return pltpu.make_async_copy(wqkv_hbm.at[:, pl.ds(i * D, D)], wqkv_raw.at[i], sem_w.at[1 + i])

    wo_copy = pltpu.make_async_copy(wo_hbm, wo_raw, sem_w.at[4])
    w1_copy = pltpu.make_async_copy(w1_hbm, w1_raw, sem_w.at[5])
    w2_copy = pltpu.make_async_copy(w2_hbm, w2_raw, sem_w.at[6])

    for copy in (x_copy(0), wq_copy(0), wq_copy(1), x_copy(1), wkv_copy(1), x_copy(2), wkv_copy(2), wo_copy,
                 x_copy(3), w1_copy, w2_copy, *[x_copy(t) for t in range(4, NT)]):
        copy.start()

    bias[0:NF, :] = b1_ref[...].astype(f32)
    bias[32:32 + NC, :] = b2_ref[...].astype(f32)
    zero_ref[...] = jnp.zeros((8, 128), u32)

    sched = _Schedule(zero_ref)
    tuning = [512, 0]
    gate, run, solo = sched.gate, sched.run, sched.solo

    def wait(copy):
        sched.barrier()
        copy.wait()

    def store_b7(dst, row, col, u11, u12, u21, u22):
        b11, b12, b21, b22 = ((_as_bf16(u) if u.dtype == u32 else u).astype(f32) for u in (u11, u12, u21, u22))
        at = (pl.ds(row, u11.shape[0]), pl.ds(col, u11.shape[1]))
        dst[(0,) + at] = _pack_rows(b11 + b22)
        dst[(1,) + at] = u11
        dst[(2,) + at] = _pack_rows(b12 - b22)
        dst[(3,) + at] = _pack_rows(b21 - b11)
        dst[(4,) + at] = u22
        dst[(5,) + at] = _pack_rows(b11 + b12)
        last = _pack_rows(b21 + b22)
        dst[(6,) + at] = last
        return last

    def a7_pieces(src, inv, dst):
        nk = src.shape[0] // 2
        for r in range(0, TH, 16):
            top, bot = inv[r:r + 16, :], inv[TH + r:TH + r + 16, :]
            for j in range(nk):
                top, bot = gate(top, bot)
                a11, a12, a21, a22 = (src[c, r0:r0 + 16, :] * scale
                                      for r0, scale in ((r, top), (TH + r, bot)) for c in (j, nk + j))
                at = (slice(r // 2, r // 2 + 8), slice(j * 128, (j + 1) * 128))
                dst[(0,) + at] = _pack_rows(a11 + a22)
                dst[(1,) + at] = _pack_rows(a21 + a22)
                dst[(2,) + at] = _pack_rows(a11)
                dst[(3,) + at] = _pack_rows(a22)
                dst[(4,) + at] = _pack_rows(a11 + a12)
                dst[(5,) + at] = _pack_rows(a21 - a11)
                last = _pack_rows(a12 - a22)
                dst[(6,) + at] = last
                yield last

    def matmul(a7, b7, emit, j0=0, j1=None):
        kh, nh = a7.shape[2], b7.shape[2] // 128
        k_step, order = tuning
        j1 = nh if j1 is None else j1

        def product(i, j):
            y = None
            for k in range(0, kh, k_step):
                ke = min(k + k_step, kh)
                yk = lax.dot_general(_as_bf16(sched.hold(a7[i, :, k:ke])),
                                     _as_bf16(b7[i, k // 2:ke // 2, j * 128:(j + 1) * 128]),
                                     (((1,), (0,)), ((), ())), preferred_element_type=f32)
                sched.results.append(yk)
                y = yk if y is None else y + yk
            return y

        def gen():
            for j in range(j0, j1):
                if order == 0:
                    m1, m2 = product(0, j), product(1, j)
                    c22 = m1 - m2
                    m4 = product(3, j)
                    emit(1, j, m2 + m4)
                    c11 = m1 + m4
                    c11 = c11 + product(6, j)
                    m5 = product(4, j)
                    emit(0, j, c11 - m5)
                    m3 = product(2, j)
                    emit(0, nh + j, m3 + m5)
                    c22 = c22 + m3
                    emit(1, nh + j, c22 + product(5, j))
                else:
                    m6, m2 = product(5, j), product(1, j)
                    c22 = m6 - m2
                    m3 = product(2, j)
                    c22 = c22 + m3
                    m1 = product(0, j)
                    emit(1, nh + j, c22 + m1)
                    m5 = product(4, j)
                    emit(0, nh + j, m3 + m5)
                    c11 = m1 - m5
                    m4 = product(3, j)
                    emit(1, j, m2 + m4)
                    c11 = c11 + m4
                    emit(0, j, c11 + product(6, j))
                yield
        return _Phase(j1 - j0, gen())

    def store_row_norm(ss, inv_ref, s_ref, r):
        ss = ss + TINY
        inv = lax.rsqrt(ss)
        shape = (ss.shape[0], 128)
        inv_ref[r:r + shape[0], :] = jnp.broadcast_to(inv, shape)
        norm = jnp.broadcast_to(ss * inv, shape)
        s_ref[r:r + shape[0], :] = norm
        return norm

    def qkv_skew(i, r0=0, r1=D):
        def gen(group=4):
            lane = lax.broadcasted_iota(jnp.int32, (8, 128), 1)
            bits = [(lane & (1 << b)) != 0 for b in range(3)]
            for g0 in range(r0 // 16, r1 // 16, group):
                xs = [[None] * NC for _ in range(group)]
                for c in range(NC):
                    for g in range(group):
                        rows = slice((g0 + g) * 16, (g0 + g + 1) * 16)
                        u, = gate(pltpu.bitcast(wqkv_raw[i, rows, c * 128:(c + 1) * 128], u32))
                        xs[g][c] = pltpu.roll(u, c, 1) if c else u
                for g in range(group):
                    ws = [xs[g][(-c) % NC] for c in range(NC)]
                    for b in range(3):
                        ws = [jnp.where(bits[b], ws[(c - (1 << b)) % NC], ws[c]) for c in range(NC)]
                    for c in range(NC):
                        w_tmp[c, (g0 + g) * 8:(g0 + g + 1) * 8, :] = ws[c]
                yield ws[0]
        return _Phase((r1 - r0) // 64, gen())

    def gather_lanes(c, r0):
        lane = lax.broadcasted_iota(jnp.int32, (64, 128), 1)
        base = (lane & 3) * 32 + (lane >> 5) * 8 + ((lane >> 2) & 7)
        for r in range(r0 // 2, r0 // 2 + D // 4, 64):
            u, = gate(w_tmp[c, r:r + 64, :])
            u = jnp.take_along_axis(u, (base + c) & 127, axis=1)
            w_tmp[c, r:r + 64, :] = u
        return u

    def qkv_finish(dst, j0, j1):
        def gen():
            for j in range(j0, j1):
                left, right = j, NC // 2 + j
                for c in (left, right):
                    gather_lanes(c, 0)
                    yield gather_lanes(c, D // 2)
                for r in range(0, D // 4, 16):
                    top, bot = slice(r, r + 16), slice(D // 4 + r, D // 4 + r + 16)
                    last = store_b7(dst, r, j * 128, w_tmp[left, top, :], w_tmp[right, top, :],
                                    w_tmp[left, bot, :], w_tmp[right, bot, :])
                yield last
        return _Phase(3 * (j1 - j0), gen())

    def wo_stage():
        def gen():
            for n in range(NC):
                for g in range(D // 64):
                    u, = gate(pltpu.bitcast(wo_raw[64 * g:64 * (g + 1), n * 128:(n + 1) * 128], u32))
                    wo_tmp[n, pl.ds(PAD * g, 32), :] = u
                    if g % 4 == 3:
                        yield u
        return _Phase(NC * 4, gen())

    def wo_finish():
        def rows16(n, cp, a):
            start = PAD * 8 * (a % 2) + 4 * (a // 2) + cp
            lo = wo_tmp[n, pl.ds(start, 8, stride=PAD), :]
            hi = wo_tmp[n, pl.ds(start + 16, 8, stride=PAD), :]
            return (lo & u32(0xFFFF)) | (hi << 16), (lo >> 16) | (hi & u32(0xFFFF0000))

        def gen():
            for j in range(NC // 2):
                for cp in range(NC // 4):
                    for a in range(8):
                        u11, u12 = rows16(j, cp, a), rows16(NC // 2 + j, cp, a)
                        u21, u22 = rows16(j, NC // 4 + cp, a), rows16(NC // 2 + j, NC // 4 + cp, a)
                        u11, u22 = gate(*u11), gate(*u22)
                        for odd in range(2):
                            last = store_b7(wo7, (2 * cp + odd) * 64 + 8 * a, j * 128,
                                            u11[odd], u12[odd], u21[odd], u22[odd])
                        if a % 2:
                            yield last
        return _Phase(NC * NC // 2, gen())

    def ffn_prepare(raw, dst, j0, j1, rows=32):
        kh, nh = raw.shape[0] // 2, raw.shape[1] // 2

        def gen():
            for c in range(j0 * 128, j1 * 128, 256):
                for r in range(0, kh, rows):
                    q = [raw[r0:r0 + rows, c0:c0 + 256] for r0 in (r, kh + r) for c0 in (c, nh + c)]
                    q[0], q[3] = gate(pltpu.bitcast(q[0], u32), pltpu.bitcast(q[3], u32))
                    yield store_b7(dst, r // 2, c, *q)
        return _Phase((j1 - j0) // 2 * kh // rows, gen())

    def layernorm(t, a7, s_ref):
        def gen():
            for r in range(0, T, 16):
                rows = pl.ds(pl.multiple_of(t * T + r, 16), 16)
                acc = None
                for c in range(NC):
                    x = xb[rows, c * 128:(c + 1) * 128]
                    if c == 0:
                        x, = gate(x)
                    acc = x.astype(f32) if acc is None else acc + x.astype(f32)
                mean = jnp.broadcast_to(jnp.sum(acc, axis=-1, keepdims=True) * (1.0 / D), (16, 128))
                yield mean
                mean, = gate(mean)
                acc = None
                for c in range(NC):
                    xc = xb[rows, c * 128:(c + 1) * 128].astype(f32) - mean
                    stage[c, r:r + 16, :] = xc
                    acc = xc * xc if acc is None else acc + xc * xc
                var = jnp.sum(acc, axis=-1, keepdims=True) * (1.0 / D)
                inv = lax.rsqrt(var + TINY)
                stage_inv[r:r + 16, :] = jnp.broadcast_to(inv, (16, 128))
                scale = jnp.broadcast_to((var + TINY) * inv * lax.rsqrt(var + EPS), (16, 128))
                s_ref[r:r + 16, :] = scale
                yield scale
            yield from a7_pieces(stage, stage_inv, a7)
        return _Phase(2 * T // 16 + TH // 16 * NC // 2, gen())

    def project(a7, s_ref, b7, dst, row0):
        def emit(half, c, y):
            dst[c, pl.ds(row0 + half * TH, TH), :] = y * s_ref[half * TH:(half + 1) * TH, :]
        return matmul(a7, b7, emit)

    def plain_lhs():
        for r in range(0, TH, 16):
            for j in range(NC // 2):
                at = (slice(r // 2, r // 2 + 8), slice(j * 128, (j + 1) * 128))
                ob7[(0,) + at] = _pack_rows(stage[NC // 2 + j, r:r + 16, :] * stage_inv[r:r + 16, :])
                ob7[(1,) + at] = _pack_rows(stage[j, TH + r:TH + r + 16, :] * stage_inv[TH + r:TH + r + 16, :])

    def first_q(k_half):
        def gen():
            blocks = (ob7[0], xa7[3]) if k_half else (xa7[2], ob7[1])
            for c in range(NC):
                lhs = jnp.concatenate([sched.hold(blocks[0]), blocks[1]], axis=0)
                rhs = w_tmp[c, k_half * (D // 4):(k_half + 1) * (D // 4), :]
                y = lax.dot_general(_as_bf16(lhs), _as_bf16(rhs), (((1,), (0,)), ((), ())),
                                    preferred_element_type=f32)
                sched.results.append(y)
                qa[c] = (qa[c] + y) * sa[...] if k_half else y
                yield
        return _Phase(NC, gen())

    def gather_bottom(c0, c1):
        return _Phase(c1 - c0, (gather_lanes(c, D // 2) for c in range(c0, c1)))

    def qkv_combine(dst):
        def gen():
            for j in range(NC // 2):
                for r in range(0, D // 4, 16):
                    q = [w_tmp[c, r0:r0 + 16, :] for r0 in (r, D // 4 + r) for c in (j, NC // 2 + j)]
                    q[0], q[3] = gate(q[0], q[3])
                    last = store_b7(dst, r, j * 128, *q)
                    if r % 64 == 48:
                        yield last
        return _Phase(NC * 2, gen())

    def attn_scores(q, row0, first, r0, r1, chunks):
        def gen():
            for r in range(r0, r1, 8):
                ls = [None] * W
                for c in range(NC):
                    qv, = gate(q[c, r:r + 8, :])
                    for w in range(W):
                        t = qv * kk[c, pl.ds(HALO + row0 + r - DIL * w, 8), :]
                        ls[w] = t if ls[w] is None else ls[w] + t
                    if c % chunks == chunks - 1 and c != NC - 1:
                        yield None
                for w in range(W):
                    t = ls[w] + pltpu.roll(ls[w], 64, 1)
                    t = t + pltpu.roll(t, 32, 1)
                    if first is not None and r < DIL * w:
                        row = lax.broadcasted_iota(jnp.int32, (8, 128), 0) + r
                        t = jnp.where(row < first * (DIL * w), MASKED / SCALE, t)
                    ls[w] = t
                m = ls[0]
                for w in range(1, W):
                    m = jnp.maximum(m, ls[w])
                es = [jnp.exp2((t - m) * (SCALE * LOG2E)) for t in ls]
                total = es[0]
                for w in range(1, W):
                    total = total + es[w]
                inv = 1.0 / total
                for w in range(W):
                    pp[w, r:r + 8, :] = es[w] * inv
                yield inv
        return _Phase((r1 - r0) // 8 * (NC // chunks), gen())

    def attn_mix(row0, o7, s_ref, r0, r1, chunks):
        def gen():
            for r in range(r0, r1, 8):
                ps = [pp[w, r:r + 8, :] for w in range(W)]
                ss = None
                for c in range(NC):
                    if c % chunks == 0:
                        ps = gate(*ps)
                    acc = None
                    for w in range(W):
                        t = ps[w] * vv[c, pl.ds(HALO + row0 + r - DIL * w, 8), :]
                        acc = t if acc is None else acc + t
                    stage[c, r:r + 8, :] = acc
                    ss = acc * acc if ss is None else ss + acc * acc
                    if c % chunks == chunks - 1 and c != NC - 1:
                        yield None
                yield store_row_norm(jnp.sum(ss, axis=-1, keepdims=True), stage_inv, s_ref, r)
            if r1 == T:
                yield from a7_pieces(stage, stage_inv, o7)
        return _Phase((r1 - r0) // 8 * (NC // chunks) + (TH // 16 * NC // 2 if r1 == T else 0), gen())

    def add_residual(t, a7, s_ref, b7, bias_row):
        def emit(half, c, y):
            rows = pl.ds(pl.multiple_of(t * T + half * TH, TH), TH)
            cols = slice(c * 128, (c + 1) * 128)
            z = y * s_ref[half * TH:(half + 1) * TH, :]
            if bias_row is not None:
                z = z + bias[bias_row + c:bias_row + c + 1, :]
            xb[rows, cols] = (xb[rows, cols].astype(f32) + z).astype(bf16)
        return matmul(a7, b7, emit)

    def attn_out(t, o7, s_ref):
        return add_residual(t, o7, s_ref, wo7, None)

    def ffn_up(j0=0, j1=NF // 2, a7=xf7, s_ref=sf):
        started = [j0 > 0, j0 > 0]

        def emit(half, c, y):
            rows = slice(half * TH, (half + 1) * TH)
            z = jnp.maximum(y * s_ref[rows, :] + bias[c:c + 1, :], 0.0)
            z = z * z
            h_stage[c, rows, :] = z
            h_ss[rows, :] = h_ss[rows, :] + z * z if started[half] else z * z
            started[half] = True
        return matmul(a7, w17, emit, j0, j1)

    def ffn_mid(h7=ha7, s_ref=sh):
        def gen():
            for r in range(0, T, 32):
                ss, = gate(h_ss[r:r + 32, :])
                yield store_row_norm(jnp.sum(ss, axis=-1, keepdims=True), h_inv, s_ref, r)
            yield from a7_pieces(h_stage, h_inv, h7)
        return _Phase(T // 32 + TH // 16 * NF // 2, gen())

    def ffn_down(t, h7=ha7, s_ref=sh):
        return add_residual(t, h7, s_ref, w27, 32)

    def move_halo(ref, src, dst):
        for c in range(NC):
            ref[c, pl.ds(dst, HALO), :] = ref[c, pl.ds(src, HALO), :]

    k0, k1, k2 = HALO, HALO + T, HALO + 2 * T
    wait(x_copy(0))
    solo(layernorm(0, xa7, sa))
    plain_lhs()
    wait(wq_copy(0))
    solo(qkv_skew(0, 0, D // 2))
    for c in range(NC):
        gather_lanes(c, 0)
    solo(first_q(0))
    wait(wq_copy(1))
    solo(qkv_skew(0, D // 2, D), gather_bottom(0, 2))
    wait(x_copy(1))
    run(first_q(1), _mix(layernorm(1, xb7, sb), _chain(gather_bottom(2, NC), qkv_combine(wq7))), lead=0, lag=9)
    q1 = project(xb7, sb, wq7, qb, 0)
    solo(_take(q1, 1))
    wait(wkv_copy(1))
    run(_chain(_take(q1, 3), project(xa7, sa, wk7, kk, k0)), qkv_skew(1), qkv_finish(wk7, 0, 4), lead=3, lag=2)
    for c in range(NC):
        kk[c, 0:HALO, :] = jnp.zeros((HALO, 128), f32)
    wait(x_copy(2))
    run(project(xb7, sb, wk7, kk, k1), layernorm(2, xf7, sf), attn_scores(qa, 0, 1, 0, 160, 4), lead=0, lag=9)
    wait(wkv_copy(2))
    run(project(xf7, sf, wk7, kk, k2), qkv_skew(2), qkv_finish(wv7, 0, 2))
    wait(wo_copy)
    run(project(xa7, sa, wv7, vv, k0), qkv_finish(wv7, 2, 4), attn_scores(qa, 0, 1, 160, T, 4), wo_stage(), lead=0)
    for c in range(NC):
        vv[c, 0:HALO, :] = jnp.broadcast_to(vv[c, HALO:HALO + 1, :], (HALO, 128))
    wait(x_copy(3))
    run(project(xb7, sb, wv7, vv, k1), wo_finish(), attn_mix(0, oa7, soa, 0, 160, 4), lead=0, lag=9)
    run(project(xf7, sf, wq7, qa, 0), attn_mix(0, oa7, soa, 160, T, 4), attn_scores(qb, T, None, 0, 192, 4),
        lead=0, lag=9)
    wait(w1_copy)
    run(project(xf7, sf, wv7, vv, k2), attn_scores(qb, T, None, 192, T, 4), attn_mix(T, ob7, sob, 0, 128, 4),
        ffn_prepare(w1_raw, w17, 0, 4), lead=0)
    run(attn_out(0, oa7, soa), attn_mix(T, ob7, sob, 128, T, 4), ffn_prepare(w1_raw, w17, 4, 6), lead=0)
    run(attn_out(1, ob7, sob), _mix(layernorm(0, xf7, sf), ffn_prepare(w1_raw, w17, 6, 8)), lead=0, lag=2)
    run(ffn_up(0, 6), ffn_prepare(w1_raw, w17, 8, NF // 2), attn_scores(qa, 2 * T, None, 0, T, 8),
        attn_mix(2 * T, oa7, soa, 0, 192, 8), lead=0, lag=9)
    move_halo(kk, 3 * T, T)
    wait(w2_copy)
    run(ffn_up(6, UP_SPLIT), attn_mix(2 * T, oa7, soa, 192, T, 8), layernorm(3, xa7, sa),
        ffn_prepare(w2_raw, w27, 0, 2, 16), lead=0)
    move_halo(vv, 3 * T, T)
    run(attn_out(2, oa7, soa), ffn_prepare(w2_raw, w27, 2, NC // 2, 16), lead=0, lag=9)

    sched.barrier()
    tuning[:] = 1024, 1

    def step(i, _):
        t_attn = (i + SKEW) % NT
        first = (t_attn == 0).astype(jnp.int32)

        @pl.when(i + SKEW + 1 < NT)
        def _():
            x_copy(i + SKEW + 1).wait()

        move_halo(kk, T, 0)
        move_halo(vv, T, 0)
        solo(ffn_up(UP_SPLIT))
        run(_chain(project(xa7, sa, wq7, qa, 0), project(xa7, sa, wk7, kk, k0)),
            layernorm((i + 1) % NT, xf7, sf), ffn_mid(), lag=2)
        run(project(xa7, sa, wv7, vv, k0), attn_scores(qa, 0, first, 0, 112, 8), lead=0, lag=2)
        for c in range(NC):
            v0 = jnp.broadcast_to(vv[c, HALO:HALO + 1, :], (HALO, 128))
            vv[c, 0:HALO, :] = jnp.where(t_attn == 0, v0, vv[c, 0:HALO, :])
        run(ffn_down(i % NT), attn_scores(qa, 0, first, 112, T, 4), attn_mix(0, oa7, soa, 0, T, 4), lag=2)
        solo(attn_out(t_attn, oa7, soa))
        run(ffn_up(0, UP_SPLIT), layernorm((i + SKEW + 1) % NT, xa7, sa), lead=4)
        sched.barrier()

        @pl.when(i >= NT)
        def _():
            o_copy(i - NT).start()
        return 0

    lax.fori_loop(0, 2 * NT - SKEW, step, 0)

    down_a, down_b = ffn_down(NT - 3), ffn_down(NT - 2, hb7, sob)
    solo(ffn_up(UP_SPLIT), ffn_mid())
    run(_take(down_a, 2), layernorm(NT - 2, xf7, sf), lead=0)
    run(ffn_up(), layernorm(NT - 1, xa7, sa), lead=6)
    run(_chain(_take(down_a, 2), _take(down_b, 1)), ffn_mid(hb7, sob), lead=2)
    solo(ffn_up(a7=xa7, s_ref=sa))
    run(_take(down_b, 3), ffn_mid(), lead=0)
    sched.barrier()
    o_copy(NT - 3).start()
    o_copy(NT - 2).start()
    down_c = ffn_down(NT - 1)
    last = []
    for j in range(NC // 2):
        solo(_take(down_c, 1))
        for c in (j, NC // 2 + j):
            at = (pl.ds((NT - 1) * T, T), pl.ds(c * 128, 128))
            last.append(pltpu.make_async_copy(xb.at[at], o_hbm.at[at], sem_o.at[NT - 1 + c]))
            last[-1].start()
    for copy in [o_copy(t) for t in range(NT - 1)] + last:
        copy.wait()


def _scratch_shapes():
    vmem = pltpu.VMEM
    lhs = vmem((7, T // 4, D // 2), u32)
    square = vmem((7, D // 4, D // 2), u32)
    per_row = vmem((T, 128), f32)
    chunks = vmem((NC, T, 128), f32)
    window = vmem((NC, HALO + 3 * T, 128), f32)
    return [
        vmem((S, D), bf16),
        vmem((3, D, D), bf16), vmem((D, D), bf16),
        vmem((D, F), bf16), vmem((F, D), bf16),
        vmem((NC, D // 2, 128), u32),
        vmem((NC, PAD * D // 64, 128), u32),
        square, square, square, square,
        vmem((7, D // 4, F // 2), u32), vmem((7, F // 4, D // 2), u32),
        vmem((40, 128), f32),
        lhs, lhs, lhs, lhs, lhs,
        vmem((7, T // 4, F // 2), u32), vmem((7, T // 4, F // 2), u32),
        per_row, per_row, per_row, per_row, per_row, per_row,
        chunks, per_row, vmem((NF, T, 128), f32), per_row, per_row,
        chunks, chunks, window, window, vmem((W, T, 128), f32),
        vmem((8, 128), u32),
        pltpu.SemaphoreType.DMA((NT,)), pltpu.SemaphoreType.DMA((7,)), pltpu.SemaphoreType.DMA((NT + NC,)),
    ]


@jax.jit
def pallas_interleave_layers__sliding_local_dilated__dense_activation_squared_relu__prompt_kernel(
    A_x: jax.Array,
    A_wqkv: jax.Array,
    A_wo: jax.Array,
    B_x: jax.Array,
    B_w1: jax.Array,
    B_b1: jax.Array,
    B_w2: jax.Array,
    B_b2: jax.Array,
):
    del B_x
    hbm = pl.BlockSpec(memory_space=pl.ANY)
    vmem = pl.BlockSpec(memory_space=pltpu.VMEM)
    out = pl.pallas_call(
        _kernel,
        in_specs=[hbm, hbm, hbm, hbm, vmem, hbm, vmem],
        out_specs=hbm,
        out_shape=jax.ShapeDtypeStruct((S, D), bf16),
        scratch_shapes=_scratch_shapes(),
        compiler_params=pltpu.CompilerParams(vmem_limit_bytes=110 * 2 ** 20),
    )(A_x.reshape(S, D), A_wqkv, A_wo, B_w1, B_b1.reshape(NF, 128), B_w2, B_b2.reshape(NC, 128))
    return out.reshape(1, S, D)
```

```python
import jax
import jax.numpy as jnp
from jax import lax
from jax.experimental import pallas as pl
from jax.experimental.pallas import tpu as pltpu

S, D, F = 2048, 1024, 3584
DH, W, DIL = 32, 8, 2
EPS = 1e-5
SCALE = DH ** -0.5
MASKED = -1e9
LOG2E = 1.4426950408889634
TINY = 1e-36

T = 256
TH = T // 2
NT = S // T
HALO = 16
NC = D // 128
NF = F // 128
SKEW = 3
UP_SPLIT = 13
PAD = DH + 1

f32 = jnp.float32
bf16 = jnp.bfloat16
u32 = jnp.uint32


def _pack_rows(x):
    return pltpu.bitcast(x.astype(bf16), u32)


def _as_bf16(u):
    return pltpu.bitcast(u, bf16)


class _Phase:
    def __init__(self, n, gen):
        self.n, self.gen = n, gen


def _chain(*phases):
    def gen():
        for p in phases:
            yield from p.gen
    return _Phase(sum(p.n for p in phases), gen())


def _take(phase, n):
    return _Phase(n, (next(phase.gen) for _ in range(n)))


def _mix(a, b):
    def gen():
        done = 0
        for i in range(a.n):
            yield next(a.gen)
            while done < (i + 1) * b.n // a.n:
                yield next(b.gen)
                done += 1
    return _Phase(a.n + b.n, gen())


class _Schedule:
    def __init__(self, zero_ref):
        self.zero_ref = zero_ref
        self.results = []
        self.token = None
        self.due = None
        self.carry = {}
        self.lag = 3

    def gate(self, *xs):
        if self.token is None:
            return list(xs)
        zero = pltpu.bitcast(self.token, u32) & self.zero_ref[...]
        out = []
        for x in xs:
            u = pltpu.bitcast(x, u32)
            out.append(pltpu.bitcast(u | jnp.tile(zero, (u.shape[0] // 8, u.shape[1] // 128)), x.dtype))
        return out

    def hold(self, lhs):
        if self.due is None:
            return lhs
        n = min(lhs.shape[1], 512)
        head = [lhs[:8, c:c + 128] | self.due for c in range(0, n, 128)]
        if lhs.shape[1] > n:
            head.append(lhs[:8, n:])
        self.due = None
        return jnp.concatenate([jnp.concatenate(head, axis=1), lhs[8:]], axis=0)

    def run(self, main, *side, lead=1, lag=None):
        lag = self.lag if lag is None else lag
        side = _chain(*side)
        slots = max(main.n - lead, 1)
        dues, done = dict(self.carry), 0
        self.carry = {}
        for i in range(main.n):
            self.results = []
            self.due = dues.pop(i, None)
            next(main.gen)
            tokens = [(y, r) for y in self.results for r in range(0, y.shape[0], 8)]
            want = min(side.n, -(-side.n * (i + 1) // slots))
            finished = None
            for j in range(want - done):
                y, r = tokens[j * len(tokens) // (want - done)]
                self.token = y[r:r + 8]
                last = next(side.gen)
                if last is not None:
                    last = pltpu.bitcast(last, u32)[:8, :128]
                    finished = last if finished is None else finished & last
            if finished is not None:
                dues[i + lag] = finished & self.zero_ref[...]
            done = want
        self.token = self.due = None
        self.carry = {i - main.n: z for i, z in dues.items()}
        for p in (main, side):
            assert next(p.gen, _Schedule) is _Schedule, "wrong piece count"

    def solo(self, *phases):
        self.due = self.carry.pop(0, None)
        self.carry = {}
        for p in phases:
            for _ in p.gen:
                pass
        self.due = None

    def barrier(self):
        self.carry = {}


def _kernel(x_hbm, wqkv_hbm, wo_hbm, w1_hbm, b1_hbm, w2_hbm, b2_hbm, o_hbm,
            xb, wqkv_raw, wo_raw, w1_raw, w2_raw, b1_raw, b2_raw, w_tmp, wo_tmp,
            wq7, wk7, wv7, wo7, w17, w27, bias,
            xa7, xb7, xf7, oa7, ob7, ha7, hb7, sa, sb, sf, soa, sob, sh,
            stage, stage_inv, h_stage, h_inv, h_ss,
            qa, qb, kk, vv, pp, zero_ref, sem_x, sem_w, sem_o):
    def x_copy(t):
        return pltpu.make_async_copy(x_hbm.at[pl.ds(t * T, T)], xb.at[pl.ds(t * T, T)], sem_x.at[t])

    def o_copy(t):
        return pltpu.make_async_copy(xb.at[pl.ds(t * T, T)], o_hbm.at[pl.ds(t * T, T)], sem_o.at[t])

    def wq_copy(half):
        rows = pl.ds(half * (D // 2), D // 2)
        return pltpu.make_async_copy(wqkv_hbm.at[rows, pl.ds(0, D)], wqkv_raw.at[0, rows], sem_w.at[half])

    def wkv_copy(i):
        return pltpu.make_async_copy(wqkv_hbm.at[:, pl.ds(i * D, D)], wqkv_raw.at[i], sem_w.at[1 + i])

    wo_copy = pltpu.make_async_copy(wo_hbm, wo_raw, sem_w.at[4])
    w1_copy = pltpu.make_async_copy(w1_hbm, w1_raw, sem_w.at[5])
    w2_copy = pltpu.make_async_copy(w2_hbm, w2_raw, sem_w.at[6])
    b1_copy = pltpu.make_async_copy(b1_hbm, b1_raw, sem_w.at[7])
    b2_copy = pltpu.make_async_copy(b2_hbm, b2_raw, sem_w.at[8])

    for copy in (x_copy(0), wq_copy(0), wq_copy(1), x_copy(1), wkv_copy(1), x_copy(2), wkv_copy(2), wo_copy,
                 x_copy(3), b1_copy, b2_copy, w1_copy, w2_copy, *[x_copy(t) for t in range(4, NT)]):
        copy.start()

    zero_ref[...] = jnp.zeros((8, 128), u32)

    sched = _Schedule(zero_ref)
    tuning = [512, 0]
    gate, run, solo = sched.gate, sched.run, sched.solo

    def wait(copy):
        sched.barrier()
        copy.wait()

    def store_b7(dst, row, col, u11, u12, u21, u22):
        b11, b12, b21, b22 = ((_as_bf16(u) if u.dtype == u32 else u).astype(f32) for u in (u11, u12, u21, u22))
        at = (pl.ds(row, u11.shape[0]), pl.ds(col, u11.shape[1]))
        dst[(0,) + at] = _pack_rows(b11 + b22)
        dst[(1,) + at] = u11
        dst[(2,) + at] = _pack_rows(b12 - b22)
        dst[(3,) + at] = _pack_rows(b21 - b11)
        dst[(4,) + at] = u22
        dst[(5,) + at] = _pack_rows(b11 + b12)
        last = _pack_rows(b21 + b22)
        dst[(6,) + at] = last
        return last

    def a7_pieces(src, inv, dst):
        nk = src.shape[0] // 2
        for r in range(0, TH, 16):
            top, bot = inv[r:r + 16, :], inv[TH + r:TH + r + 16, :]
            for j in range(nk):
                top, bot = gate(top, bot)
                a11, a12, a21, a22 = (src[c, r0:r0 + 16, :] * scale
                                      for r0, scale in ((r, top), (TH + r, bot)) for c in (j, nk + j))
                at = (slice(r // 2, r // 2 + 8), slice(j * 128, (j + 1) * 128))
                dst[(0,) + at] = _pack_rows(a11 + a22)
                dst[(1,) + at] = _pack_rows(a21 + a22)
                dst[(2,) + at] = _pack_rows(a11)
                dst[(3,) + at] = _pack_rows(a22)
                dst[(4,) + at] = _pack_rows(a11 + a12)
                dst[(5,) + at] = _pack_rows(a21 - a11)
                last = _pack_rows(a12 - a22)
                dst[(6,) + at] = last
                yield last

    def matmul(a7, b7, emit, j0=0, j1=None):
        kh, nh = a7.shape[2], b7.shape[2] // 128
        k_step, order = tuning
        j1 = nh if j1 is None else j1

        def product(i, j):
            y = None
            for k in range(0, kh, k_step):
                ke = min(k + k_step, kh)
                yk = lax.dot_general(_as_bf16(sched.hold(a7[i, :, k:ke])),
                                     _as_bf16(b7[i, k // 2:ke // 2, j * 128:(j + 1) * 128]),
                                     (((1,), (0,)), ((), ())), preferred_element_type=f32)
                sched.results.append(yk)
                y = yk if y is None else y + yk
            return y

        def gen():
            for j in range(j0, j1):
                if order == 0:
                    m1, m2 = product(0, j), product(1, j)
                    c22 = m1 - m2
                    m4 = product(3, j)
                    emit(1, j, m2 + m4)
                    c11 = m1 + m4
                    c11 = c11 + product(6, j)
                    m5 = product(4, j)
                    emit(0, j, c11 - m5)
                    m3 = product(2, j)
                    emit(0, nh + j, m3 + m5)
                    c22 = c22 + m3
                    emit(1, nh + j, c22 + product(5, j))
                else:
                    m6, m2 = product(5, j), product(1, j)
                    c22 = m6 - m2
                    m3 = product(2, j)
                    c22 = c22 + m3
                    m1 = product(0, j)
                    emit(1, nh + j, c22 + m1)
                    m5 = product(4, j)
                    emit(0, nh + j, m3 + m5)
                    c11 = m1 - m5
                    m4 = product(3, j)
                    emit(1, j, m2 + m4)
                    c11 = c11 + m4
                    emit(0, j, c11 + product(6, j))
                yield
        return _Phase(j1 - j0, gen())

    def store_row_norm(ss, inv_ref, s_ref, r):
        ss = ss + TINY
        inv = lax.rsqrt(ss)
        shape = (ss.shape[0], 128)
        inv_ref[r:r + shape[0], :] = jnp.broadcast_to(inv, shape)
        norm = jnp.broadcast_to(ss * inv, shape)
        s_ref[r:r + shape[0], :] = norm
        return norm

    def qkv_skew(i, r0=0, r1=D):
        def gen(group=4):
            lane = lax.broadcasted_iota(jnp.int32, (8, 128), 1)
            bits = [(lane & (1 << b)) != 0 for b in range(3)]
            for g0 in range(r0 // 16, r1 // 16, group):
                xs = [[None] * NC for _ in range(group)]
                for c in range(NC):
                    for g in range(group):
                        rows = slice((g0 + g) * 16, (g0 + g + 1) * 16)
                        u, = gate(pltpu.bitcast(wqkv_raw[i, rows, c * 128:(c + 1) * 128], u32))
                        xs[g][c] = pltpu.roll(u, c, 1) if c else u
                for g in range(group):
                    ws = [xs[g][(-c) % NC] for c in range(NC)]
                    for b in range(3):
                        ws = [jnp.where(bits[b], ws[(c - (1 << b)) % NC], ws[c]) for c in range(NC)]
                    for c in range(NC):
                        w_tmp[c, (g0 + g) * 8:(g0 + g + 1) * 8, :] = ws[c]
                yield ws[0]
        return _Phase((r1 - r0) // 64, gen())

    def gather_lanes(c, r0):
        lane = lax.broadcasted_iota(jnp.int32, (64, 128), 1)
        base = (lane & 3) * 32 + (lane >> 5) * 8 + ((lane >> 2) & 7)
        for r in range(r0 // 2, r0 // 2 + D // 4, 64):
            u, = gate(w_tmp[c, r:r + 64, :])
            u = jnp.take_along_axis(u, (base + c) & 127, axis=1)
            w_tmp[c, r:r + 64, :] = u
        return u

    def qkv_finish(dst, j0, j1):
        def gen():
            for j in range(j0, j1):
                left, right = j, NC // 2 + j
                for c in (left, right):
                    gather_lanes(c, 0)
                    yield gather_lanes(c, D // 2)
                for r in range(0, D // 4, 16):
                    top, bot = slice(r, r + 16), slice(D // 4 + r, D // 4 + r + 16)
                    last = store_b7(dst, r, j * 128, w_tmp[left, top, :], w_tmp[right, top, :],
                                    w_tmp[left, bot, :], w_tmp[right, bot, :])
                yield last
        return _Phase(3 * (j1 - j0), gen())

    def wo_stage():
        def gen():
            for n in range(NC):
                for g in range(D // 64):
                    u, = gate(pltpu.bitcast(wo_raw[64 * g:64 * (g + 1), n * 128:(n + 1) * 128], u32))
                    wo_tmp[n, pl.ds(PAD * g, 32), :] = u
                    if g % 4 == 3:
                        yield u
        return _Phase(NC * 4, gen())

    def wo_finish():
        def rows16(n, cp, a):
            start = PAD * 8 * (a % 2) + 4 * (a // 2) + cp
            lo = wo_tmp[n, pl.ds(start, 8, stride=PAD), :]
            hi = wo_tmp[n, pl.ds(start + 16, 8, stride=PAD), :]
            return (lo & u32(0xFFFF)) | (hi << 16), (lo >> 16) | (hi & u32(0xFFFF0000))

        def gen():
            for j in range(NC // 2):
                for cp in range(NC // 4):
                    for a in range(8):
                        u11, u12 = rows16(j, cp, a), rows16(NC // 2 + j, cp, a)
                        u21, u22 = rows16(j, NC // 4 + cp, a), rows16(NC // 2 + j, NC // 4 + cp, a)
                        u11, u22 = gate(*u11), gate(*u22)
                        for odd in range(2):
                            last = store_b7(wo7, (2 * cp + odd) * 64 + 8 * a, j * 128,
                                            u11[odd], u12[odd], u21[odd], u22[odd])
                        if a % 2:
                            yield last
        return _Phase(NC * NC // 2, gen())

    def ffn_prepare(raw, dst, j0, j1, rows=32):
        kh, nh = raw.shape[0] // 2, raw.shape[1] // 2

        def gen():
            for c in range(j0 * 128, j1 * 128, 256):
                for r in range(0, kh, rows):
                    q = [raw[r0:r0 + rows, c0:c0 + 256] for r0 in (r, kh + r) for c0 in (c, nh + c)]
                    q[0], q[3] = gate(pltpu.bitcast(q[0], u32), pltpu.bitcast(q[3], u32))
                    yield store_b7(dst, r // 2, c, *q)
        return _Phase((j1 - j0) // 2 * kh // rows, gen())

    def layernorm(t, a7, s_ref):
        def gen():
            for r in range(0, T, 16):
                rows = pl.ds(pl.multiple_of(t * T + r, 16), 16)
                acc = None
                for c in range(NC):
                    x = xb[rows, c * 128:(c + 1) * 128]
                    if c == 0:
                        x, = gate(x)
                    acc = x.astype(f32) if acc is None else acc + x.astype(f32)
                mean = jnp.broadcast_to(jnp.sum(acc, axis=-1, keepdims=True) * (1.0 / D), (16, 128))
                yield mean
                mean, = gate(mean)
                acc = None
                for c in range(NC):
                    xc = xb[rows, c * 128:(c + 1) * 128].astype(f32) - mean
                    stage[c, r:r + 16, :] = xc
                    acc = xc * xc if acc is None else acc + xc * xc
                var = jnp.sum(acc, axis=-1, keepdims=True) * (1.0 / D)
                inv = lax.rsqrt(var + TINY)
                stage_inv[r:r + 16, :] = jnp.broadcast_to(inv, (16, 128))
                scale = jnp.broadcast_to((var + TINY) * inv * lax.rsqrt(var + EPS), (16, 128))
                s_ref[r:r + 16, :] = scale
                yield scale
            yield from a7_pieces(stage, stage_inv, a7)
        return _Phase(2 * T // 16 + TH // 16 * NC // 2, gen())

    def project(a7, s_ref, b7, dst, row0):
        def emit(half, c, y):
            dst[c, pl.ds(row0 + half * TH, TH), :] = y * s_ref[half * TH:(half + 1) * TH, :]
        return matmul(a7, b7, emit)

    def plain_lhs():
        for r in range(0, TH, 16):
            for j in range(NC // 2):
                at = (slice(r // 2, r // 2 + 8), slice(j * 128, (j + 1) * 128))
                ob7[(0,) + at] = _pack_rows(stage[NC // 2 + j, r:r + 16, :] * stage_inv[r:r + 16, :])
                ob7[(1,) + at] = _pack_rows(stage[j, TH + r:TH + r + 16, :] * stage_inv[TH + r:TH + r + 16, :])

    def first_q(k_half):
        def gen():
            blocks = (ob7[0], xa7[3]) if k_half else (xa7[2], ob7[1])
            for c in range(NC):
                lhs = jnp.concatenate([sched.hold(blocks[0]), blocks[1]], axis=0)
                rhs = w_tmp[c, k_half * (D // 4):(k_half + 1) * (D // 4), :]
                y = lax.dot_general(_as_bf16(lhs), _as_bf16(rhs), (((1,), (0,)), ((), ())),
                                    preferred_element_type=f32)
                sched.results.append(y)
                qa[c] = (qa[c] + y) * sa[...] if k_half else y
                yield
        return _Phase(NC, gen())

    def gather_bottom(c0, c1):
        return _Phase(c1 - c0, (gather_lanes(c, D // 2) for c in range(c0, c1)))

    def qkv_combine(dst):
        def gen():
            for j in range(NC // 2):
                for r in range(0, D // 4, 16):
                    q = [w_tmp[c, r0:r0 + 16, :] for r0 in (r, D // 4 + r) for c in (j, NC // 2 + j)]
                    q[0], q[3] = gate(q[0], q[3])
                    last = store_b7(dst, r, j * 128, *q)
                    if r % 64 == 48:
                        yield last
        return _Phase(NC * 2, gen())

    def attn_scores(q, row0, first, r0, r1, chunks):
        def gen():
            for r in range(r0, r1, 8):
                ls = [None] * W
                for c in range(NC):
                    qv, = gate(q[c, r:r + 8, :])
                    for w in range(W):
                        t = qv * kk[c, pl.ds(HALO + row0 + r - DIL * w, 8), :]
                        ls[w] = t if ls[w] is None else ls[w] + t
                    if c % chunks == chunks - 1 and c != NC - 1:
                        yield None
                for w in range(W):
                    t = ls[w] + pltpu.roll(ls[w], 64, 1)
                    t = t + pltpu.roll(t, 32, 1)
                    if first is not None and r < DIL * w:
                        row = lax.broadcasted_iota(jnp.int32, (8, 128), 0) + r
                        t = jnp.where(row < first * (DIL * w), MASKED / SCALE, t)
                    ls[w] = t
                m = ls[0]
                for w in range(1, W):
                    m = jnp.maximum(m, ls[w])
                es = [jnp.exp2((t - m) * (SCALE * LOG2E)) for t in ls]
                total = es[0]
                for w in range(1, W):
                    total = total + es[w]
                inv = 1.0 / total
                for w in range(W):
                    pp[w, r:r + 8, :] = es[w] * inv
                yield inv
        return _Phase((r1 - r0) // 8 * (NC // chunks), gen())

    def attn_mix(row0, o7, s_ref, r0, r1, chunks):
        def gen():
            for r in range(r0, r1, 8):
                ps = [pp[w, r:r + 8, :] for w in range(W)]
                ss = None
                for c in range(NC):
                    if c % chunks == 0:
                        ps = gate(*ps)
                    acc = None
                    for w in range(W):
                        t = ps[w] * vv[c, pl.ds(HALO + row0 + r - DIL * w, 8), :]
                        acc = t if acc is None else acc + t
                    stage[c, r:r + 8, :] = acc
                    ss = acc * acc if ss is None else ss + acc * acc
                    if c % chunks == chunks - 1 and c != NC - 1:
                        yield None
                yield store_row_norm(jnp.sum(ss, axis=-1, keepdims=True), stage_inv, s_ref, r)
            if r1 == T:
                yield from a7_pieces(stage, stage_inv, o7)
        return _Phase((r1 - r0) // 8 * (NC // chunks) + (TH // 16 * NC // 2 if r1 == T else 0), gen())

    def add_residual(t, a7, s_ref, b7, bias_row):
        def emit(half, c, y):
            rows = pl.ds(pl.multiple_of(t * T + half * TH, TH), TH)
            cols = slice(c * 128, (c + 1) * 128)
            z = y * s_ref[half * TH:(half + 1) * TH, :]
            if bias_row is not None:
                z = z + bias[bias_row + c:bias_row + c + 1, :]
            xb[rows, cols] = (xb[rows, cols].astype(f32) + z).astype(bf16)
        return matmul(a7, b7, emit)

    def attn_out(t, o7, s_ref):
        return add_residual(t, o7, s_ref, wo7, None)

    def ffn_up(j0=0, j1=NF // 2, a7=xf7, s_ref=sf):
        started = [j0 > 0, j0 > 0]

        def emit(half, c, y):
            rows = slice(half * TH, (half + 1) * TH)
            z = jnp.maximum(y * s_ref[rows, :] + bias[c:c + 1, :], 0.0)
            z = z * z
            h_stage[c, rows, :] = z
            h_ss[rows, :] = h_ss[rows, :] + z * z if started[half] else z * z
            started[half] = True
        return matmul(a7, w17, emit, j0, j1)

    def ffn_mid(h7=ha7, s_ref=sh):
        def gen():
            for r in range(0, T, 32):
                ss, = gate(h_ss[r:r + 32, :])
                yield store_row_norm(jnp.sum(ss, axis=-1, keepdims=True), h_inv, s_ref, r)
            yield from a7_pieces(h_stage, h_inv, h7)
        return _Phase(T // 32 + TH // 16 * NF // 2, gen())

    def ffn_down(t, h7=ha7, s_ref=sh):
        return add_residual(t, h7, s_ref, w27, 32)

    def move_halo(ref, src, dst):
        for c in range(NC):
            ref[c, pl.ds(dst, HALO), :] = ref[c, pl.ds(src, HALO), :]

    k0, k1, k2 = HALO, HALO + T, HALO + 2 * T
    wait(x_copy(0))
    solo(layernorm(0, xa7, sa))
    plain_lhs()
    wait(wq_copy(0))
    solo(qkv_skew(0, 0, D // 2))
    for c in range(NC):
        gather_lanes(c, 0)
    solo(first_q(0))
    wait(wq_copy(1))
    solo(qkv_skew(0, D // 2, D), gather_bottom(0, 2))
    wait(x_copy(1))
    run(first_q(1), _mix(layernorm(1, xb7, sb), _chain(gather_bottom(2, NC), qkv_combine(wq7))), lead=0, lag=9)
    q1 = project(xb7, sb, wq7, qb, 0)
    solo(_take(q1, 1))
    wait(wkv_copy(1))
    run(_chain(_take(q1, 3), project(xa7, sa, wk7, kk, k0)), qkv_skew(1), qkv_finish(wk7, 0, 4), lead=3, lag=2)
    for c in range(NC):
        kk[c, 0:HALO, :] = jnp.zeros((HALO, 128), f32)
    wait(x_copy(2))
    run(project(xb7, sb, wk7, kk, k1), layernorm(2, xf7, sf), attn_scores(qa, 0, 1, 0, 160, 4), lead=0, lag=9)
    wait(wkv_copy(2))
    run(project(xf7, sf, wk7, kk, k2), qkv_skew(2), qkv_finish(wv7, 0, 2))
    wait(wo_copy)
    run(project(xa7, sa, wv7, vv, k0), qkv_finish(wv7, 2, 4), attn_scores(qa, 0, 1, 160, T, 4), wo_stage(), lead=0)
    for c in range(NC):
        vv[c, 0:HALO, :] = jnp.broadcast_to(vv[c, HALO:HALO + 1, :], (HALO, 128))
    wait(x_copy(3))
    run(project(xb7, sb, wv7, vv, k1), wo_finish(), attn_mix(0, oa7, soa, 0, 160, 4), lead=0, lag=9)
    run(project(xf7, sf, wq7, qa, 0), attn_mix(0, oa7, soa, 160, T, 4), attn_scores(qb, T, None, 0, 192, 4),
        lead=0, lag=9)
    wait(b1_copy)
    wait(b2_copy)
    wait(w1_copy)
    bias[0:NF, :] = b1_raw[...].astype(f32)
    bias[32:32 + NC, :] = b2_raw[...].astype(f32)
    run(project(xf7, sf, wv7, vv, k2), attn_scores(qb, T, None, 192, T, 4), attn_mix(T, ob7, sob, 0, 128, 4),
        ffn_prepare(w1_raw, w17, 0, 4), lead=0)
    run(attn_out(0, oa7, soa), attn_mix(T, ob7, sob, 128, T, 4), ffn_prepare(w1_raw, w17, 4, 6), lead=0)
    run(attn_out(1, ob7, sob), _mix(layernorm(0, xf7, sf), ffn_prepare(w1_raw, w17, 6, 8)), lead=0, lag=2)
    run(ffn_up(0, 6), ffn_prepare(w1_raw, w17, 8, NF // 2), attn_scores(qa, 2 * T, None, 0, T, 8),
        attn_mix(2 * T, oa7, soa, 0, 192, 8), lead=0, lag=9)
    move_halo(kk, 3 * T, T)
    wait(w2_copy)
    run(ffn_up(6, UP_SPLIT), attn_mix(2 * T, oa7, soa, 192, T, 8), layernorm(3, xa7, sa),
        ffn_prepare(w2_raw, w27, 0, 2, 16), lead=0)
    move_halo(vv, 3 * T, T)
    run(attn_out(2, oa7, soa), ffn_prepare(w2_raw, w27, 2, NC // 2, 16), lead=0, lag=9)

    sched.barrier()
    tuning[:] = 1024, 1

    def step(i, _):
        t_attn = (i + SKEW) % NT
        first = (t_attn == 0).astype(jnp.int32)

        @pl.when(i + SKEW + 1 < NT)
        def _():
            x_copy(i + SKEW + 1).wait()

        move_halo(kk, T, 0)
        move_halo(vv, T, 0)
        solo(ffn_up(UP_SPLIT))
        run(_chain(project(xa7, sa, wq7, qa, 0), project(xa7, sa, wk7, kk, k0)),
            layernorm((i + 1) % NT, xf7, sf), ffn_mid(), lag=2)
        run(project(xa7, sa, wv7, vv, k0), attn_scores(qa, 0, first, 0, 112, 8), lead=0, lag=2)
        for c in range(NC):
            v0 = jnp.broadcast_to(vv[c, HALO:HALO + 1, :], (HALO, 128))
            vv[c, 0:HALO, :] = jnp.where(t_attn == 0, v0, vv[c, 0:HALO, :])
        run(ffn_down(i % NT), attn_scores(qa, 0, first, 112, T, 4), attn_mix(0, oa7, soa, 0, T, 4), lag=2)
        solo(attn_out(t_attn, oa7, soa))
        run(ffn_up(0, UP_SPLIT), layernorm((i + SKEW + 1) % NT, xa7, sa), lead=4)
        sched.barrier()

        @pl.when(i >= NT)
        def _():
            o_copy(i - NT).start()
        return 0

    lax.fori_loop(0, 2 * NT - SKEW, step, 0)

    down_a, down_b = ffn_down(NT - 3), ffn_down(NT - 2, hb7, sob)
    solo(ffn_up(UP_SPLIT), ffn_mid())
    run(_take(down_a, 2), layernorm(NT - 2, xf7, sf), lead=0)
    run(ffn_up(), layernorm(NT - 1, xa7, sa), lead=6)
    run(_chain(_take(down_a, 2), _take(down_b, 1)), ffn_mid(hb7, sob), lead=2)
    solo(ffn_up(a7=xa7, s_ref=sa))
    run(_take(down_b, 3), ffn_mid(), lead=0)
    sched.barrier()
    o_copy(NT - 3).start()
    o_copy(NT - 2).start()
    down_c = ffn_down(NT - 1)
    last = []
    for j in range(NC // 2):
        solo(_take(down_c, 1))
        for c in (j, NC // 2 + j):
            at = (pl.ds((NT - 1) * T, T), pl.ds(c * 128, 128))
            last.append(pltpu.make_async_copy(xb.at[at], o_hbm.at[at], sem_o.at[NT - 1 + c]))
            last[-1].start()
    for copy in [o_copy(t) for t in range(NT - 1)] + last:
        copy.wait()


def _scratch_shapes():
    vmem = pltpu.VMEM
    lhs = vmem((7, T // 4, D // 2), u32)
    square = vmem((7, D // 4, D // 2), u32)
    per_row = vmem((T, 128), f32)
    chunks = vmem((NC, T, 128), f32)
    window = vmem((NC, HALO + 3 * T, 128), f32)
    return [
        vmem((S, D), bf16),
        vmem((3, D, D), bf16), vmem((D, D), bf16),
        vmem((D, F), bf16), vmem((F, D), bf16),
        vmem((NF, 128), bf16), vmem((NC, 128), bf16),
        vmem((NC, D // 2, 128), u32),
        vmem((NC, PAD * D // 64, 128), u32),
        square, square, square, square,
        vmem((7, D // 4, F // 2), u32), vmem((7, F // 4, D // 2), u32),
        vmem((40, 128), f32),
        lhs, lhs, lhs, lhs, lhs,
        vmem((7, T // 4, F // 2), u32), vmem((7, T // 4, F // 2), u32),
        per_row, per_row, per_row, per_row, per_row, per_row,
        chunks, per_row, vmem((NF, T, 128), f32), per_row, per_row,
        chunks, chunks, window, window, vmem((W, T, 128), f32),
        vmem((8, 128), u32),
        pltpu.SemaphoreType.DMA((NT,)), pltpu.SemaphoreType.DMA((9,)), pltpu.SemaphoreType.DMA((NT + NC,)),
    ]


@jax.jit
def pallas_interleave_layers__sliding_local_dilated__dense_activation_squared_relu__prompt_kernel(
    A_x: jax.Array,
    A_wqkv: jax.Array,
    A_wo: jax.Array,
    B_x: jax.Array,
    B_w1: jax.Array,
    B_b1: jax.Array,
    B_w2: jax.Array,
    B_b2: jax.Array,
):
    del B_x
    hbm = pl.BlockSpec(memory_space=pl.ANY)
    out = pl.pallas_call(
        _kernel,
        in_specs=[hbm] * 7,
        out_specs=hbm,
        out_shape=jax.ShapeDtypeStruct((S, D), bf16),
        scratch_shapes=_scratch_shapes(),
        compiler_params=pltpu.CompilerParams(vmem_limit_bytes=110 * 2 ** 20),
    )(A_x.reshape(S, D), A_wqkv, A_wo, B_w1, B_b1.reshape(NF, 128), B_w2, B_b2.reshape(NC, 128))
    return out.reshape(1, S, D)
```

```python
import jax
import jax.numpy as jnp
from jax import lax
from jax.experimental import pallas as pl
from jax.experimental.pallas import tpu as pltpu

S, D, F = 2048, 1024, 3584
DH, W, DIL = 32, 8, 2
EPS = 1e-5
SCALE = DH ** -0.5
MASKED = -1e9
LOG2E = 1.4426950408889634
TINY = 1e-36

T = 256
TH = T // 2
NT = S // T
HALO = 16
NC = D // 128
NF = F // 128
SKEW = 3
UP_SPLIT = 13
PAD = DH + 1

f32 = jnp.float32
bf16 = jnp.bfloat16
u32 = jnp.uint32


def _pack_rows(x):
    return pltpu.bitcast(x.astype(bf16), u32)


def _as_bf16(u):
    return pltpu.bitcast(u, bf16)


class _Phase:
    def __init__(self, n, gen):
        self.n, self.gen = n, gen


def _chain(*phases):
    def gen():
        for p in phases:
            yield from p.gen
    return _Phase(sum(p.n for p in phases), gen())


def _take(phase, n):
    return _Phase(n, (next(phase.gen) for _ in range(n)))


def _mix(a, b):
    def gen():
        done = 0
        for i in range(a.n):
            yield next(a.gen)
            while done < (i + 1) * b.n // a.n:
                yield next(b.gen)
                done += 1
    return _Phase(a.n + b.n, gen())


class _Schedule:
    def __init__(self, zero_ref):
        self.zero_ref = zero_ref
        self.results = []
        self.token = None
        self.due = None
        self.carry = {}
        self.lag = 3

    def gate(self, *xs):
        if self.token is None:
            return list(xs)
        zero = pltpu.bitcast(self.token, u32) & self.zero_ref[...]
        out = []
        for x in xs:
            u = pltpu.bitcast(x, u32)
            out.append(pltpu.bitcast(u | jnp.tile(zero, (u.shape[0] // 8, u.shape[1] // 128)), x.dtype))
        return out

    def hold(self, lhs):
        if self.due is None:
            return lhs
        n = min(lhs.shape[1], 512)
        head = [lhs[:8, c:c + 128] | self.due for c in range(0, n, 128)]
        if lhs.shape[1] > n:
            head.append(lhs[:8, n:])
        self.due = None
        return jnp.concatenate([jnp.concatenate(head, axis=1), lhs[8:]], axis=0)

    def run(self, main, *side, lead=1, lag=None):
        lag = self.lag if lag is None else lag
        side = _chain(*side)
        slots = max(main.n - lead, 1)
        dues, done = dict(self.carry), 0
        self.carry = {}
        for i in range(main.n):
            self.results = []
            self.due = dues.pop(i, None)
            next(main.gen)
            tokens = [(y, r) for y in self.results for r in range(0, y.shape[0], 8)]
            want = min(side.n, -(-side.n * (i + 1) // slots))
            finished = None
            for j in range(want - done):
                y, r = tokens[j * len(tokens) // (want - done)]
                self.token = y[r:r + 8]
                last = next(side.gen)
                if last is not None:
                    last = pltpu.bitcast(last, u32)[:8, :128]
                    finished = last if finished is None else finished & last
            if finished is not None:
                dues[i + lag] = finished & self.zero_ref[...]
            done = want
        self.token = self.due = None
        self.carry = {i - main.n: z for i, z in dues.items()}
        for p in (main, side):
            assert next(p.gen, _Schedule) is _Schedule, "wrong piece count"

    def solo(self, *phases):
        self.due = self.carry.pop(0, None)
        self.carry = {}
        for p in phases:
            for _ in p.gen:
                pass
        self.due = None

    def barrier(self):
        self.carry = {}


def _kernel(x_hbm, wqkv_hbm, wo_hbm, w1_hbm, b1_hbm, w2_hbm, b2_hbm, o_hbm,
            xb, wqkv_raw, wo_raw, w1_raw, w2_raw, b1_raw, b2_raw, w_tmp, wo_tmp,
            wq7, wk7, wv7, wo7, w17, w27, bias,
            xa7, xb7, xf7, oa7, ob7, ha7, hb7, sa, sb, sf, soa, sob, sh,
            stage, stage_inv, h_stage, h_inv, h_ss,
            qa, qb, kk, vv, pp, zero_ref, sem_x, sem_w, sem_o):
    def x_copy(t):
        return pltpu.make_async_copy(x_hbm.at[pl.ds(t * T, T)], xb.at[pl.ds(t * T, T)], sem_x.at[t])

    def o_copy(t):
        return pltpu.make_async_copy(xb.at[pl.ds(t * T, T)], o_hbm.at[pl.ds(t * T, T)], sem_o.at[t])

    def wq_copy(half):
        rows = pl.ds(half * (D // 2), D // 2)
        return pltpu.make_async_copy(wqkv_hbm.at[rows, pl.ds(0, D)], wqkv_raw.at[0, rows], sem_w.at[half])

    def wkv_copy(i):
        return pltpu.make_async_copy(wqkv_hbm.at[:, pl.ds(i * D, D)], wqkv_raw.at[i], sem_w.at[1 + i])

    wo_copy = pltpu.make_async_copy(wo_hbm, wo_raw, sem_w.at[4])
    w1_copy = pltpu.make_async_copy(w1_hbm, w1_raw, sem_w.at[5])
    w2_copy = pltpu.make_async_copy(w2_hbm, w2_raw, sem_w.at[6])
    b1_copy = pltpu.make_async_copy(b1_hbm, b1_raw, sem_w.at[7])
    b2_copy = pltpu.make_async_copy(b2_hbm, b2_raw, sem_w.at[8])

    for copy in (x_copy(0), wq_copy(0), wq_copy(1), x_copy(1), wkv_copy(1), x_copy(2), wkv_copy(2), wo_copy,
                 x_copy(3), b1_copy, b2_copy, w1_copy, w2_copy, *[x_copy(t) for t in range(4, NT)]):
        copy.start()

    zero_ref[...] = jnp.zeros((8, 128), u32)

    sched = _Schedule(zero_ref)
    tuning = [512, 0]
    gate, run, solo = sched.gate, sched.run, sched.solo

    def wait(copy):
        sched.barrier()
        copy.wait()

    def store_b7(dst, row, col, u11, u12, u21, u22):
        b11, b12, b21, b22 = ((_as_bf16(u) if u.dtype == u32 else u).astype(f32) for u in (u11, u12, u21, u22))
        at = (pl.ds(row, u11.shape[0]), pl.ds(col, u11.shape[1]))
        dst[(0,) + at] = _pack_rows(b11 + b22)
        dst[(1,) + at] = u11
        dst[(2,) + at] = _pack_rows(b12 - b22)
        dst[(3,) + at] = _pack_rows(b21 - b11)
        dst[(4,) + at] = u22
        dst[(5,) + at] = _pack_rows(b11 + b12)
        last = _pack_rows(b21 + b22)
        dst[(6,) + at] = last
        return last

    def a7_pieces(src, inv, dst):
        nk = src.shape[0] // 2
        for r in range(0, TH, 16):
            top, bot = inv[r:r + 16, :], inv[TH + r:TH + r + 16, :]
            for j in range(nk):
                top, bot = gate(top, bot)
                a11, a12, a21, a22 = (src[c, r0:r0 + 16, :] * scale
                                      for r0, scale in ((r, top), (TH + r, bot)) for c in (j, nk + j))
                at = (slice(r // 2, r // 2 + 8), slice(j * 128, (j + 1) * 128))
                dst[(0,) + at] = _pack_rows(a11 + a22)
                dst[(1,) + at] = _pack_rows(a21 + a22)
                dst[(2,) + at] = _pack_rows(a11)
                dst[(3,) + at] = _pack_rows(a22)
                dst[(4,) + at] = _pack_rows(a11 + a12)
                dst[(5,) + at] = _pack_rows(a21 - a11)
                last = _pack_rows(a12 - a22)
                dst[(6,) + at] = last
                yield last

    def matmul(a7, b7, emit, j0=0, j1=None):
        kh, nh = a7.shape[2], b7.shape[2] // 128
        k_step, order = tuning
        j1 = nh if j1 is None else j1

        def product(i, j):
            y = None
            for k in range(0, kh, k_step):
                ke = min(k + k_step, kh)
                yk = lax.dot_general(_as_bf16(sched.hold(a7[i, :, k:ke])),
                                     _as_bf16(b7[i, k // 2:ke // 2, j * 128:(j + 1) * 128]),
                                     (((1,), (0,)), ((), ())), preferred_element_type=f32)
                sched.results.append(yk)
                y = yk if y is None else y + yk
            return y

        def gen():
            for j in range(j0, j1):
                if order == 0:
                    m1, m2 = product(0, j), product(1, j)
                    c22 = m1 - m2
                    m4 = product(3, j)
                    emit(1, j, m2 + m4)
                    c11 = m1 + m4
                    c11 = c11 + product(6, j)
                    m5 = product(4, j)
                    emit(0, j, c11 - m5)
                    m3 = product(2, j)
                    emit(0, nh + j, m3 + m5)
                    c22 = c22 + m3
                    emit(1, nh + j, c22 + product(5, j))
                else:
                    m6, m2 = product(5, j), product(1, j)
                    c22 = m6 - m2
                    m3 = product(2, j)
                    c22 = c22 + m3
                    m1 = product(0, j)
                    emit(1, nh + j, c22 + m1)
                    m5 = product(4, j)
                    emit(0, nh + j, m3 + m5)
                    c11 = m1 - m5
                    m4 = product(3, j)
                    emit(1, j, m2 + m4)
                    c11 = c11 + m4
                    emit(0, j, c11 + product(6, j))
                yield
        return _Phase(j1 - j0, gen())

    def store_row_norm(ss, inv_ref, s_ref, r):
        ss = ss + TINY
        inv = lax.rsqrt(ss)
        shape = (ss.shape[0], 128)
        inv_ref[r:r + shape[0], :] = jnp.broadcast_to(inv, shape)
        norm = jnp.broadcast_to(ss * inv, shape)
        s_ref[r:r + shape[0], :] = norm
        return norm

    def qkv_skew(i, r0=0, r1=D):
        def gen(group=4):
            lane = lax.broadcasted_iota(jnp.int32, (8, 128), 1)
            bits = [(lane & (1 << b)) != 0 for b in range(3)]
            for g0 in range(r0 // 16, r1 // 16, group):
                xs = [[None] * NC for _ in range(group)]
                for c in range(NC):
                    for g in range(group):
                        rows = slice((g0 + g) * 16, (g0 + g + 1) * 16)
                        u, = gate(pltpu.bitcast(wqkv_raw[i, rows, c * 128:(c + 1) * 128], u32))
                        xs[g][c] = pltpu.roll(u, c, 1) if c else u
                for g in range(group):
                    ws = [xs[g][(-c) % NC] for c in range(NC)]
                    for b in range(3):
                        ws = [jnp.where(bits[b], ws[(c - (1 << b)) % NC], ws[c]) for c in range(NC)]
                    for c in range(NC):
                        w_tmp[c, (g0 + g) * 8:(g0 + g + 1) * 8, :] = ws[c]
                yield ws[0]
        return _Phase((r1 - r0) // 64, gen())

    def gather_lanes(c, r0):
        lane = lax.broadcasted_iota(jnp.int32, (64, 128), 1)
        base = (lane & 3) * 32 + (lane >> 5) * 8 + ((lane >> 2) & 7)
        for r in range(r0 // 2, r0 // 2 + D // 4, 64):
            u, = gate(w_tmp[c, r:r + 64, :])
            u = jnp.take_along_axis(u, (base + c) & 127, axis=1)
            w_tmp[c, r:r + 64, :] = u
        return u

    def qkv_finish(dst, j0, j1):
        def gen():
            for j in range(j0, j1):
                left, right = j, NC // 2 + j
                for c in (left, right):
                    gather_lanes(c, 0)
                    yield gather_lanes(c, D // 2)
                for r in range(0, D // 4, 16):
                    top, bot = slice(r, r + 16), slice(D // 4 + r, D // 4 + r + 16)
                    last = store_b7(dst, r, j * 128, w_tmp[left, top, :], w_tmp[right, top, :],
                                    w_tmp[left, bot, :], w_tmp[right, bot, :])
                yield last
        return _Phase(3 * (j1 - j0), gen())

    def wo_stage():
        def gen():
            for n in range(NC):
                for g in range(D // 64):
                    u, = gate(pltpu.bitcast(wo_raw[64 * g:64 * (g + 1), n * 128:(n + 1) * 128], u32))
                    wo_tmp[n, pl.ds(PAD * g, 32), :] = u
                    if g % 4 == 3:
                        yield u
        return _Phase(NC * 4, gen())

    def wo_finish():
        def rows16(n, cp, a):
            start = PAD * 8 * (a % 2) + 4 * (a // 2) + cp
            lo = wo_tmp[n, pl.ds(start, 8, stride=PAD), :]
            hi = wo_tmp[n, pl.ds(start + 16, 8, stride=PAD), :]
            return (lo & u32(0xFFFF)) | (hi << 16), (lo >> 16) | (hi & u32(0xFFFF0000))

        def gen():
            for j in range(NC // 2):
                for cp in range(NC // 4):
                    for a in range(8):
                        u11, u12 = rows16(j, cp, a), rows16(NC // 2 + j, cp, a)
                        u21, u22 = rows16(j, NC // 4 + cp, a), rows16(NC // 2 + j, NC // 4 + cp, a)
                        u11, u22 = gate(*u11), gate(*u22)
                        for odd in range(2):
                            last = store_b7(wo7, (2 * cp + odd) * 64 + 8 * a, j * 128,
                                            u11[odd], u12[odd], u21[odd], u22[odd])
                        if a % 2:
                            yield last
        return _Phase(NC * NC // 2, gen())

    def ffn_prepare(raw, dst, j0, j1, rows=32):
        kh, nh = raw.shape[0] // 2, raw.shape[1] // 2

        def gen():
            for c in range(j0 * 128, j1 * 128, 256):
                for r in range(0, kh, rows):
                    q = [raw[r0:r0 + rows, c0:c0 + 256] for r0 in (r, kh + r) for c0 in (c, nh + c)]
                    q[0], q[3] = gate(pltpu.bitcast(q[0], u32), pltpu.bitcast(q[3], u32))
                    yield store_b7(dst, r // 2, c, *q)
        return _Phase((j1 - j0) // 2 * kh // rows, gen())

    def layernorm(t, a7, s_ref):
        def gen():
            for r in range(0, T, 16):
                rows = pl.ds(pl.multiple_of(t * T + r, 16), 16)
                acc = None
                for c in range(NC):
                    x = xb[rows, c * 128:(c + 1) * 128]
                    if c == 0:
                        x, = gate(x)
                    acc = x.astype(f32) if acc is None else acc + x.astype(f32)
                mean = jnp.broadcast_to(jnp.sum(acc, axis=-1, keepdims=True) * (1.0 / D), (16, 128))
                yield mean
                mean, = gate(mean)
                acc = None
                for c in range(NC):
                    xc = xb[rows, c * 128:(c + 1) * 128].astype(f32) - mean
                    stage[c, r:r + 16, :] = xc
                    acc = xc * xc if acc is None else acc + xc * xc
                var = jnp.sum(acc, axis=-1, keepdims=True) * (1.0 / D)
                inv = lax.rsqrt(var + TINY)
                stage_inv[r:r + 16, :] = jnp.broadcast_to(inv, (16, 128))
                scale = jnp.broadcast_to((var + TINY) * inv * lax.rsqrt(var + EPS), (16, 128))
                s_ref[r:r + 16, :] = scale
                yield scale
            yield from a7_pieces(stage, stage_inv, a7)
        return _Phase(2 * T // 16 + TH // 16 * NC // 2, gen())

    def project(a7, s_ref, b7, dst, row0):
        def emit(half, c, y):
            dst[c, pl.ds(row0 + half * TH, TH), :] = y * s_ref[half * TH:(half + 1) * TH, :]
        return matmul(a7, b7, emit)

    def plain_lhs():
        for r in range(0, TH, 16):
            for j in range(NC // 2):
                at = (slice(r // 2, r // 2 + 8), slice(j * 128, (j + 1) * 128))
                ob7[(0,) + at] = _pack_rows(stage[NC // 2 + j, r:r + 16, :] * stage_inv[r:r + 16, :])
                ob7[(1,) + at] = _pack_rows(stage[j, TH + r:TH + r + 16, :] * stage_inv[TH + r:TH + r + 16, :])

    def first_q(k_half):
        def gen():
            blocks = (ob7[0], xa7[3]) if k_half else (xa7[2], ob7[1])
            for c in range(NC):
                lhs = jnp.concatenate([sched.hold(blocks[0]), blocks[1]], axis=0)
                rhs = w_tmp[c, k_half * (D // 4):(k_half + 1) * (D // 4), :]
                y = lax.dot_general(_as_bf16(lhs), _as_bf16(rhs), (((1,), (0,)), ((), ())),
                                    preferred_element_type=f32)
                sched.results.append(y)
                qa[c] = (qa[c] + y) * sa[...] if k_half else y
                yield
        return _Phase(NC, gen())

    def gather_bottom(c0, c1):
        return _Phase(c1 - c0, (gather_lanes(c, D // 2) for c in range(c0, c1)))

    def qkv_combine(dst):
        def gen():
            for j in range(NC // 2):
                for r in range(0, D // 4, 16):
                    q = [w_tmp[c, r0:r0 + 16, :] for r0 in (r, D // 4 + r) for c in (j, NC // 2 + j)]
                    q[0], q[3] = gate(q[0], q[3])
                    last = store_b7(dst, r, j * 128, *q)
                    if r % 64 == 48:
                        yield last
        return _Phase(NC * 2, gen())

    def attn_scores(q, row0, first, r0, r1, chunks):
        def gen():
            for r in range(r0, r1, 8):
                ls = [None] * W
                for c in range(NC):
                    qv, = gate(q[c, r:r + 8, :])
                    for w in range(W):
                        t = qv * kk[c, pl.ds(HALO + row0 + r - DIL * w, 8), :]
                        ls[w] = t if ls[w] is None else ls[w] + t
                    if c % chunks == chunks - 1 and c != NC - 1:
                        yield None
                for w in range(W):
                    t = ls[w] + pltpu.roll(ls[w], 64, 1)
                    t = t + pltpu.roll(t, 32, 1)
                    if first is not None and r < DIL * w:
                        row = lax.broadcasted_iota(jnp.int32, (8, 128), 0) + r
                        t = jnp.where(row < first * (DIL * w), MASKED / SCALE, t)
                    ls[w] = t
                m = ls[0]
                for w in range(1, W):
                    m = jnp.maximum(m, ls[w])
                es = [jnp.exp2((t - m) * (SCALE * LOG2E)) for t in ls]
                total = es[0]
                for w in range(1, W):
                    total = total + es[w]
                inv = 1.0 / total
                for w in range(W):
                    pp[w, r:r + 8, :] = es[w] * inv
                yield inv
        return _Phase((r1 - r0) // 8 * (NC // chunks), gen())

    def attn_mix(row0, o7, s_ref, r0, r1, chunks):
        def gen():
            for r in range(r0, r1, 8):
                ps = [pp[w, r:r + 8, :] for w in range(W)]
                ss = None
                for c in range(NC):
                    if c % chunks == 0:
                        ps = gate(*ps)
                    acc = None
                    for w in range(W):
                        t = ps[w] * vv[c, pl.ds(HALO + row0 + r - DIL * w, 8), :]
                        acc = t if acc is None else acc + t
                    stage[c, r:r + 8, :] = acc
                    ss = acc * acc if ss is None else ss + acc * acc
                    if c % chunks == chunks - 1 and c != NC - 1:
                        yield None
                yield store_row_norm(jnp.sum(ss, axis=-1, keepdims=True), stage_inv, s_ref, r)
            if r1 == T:
                yield from a7_pieces(stage, stage_inv, o7)
        return _Phase((r1 - r0) // 8 * (NC // chunks) + (TH // 16 * NC // 2 if r1 == T else 0), gen())

    def add_residual(t, a7, s_ref, b7, bias_row):
        def emit(half, c, y):
            rows = pl.ds(pl.multiple_of(t * T + half * TH, TH), TH)
            cols = slice(c * 128, (c + 1) * 128)
            z = y * s_ref[half * TH:(half + 1) * TH, :]
            if bias_row is not None:
                z = z + bias[bias_row + c:bias_row + c + 1, :]
            xb[rows, cols] = (xb[rows, cols].astype(f32) + z).astype(bf16)
        return matmul(a7, b7, emit)

    def attn_out(t, o7, s_ref):
        return add_residual(t, o7, s_ref, wo7, None)

    def ffn_up(j0=0, j1=NF // 2, a7=xf7, s_ref=sf):
        started = [j0 > 0, j0 > 0]

        def emit(half, c, y):
            rows = slice(half * TH, (half + 1) * TH)
            z = jnp.maximum(y * s_ref[rows, :] + bias[c:c + 1, :], 0.0)
            z = z * z
            h_stage[c, rows, :] = z
            h_ss[rows, :] = h_ss[rows, :] + z * z if started[half] else z * z
            started[half] = True
        return matmul(a7, w17, emit, j0, j1)

    def ffn_mid(h7=ha7, s_ref=sh):
        def gen():
            for r in range(0, T, 32):
                ss, = gate(h_ss[r:r + 32, :])
                yield store_row_norm(jnp.sum(ss, axis=-1, keepdims=True), h_inv, s_ref, r)
            yield from a7_pieces(h_stage, h_inv, h7)
        return _Phase(T // 32 + TH // 16 * NF // 2, gen())

    def ffn_down(t, h7=ha7, s_ref=sh):
        return add_residual(t, h7, s_ref, w27, 32)

    def move_halo(ref, src, dst):
        for c in range(NC):
            ref[c, pl.ds(dst, HALO), :] = ref[c, pl.ds(src, HALO), :]

    k0, k1, k2 = HALO, HALO + T, HALO + 2 * T
    wait(x_copy(0))
    solo(layernorm(0, xa7, sa))
    plain_lhs()
    wait(wq_copy(0))
    solo(qkv_skew(0, 0, D // 2))
    for c in range(NC):
        gather_lanes(c, 0)
    solo(first_q(0))
    wait(wq_copy(1))
    solo(qkv_skew(0, D // 2, D), gather_bottom(0, 2))
    wait(x_copy(1))
    run(first_q(1), _mix(layernorm(1, xb7, sb), _chain(gather_bottom(2, NC), qkv_combine(wq7))), lead=0, lag=9)
    q1 = project(xb7, sb, wq7, qb, 0)
    solo(_take(q1, 1))
    wait(wkv_copy(1))
    run(_chain(_take(q1, 3), project(xa7, sa, wk7, kk, k0)), qkv_skew(1), qkv_finish(wk7, 0, 4), lead=3, lag=2)
    for c in range(NC):
        kk[c, 0:HALO, :] = jnp.zeros((HALO, 128), f32)
    wait(x_copy(2))
    run(project(xb7, sb, wk7, kk, k1), layernorm(2, xf7, sf), attn_scores(qa, 0, 1, 0, 160, 4), lead=0, lag=9)
    wait(wkv_copy(2))
    run(project(xf7, sf, wk7, kk, k2), qkv_skew(2), qkv_finish(wv7, 0, 2), lead=0)
    wait(wo_copy)
    run(project(xa7, sa, wv7, vv, k0), qkv_finish(wv7, 2, 4), attn_scores(qa, 0, 1, 160, T, 4), wo_stage(), lead=0)
    for c in range(NC):
        vv[c, 0:HALO, :] = jnp.broadcast_to(vv[c, HALO:HALO + 1, :], (HALO, 128))
    wait(x_copy(3))
    run(project(xb7, sb, wv7, vv, k1), wo_finish(), attn_mix(0, oa7, soa, 0, 160, 4), lead=0, lag=9)
    run(project(xf7, sf, wq7, qa, 0), attn_mix(0, oa7, soa, 160, T, 4), attn_scores(qb, T, None, 0, 192, 4),
        lead=0, lag=9)
    wait(b1_copy)
    wait(b2_copy)
    wait(w1_copy)
    bias[0:NF, :] = b1_raw[...].astype(f32)
    bias[32:32 + NC, :] = b2_raw[...].astype(f32)
    run(project(xf7, sf, wv7, vv, k2), attn_scores(qb, T, None, 192, T, 4), attn_mix(T, ob7, sob, 0, 64, 4),
        ffn_prepare(w1_raw, w17, 0, 4, 16), lead=0)
    run(attn_out(0, oa7, soa), attn_mix(T, ob7, sob, 64, T, 4), ffn_prepare(w1_raw, w17, 4, 6, 16), lead=0)
    run(attn_out(1, ob7, sob), _mix(layernorm(0, xf7, sf), ffn_prepare(w1_raw, w17, 6, 8)), lead=0, lag=2)
    run(ffn_up(0, 6), ffn_prepare(w1_raw, w17, 8, NF // 2), attn_scores(qa, 2 * T, None, 0, T, 4),
        attn_mix(2 * T, oa7, soa, 0, 224, 8), lead=0, lag=9)
    move_halo(kk, 3 * T, T)
    wait(w2_copy)
    run(ffn_up(6, UP_SPLIT), attn_mix(2 * T, oa7, soa, 224, T, 8), layernorm(3, xa7, sa),
        ffn_prepare(w2_raw, w27, 0, 2, 16), lead=0)
    move_halo(vv, 3 * T, T)
    run(attn_out(2, oa7, soa), ffn_prepare(w2_raw, w27, 2, NC // 2, 16), lead=0)

    sched.barrier()
    tuning[:] = 1024, 1

    def step(i, _):
        t_attn = (i + SKEW) % NT
        first = (t_attn == 0).astype(jnp.int32)

        @pl.when(i + SKEW + 1 < NT)
        def _():
            x_copy(i + SKEW + 1).wait()

        move_halo(kk, T, 0)
        move_halo(vv, T, 0)
        solo(ffn_up(UP_SPLIT))
        run(_chain(project(xa7, sa, wq7, qa, 0), project(xa7, sa, wk7, kk, k0)),
            layernorm((i + 1) % NT, xf7, sf), ffn_mid(), lag=2)
        run(project(xa7, sa, wv7, vv, k0), attn_scores(qa, 0, first, 0, 112, 8), lead=0, lag=2)
        for c in range(NC):
            v0 = jnp.broadcast_to(vv[c, HALO:HALO + 1, :], (HALO, 128))
            vv[c, 0:HALO, :] = jnp.where(t_attn == 0, v0, vv[c, 0:HALO, :])
        run(ffn_down(i % NT), attn_scores(qa, 0, first, 112, T, 4), attn_mix(0, oa7, soa, 0, T, 4), lag=2)
        solo(attn_out(t_attn, oa7, soa))
        run(ffn_up(0, UP_SPLIT), layernorm((i + SKEW + 1) % NT, xa7, sa), lead=4)
        sched.barrier()

        @pl.when(i >= NT)
        def _():
            o_copy(i - NT).start()
        return 0

    lax.fori_loop(0, 2 * NT - SKEW, step, 0)

    down_a, down_b = ffn_down(NT - 3), ffn_down(NT - 2, hb7, sob)
    solo(ffn_up(UP_SPLIT), ffn_mid())
    run(_take(down_a, 2), layernorm(NT - 2, xf7, sf), lead=0)
    run(ffn_up(), layernorm(NT - 1, xa7, sa), lead=6)
    run(_chain(_take(down_a, 2), _take(down_b, 1)), ffn_mid(hb7, sob), lead=2)
    solo(ffn_up(a7=xa7, s_ref=sa))
    run(_take(down_b, 3), ffn_mid(), lead=0)
    sched.barrier()
    o_copy(NT - 3).start()
    o_copy(NT - 2).start()
    down_c = ffn_down(NT - 1)
    last = []
    for j in range(NC // 2):
        solo(_take(down_c, 1))
        for c in (j, NC // 2 + j):
            at = (pl.ds((NT - 1) * T, T), pl.ds(c * 128, 128))
            last.append(pltpu.make_async_copy(xb.at[at], o_hbm.at[at], sem_o.at[NT - 1 + c]))
            last[-1].start()
    for copy in [o_copy(t) for t in range(NT - 1)] + last:
        copy.wait()


def _scratch_shapes():
    vmem = pltpu.VMEM
    lhs = vmem((7, T // 4, D // 2), u32)
    square = vmem((7, D // 4, D // 2), u32)
    per_row = vmem((T, 128), f32)
    chunks = vmem((NC, T, 128), f32)
    window = vmem((NC, HALO + 3 * T, 128), f32)
    return [
        vmem((S, D), bf16),
        vmem((3, D, D), bf16), vmem((D, D), bf16),
        vmem((D, F), bf16), vmem((F, D), bf16),
        vmem((NF, 128), bf16), vmem((NC, 128), bf16),
        vmem((NC, D // 2, 128), u32),
        vmem((NC, PAD * D // 64, 128), u32),
        square, square, square, square,
        vmem((7, D // 4, F // 2), u32), vmem((7, F // 4, D // 2), u32),
        vmem((40, 128), f32),
        lhs, lhs, lhs, lhs, lhs,
        vmem((7, T // 4, F // 2), u32), vmem((7, T // 4, F // 2), u32),
        per_row, per_row, per_row, per_row, per_row, per_row,
        chunks, per_row, vmem((NF, T, 128), f32), per_row, per_row,
        chunks, chunks, window, window, vmem((W, T, 128), f32),
        vmem((8, 128), u32),
        pltpu.SemaphoreType.DMA((NT,)), pltpu.SemaphoreType.DMA((9,)), pltpu.SemaphoreType.DMA((NT + NC,)),
    ]


@jax.jit
def pallas_interleave_layers__sliding_local_dilated__dense_activation_squared_relu__prompt_kernel(
    A_x: jax.Array,
    A_wqkv: jax.Array,
    A_wo: jax.Array,
    B_x: jax.Array,
    B_w1: jax.Array,
    B_b1: jax.Array,
    B_w2: jax.Array,
    B_b2: jax.Array,
):
    del B_x
    hbm = pl.BlockSpec(memory_space=pl.ANY)
    out = pl.pallas_call(
        _kernel,
        in_specs=[hbm] * 7,
        out_specs=hbm,
        out_shape=jax.ShapeDtypeStruct((S, D), bf16),
        scratch_shapes=_scratch_shapes(),
        compiler_params=pltpu.CompilerParams(vmem_limit_bytes=110 * 2 ** 20),
    )(A_x.reshape(S, D), A_wqkv, A_wo, B_w1, B_b1.reshape(NF, 128), B_w2, B_b2.reshape(NC, 128))
    return out.reshape(1, S, D)
```

```python
import jax
import jax.numpy as jnp
from jax import lax
from jax.experimental import pallas as pl
from jax.experimental.pallas import tpu as pltpu

S, D, F = 2048, 1024, 3584
DH, W, DIL = 32, 8, 2
EPS = 1e-5
SCALE = DH ** -0.5
MASKED = -1e9
LOG2E = 1.4426950408889634
TINY = 1e-36

T = 256
TH = T // 2
NT = S // T
HALO = 16
NC = D // 128
NF = F // 128
SKEW = 3
UP_SPLIT = 13
PAD = DH + 1

f32 = jnp.float32
bf16 = jnp.bfloat16
u32 = jnp.uint32


def _pack_rows(x):
    return pltpu.bitcast(x.astype(bf16), u32)


def _as_bf16(u):
    return pltpu.bitcast(u, bf16)


class _Phase:
    def __init__(self, n, gen):
        self.n, self.gen = n, gen


def _chain(*phases):
    def gen():
        for p in phases:
            yield from p.gen
    return _Phase(sum(p.n for p in phases), gen())


def _take(phase, n):
    return _Phase(n, (next(phase.gen) for _ in range(n)))


def _mix(a, b):
    def gen():
        done = 0
        for i in range(a.n):
            yield next(a.gen)
            while done < (i + 1) * b.n // a.n:
                yield next(b.gen)
                done += 1
    return _Phase(a.n + b.n, gen())


class _Schedule:
    def __init__(self, zero_ref):
        self.zero_ref = zero_ref
        self.results = []
        self.token = None
        self.due = None
        self.carry = {}
        self.lag = 3

    def gate(self, *xs):
        if self.token is None:
            return list(xs)
        zero = pltpu.bitcast(self.token, u32) & self.zero_ref[...]
        out = []
        for x in xs:
            u = pltpu.bitcast(x, u32)
            out.append(pltpu.bitcast(u | jnp.tile(zero, (u.shape[0] // 8, u.shape[1] // 128)), x.dtype))
        return out

    def hold(self, lhs):
        if self.due is None:
            return lhs
        n = min(lhs.shape[1], 512)
        head = [lhs[:8, c:c + 128] | self.due for c in range(0, n, 128)]
        if lhs.shape[1] > n:
            head.append(lhs[:8, n:])
        self.due = None
        return jnp.concatenate([jnp.concatenate(head, axis=1), lhs[8:]], axis=0)

    def run(self, main, *side, lead=1, lag=None):
        lag = self.lag if lag is None else lag
        side = _chain(*side)
        slots = max(main.n - lead, 1)
        dues, done = dict(self.carry), 0
        self.carry = {}
        for i in range(main.n):
            self.results = []
            self.due = dues.pop(i, None)
            next(main.gen)
            tokens = [(y, r) for y in self.results for r in range(0, y.shape[0], 8)]
            want = min(side.n, -(-side.n * (i + 1) // slots))
            finished = None
            for j in range(want - done):
                y, r = tokens[j * len(tokens) // (want - done)]
                self.token = y[r:r + 8]
                last = next(side.gen)
                if last is not None:
                    last = pltpu.bitcast(last, u32)[:8, :128]
                    finished = last if finished is None else finished & last
            if finished is not None:
                dues[i + lag] = finished & self.zero_ref[...]
            done = want
        self.token = self.due = None
        self.carry = {i - main.n: z for i, z in dues.items()}
        for p in (main, side):
            assert next(p.gen, _Schedule) is _Schedule, "wrong piece count"

    def solo(self, *phases):
        self.due = self.carry.pop(0, None)
        self.carry = {}
        for p in phases:
            for _ in p.gen:
                pass
        self.due = None

    def barrier(self):
        self.carry = {}


def _kernel(x_hbm, wqkv_hbm, wo_hbm, w1_hbm, b1_hbm, w2_hbm, b2_hbm, o_hbm,
            xb, wqkv_raw, wo_raw, w1_raw, w2_raw, b1_raw, b2_raw, w_tmp, wo_tmp,
            wq7, wk7, wv7, wo7, w17, w27, bias,
            xa7, xb7, xf7, oa7, ob7, ha7, hb7, sa, sb, sf, soa, sob, sh,
            stage, stage_inv, h_stage, h_inv, h_ss,
            qa, qb, kk, vv, pp, zero_ref, sem_x, sem_w, sem_o):
    def x_copy(t):
        return pltpu.make_async_copy(x_hbm.at[pl.ds(t * T, T)], xb.at[pl.ds(t * T, T)], sem_x.at[t])

    def o_copy(t):
        return pltpu.make_async_copy(xb.at[pl.ds(t * T, T)], o_hbm.at[pl.ds(t * T, T)], sem_o.at[t])

    def wq_copy(half):
        rows = pl.ds(half * (D // 2), D // 2)
        return pltpu.make_async_copy(wqkv_hbm.at[rows, pl.ds(0, D)], wqkv_raw.at[0, rows], sem_w.at[half])

    def wkv_copy(i):
        return pltpu.make_async_copy(wqkv_hbm.at[:, pl.ds(i * D, D)], wqkv_raw.at[i], sem_w.at[1 + i])

    wo_copy = pltpu.make_async_copy(wo_hbm, wo_raw, sem_w.at[4])
    w1_copy = pltpu.make_async_copy(w1_hbm, w1_raw, sem_w.at[5])
    w2_copy = pltpu.make_async_copy(w2_hbm, w2_raw, sem_w.at[6])
    b1_copy = pltpu.make_async_copy(b1_hbm, b1_raw, sem_w.at[7])
    b2_copy = pltpu.make_async_copy(b2_hbm, b2_raw, sem_w.at[8])

    for copy in (x_copy(0), wq_copy(0), wq_copy(1), x_copy(1), wkv_copy(1), x_copy(2), wkv_copy(2), wo_copy,
                 x_copy(3), b1_copy, b2_copy, w1_copy, w2_copy, *[x_copy(t) for t in range(4, NT)]):
        copy.start()

    zero_ref[...] = jnp.zeros((8, 128), u32)

    sched = _Schedule(zero_ref)
    tuning = [512, 0]
    gate, run, solo = sched.gate, sched.run, sched.solo

    def wait(copy):
        sched.barrier()
        copy.wait()

    def store_b7(dst, row, col, u11, u12, u21, u22):
        b11, b12, b21, b22 = ((_as_bf16(u) if u.dtype == u32 else u).astype(f32) for u in (u11, u12, u21, u22))
        at = (pl.ds(row, u11.shape[0]), pl.ds(col, u11.shape[1]))
        dst[(0,) + at] = _pack_rows(b11 + b22)
        dst[(1,) + at] = u11
        dst[(2,) + at] = _pack_rows(b12 - b22)
        dst[(3,) + at] = _pack_rows(b21 - b11)
        dst[(4,) + at] = u22
        dst[(5,) + at] = _pack_rows(b11 + b12)
        last = _pack_rows(b21 + b22)
        dst[(6,) + at] = last
        return last

    def a7_pieces(src, inv, dst):
        nk = src.shape[0] // 2
        for r in range(0, TH, 16):
            top, bot = inv[r:r + 16, :], inv[TH + r:TH + r + 16, :]
            for j in range(nk):
                top, bot = gate(top, bot)
                a11, a12, a21, a22 = (src[c, r0:r0 + 16, :] * scale
                                      for r0, scale in ((r, top), (TH + r, bot)) for c in (j, nk + j))
                at = (slice(r // 2, r // 2 + 8), slice(j * 128, (j + 1) * 128))
                dst[(0,) + at] = _pack_rows(a11 + a22)
                dst[(1,) + at] = _pack_rows(a21 + a22)
                dst[(2,) + at] = _pack_rows(a11)
                dst[(3,) + at] = _pack_rows(a22)
                dst[(4,) + at] = _pack_rows(a11 + a12)
                dst[(5,) + at] = _pack_rows(a21 - a11)
                last = _pack_rows(a12 - a22)
                dst[(6,) + at] = last
                yield last

    def matmul(a7, b7, emit, j0=0, j1=None):
        kh, nh = a7.shape[2], b7.shape[2] // 128
        k_step, order = tuning
        j1 = nh if j1 is None else j1

        def product(i, j):
            y = None
            for k in range(0, kh, k_step):
                ke = min(k + k_step, kh)
                yk = lax.dot_general(_as_bf16(sched.hold(a7[i, :, k:ke])),
                                     _as_bf16(b7[i, k // 2:ke // 2, j * 128:(j + 1) * 128]),
                                     (((1,), (0,)), ((), ())), preferred_element_type=f32)
                sched.results.append(yk)
                y = yk if y is None else y + yk
            return y

        def gen():
            for j in range(j0, j1):
                if order == 0:
                    m1, m2 = product(0, j), product(1, j)
                    c22 = m1 - m2
                    m4 = product(3, j)
                    emit(1, j, m2 + m4)
                    c11 = m1 + m4
                    c11 = c11 + product(6, j)
                    m5 = product(4, j)
                    emit(0, j, c11 - m5)
                    m3 = product(2, j)
                    emit(0, nh + j, m3 + m5)
                    c22 = c22 + m3
                    emit(1, nh + j, c22 + product(5, j))
                else:
                    m6, m2 = product(5, j), product(1, j)
                    c22 = m6 - m2
                    m3 = product(2, j)
                    c22 = c22 + m3
                    m1 = product(0, j)
                    emit(1, nh + j, c22 + m1)
                    m5 = product(4, j)
                    emit(0, nh + j, m3 + m5)
                    c11 = m1 - m5
                    m4 = product(3, j)
                    emit(1, j, m2 + m4)
                    c11 = c11 + m4
                    emit(0, j, c11 + product(6, j))
                yield
        return _Phase(j1 - j0, gen())

    def store_row_norm(ss, inv_ref, s_ref, r):
        ss = ss + TINY
        inv = lax.rsqrt(ss)
        shape = (ss.shape[0], 128)
        inv_ref[r:r + shape[0], :] = jnp.broadcast_to(inv, shape)
        norm = jnp.broadcast_to(ss * inv, shape)
        s_ref[r:r + shape[0], :] = norm
        return norm

    def qkv_skew(i, r0=0, r1=D):
        def gen(group=4):
            lane = lax.broadcasted_iota(jnp.int32, (8, 128), 1)
            bits = [(lane & (1 << b)) != 0 for b in range(3)]
            for g0 in range(r0 // 16, r1 // 16, group):
                xs = [[None] * NC for _ in range(group)]
                for c in range(NC):
                    for g in range(group):
                        rows = slice((g0 + g) * 16, (g0 + g + 1) * 16)
                        u, = gate(pltpu.bitcast(wqkv_raw[i, rows, c * 128:(c + 1) * 128], u32))
                        xs[g][c] = pltpu.roll(u, c, 1) if c else u
                for g in range(group):
                    ws = [xs[g][(-c) % NC] for c in range(NC)]
                    for b in range(3):
                        ws = [jnp.where(bits[b], ws[(c - (1 << b)) % NC], ws[c]) for c in range(NC)]
                    for c in range(NC):
                        w_tmp[c, (g0 + g) * 8:(g0 + g + 1) * 8, :] = ws[c]
                yield ws[0]
        return _Phase((r1 - r0) // 64, gen())

    def gather_lanes(c, r0):
        lane = lax.broadcasted_iota(jnp.int32, (64, 128), 1)
        base = (lane & 3) * 32 + (lane >> 5) * 8 + ((lane >> 2) & 7)
        for r in range(r0 // 2, r0 // 2 + D // 4, 64):
            u, = gate(w_tmp[c, r:r + 64, :])
            u = jnp.take_along_axis(u, (base + c) & 127, axis=1)
            w_tmp[c, r:r + 64, :] = u
        return u

    def qkv_finish(dst, j0, j1):
        def gen():
            for j in range(j0, j1):
                left, right = j, NC // 2 + j
                for c in (left, right):
                    gather_lanes(c, 0)
                    yield gather_lanes(c, D // 2)
                for r in range(0, D // 4, 16):
                    top, bot = slice(r, r + 16), slice(D // 4 + r, D // 4 + r + 16)
                    last = store_b7(dst, r, j * 128, w_tmp[left, top, :], w_tmp[right, top, :],
                                    w_tmp[left, bot, :], w_tmp[right, bot, :])
                yield last
        return _Phase(3 * (j1 - j0), gen())

    def wo_stage():
        def gen():
            for n in range(NC):
                for g in range(D // 64):
                    u, = gate(pltpu.bitcast(wo_raw[64 * g:64 * (g + 1), n * 128:(n + 1) * 128], u32))
                    wo_tmp[n, pl.ds(PAD * g, 32), :] = u
                    if g % 4 == 3:
                        yield u
        return _Phase(NC * 4, gen())

    def wo_finish():
        def rows16(n, cp, a):
            start = PAD * 8 * (a % 2) + 4 * (a // 2) + cp
            lo = wo_tmp[n, pl.ds(start, 8, stride=PAD), :]
            hi = wo_tmp[n, pl.ds(start + 16, 8, stride=PAD), :]
            return (lo & u32(0xFFFF)) | (hi << 16), (lo >> 16) | (hi & u32(0xFFFF0000))

        def gen():
            for j in range(NC // 2):
                for cp in range(NC // 4):
                    for a in range(8):
                        u11, u12 = rows16(j, cp, a), rows16(NC // 2 + j, cp, a)
                        u21, u22 = rows16(j, NC // 4 + cp, a), rows16(NC // 2 + j, NC // 4 + cp, a)
                        u11, u22 = gate(*u11), gate(*u22)
                        for odd in range(2):
                            last = store_b7(wo7, (2 * cp + odd) * 64 + 8 * a, j * 128,
                                            u11[odd], u12[odd], u21[odd], u22[odd])
                        if a % 2:
                            yield last
        return _Phase(NC * NC // 2, gen())

    def ffn_prepare(raw, dst, j0, j1, rows=32):
        kh, nh = raw.shape[0] // 2, raw.shape[1] // 2

        def gen():
            for c in range(j0 * 128, j1 * 128, 256):
                for r in range(0, kh, rows):
                    q = [raw[r0:r0 + rows, c0:c0 + 256] for r0 in (r, kh + r) for c0 in (c, nh + c)]
                    q[0], q[3] = gate(pltpu.bitcast(q[0], u32), pltpu.bitcast(q[3], u32))
                    yield store_b7(dst, r // 2, c, *q)
        return _Phase((j1 - j0) // 2 * kh // rows, gen())

    def layernorm(t, a7, s_ref):
        def gen():
            for r in range(0, T, 16):
                rows = pl.ds(pl.multiple_of(t * T + r, 16), 16)
                acc = None
                for c in range(NC):
                    x = xb[rows, c * 128:(c + 1) * 128]
                    if c == 0:
                        x, = gate(x)
                    acc = x.astype(f32) if acc is None else acc + x.astype(f32)
                mean = jnp.broadcast_to(jnp.sum(acc, axis=-1, keepdims=True) * (1.0 / D), (16, 128))
                yield mean
                mean, = gate(mean)
                acc = None
                for c in range(NC):
                    xc = xb[rows, c * 128:(c + 1) * 128].astype(f32) - mean
                    stage[c, r:r + 16, :] = xc
                    acc = xc * xc if acc is None else acc + xc * xc
                var = jnp.sum(acc, axis=-1, keepdims=True) * (1.0 / D)
                inv = lax.rsqrt(var + TINY)
                stage_inv[r:r + 16, :] = jnp.broadcast_to(inv, (16, 128))
                scale = jnp.broadcast_to((var + TINY) * inv * lax.rsqrt(var + EPS), (16, 128))
                s_ref[r:r + 16, :] = scale
                yield scale
            yield from a7_pieces(stage, stage_inv, a7)
        return _Phase(2 * T // 16 + TH // 16 * NC // 2, gen())

    def project(a7, s_ref, b7, dst, row0):
        def emit(half, c, y):
            dst[c, pl.ds(row0 + half * TH, TH), :] = y * s_ref[half * TH:(half + 1) * TH, :]
        return matmul(a7, b7, emit)

    def plain_lhs():
        for r in range(0, TH, 16):
            for j in range(NC // 2):
                at = (slice(r // 2, r // 2 + 8), slice(j * 128, (j + 1) * 128))
                ob7[(0,) + at] = _pack_rows(stage[NC // 2 + j, r:r + 16, :] * stage_inv[r:r + 16, :])
                ob7[(1,) + at] = _pack_rows(stage[j, TH + r:TH + r + 16, :] * stage_inv[TH + r:TH + r + 16, :])

    def first_q(k_half):
        def gen():
            blocks = (ob7[0], xa7[3]) if k_half else (xa7[2], ob7[1])
            for c in range(NC):
                lhs = jnp.concatenate([sched.hold(blocks[0]), blocks[1]], axis=0)
                rhs = w_tmp[c, k_half * (D // 4):(k_half + 1) * (D // 4), :]
                y = lax.dot_general(_as_bf16(lhs), _as_bf16(rhs), (((1,), (0,)), ((), ())),
                                    preferred_element_type=f32)
                sched.results.append(y)
                qa[c] = (qa[c] + y) * sa[...] if k_half else y
                yield
        return _Phase(NC, gen())

    def gather_bottom(c0, c1):
        return _Phase(c1 - c0, (gather_lanes(c, D // 2) for c in range(c0, c1)))

    def qkv_combine(dst):
        def gen():
            for j in range(NC // 2):
                for r in range(0, D // 4, 16):
                    q = [w_tmp[c, r0:r0 + 16, :] for r0 in (r, D // 4 + r) for c in (j, NC // 2 + j)]
                    q[0], q[3] = gate(q[0], q[3])
                    last = store_b7(dst, r, j * 128, *q)
                    if r % 64 == 48:
                        yield last
        return _Phase(NC * 2, gen())

    def attn_scores(q, row0, first, r0, r1, chunks):
        def gen():
            for r in range(r0, r1, 8):
                ls = [None] * W
                for c in range(NC):
                    qv, = gate(q[c, r:r + 8, :])
                    for w in range(W):
                        t = qv * kk[c, pl.ds(HALO + row0 + r - DIL * w, 8), :]
                        ls[w] = t if ls[w] is None else ls[w] + t
                    if c % chunks == chunks - 1 and c != NC - 1:
                        yield None
                for w in range(W):
                    t = ls[w] + pltpu.roll(ls[w], 64, 1)
                    t = t + pltpu.roll(t, 32, 1)
                    if first is not None and r < DIL * w:
                        row = lax.broadcasted_iota(jnp.int32, (8, 128), 0) + r
                        t = jnp.where(row < first * (DIL * w), MASKED / SCALE, t)
                    ls[w] = t
                m = ls[0]
                for w in range(1, W):
                    m = jnp.maximum(m, ls[w])
                es = [jnp.exp2((t - m) * (SCALE * LOG2E)) for t in ls]
                total = es[0]
                for w in range(1, W):
                    total = total + es[w]
                inv = 1.0 / total
                for w in range(W):
                    pp[w, r:r + 8, :] = es[w] * inv
                yield inv
        return _Phase((r1 - r0) // 8 * (NC // chunks), gen())

    def attn_mix(row0, o7, s_ref, r0, r1, chunks):
        def gen():
            for r in range(r0, r1, 8):
                ps = [pp[w, r:r + 8, :] for w in range(W)]
                ss = None
                for c in range(NC):
                    if c % chunks == 0:
                        ps = gate(*ps)
                    acc = None
                    for w in range(W):
                        t = ps[w] * vv[c, pl.ds(HALO + row0 + r - DIL * w, 8), :]
                        acc = t if acc is None else acc + t
                    stage[c, r:r + 8, :] = acc
                    ss = acc * acc if ss is None else ss + acc * acc
                    if c % chunks == chunks - 1 and c != NC - 1:
                        yield None
                yield store_row_norm(jnp.sum(ss, axis=-1, keepdims=True), stage_inv, s_ref, r)
            if r1 == T:
                yield from a7_pieces(stage, stage_inv, o7)
        return _Phase((r1 - r0) // 8 * (NC // chunks) + (TH // 16 * NC // 2 if r1 == T else 0), gen())

    def add_residual(t, a7, s_ref, b7, bias_row):
        def emit(half, c, y):
            rows = pl.ds(pl.multiple_of(t * T + half * TH, TH), TH)
            cols = slice(c * 128, (c + 1) * 128)
            z = y * s_ref[half * TH:(half + 1) * TH, :]
            if bias_row is not None:
                z = z + bias[bias_row + c:bias_row + c + 1, :]
            xb[rows, cols] = (xb[rows, cols].astype(f32) + z).astype(bf16)
        return matmul(a7, b7, emit)

    def attn_out(t, o7, s_ref):
        return add_residual(t, o7, s_ref, wo7, None)

    def ffn_up(j0=0, j1=NF // 2, a7=xf7, s_ref=sf):
        started = [j0 > 0, j0 > 0]

        def emit(half, c, y):
            rows = slice(half * TH, (half + 1) * TH)
            z = jnp.maximum(y * s_ref[rows, :] + bias[c:c + 1, :], 0.0)
            z = z * z
            h_stage[c, rows, :] = z
            h_ss[rows, :] = h_ss[rows, :] + z * z if started[half] else z * z
            started[half] = True
        return matmul(a7, w17, emit, j0, j1)

    def ffn_mid(h7=ha7, s_ref=sh):
        def gen():
            for r in range(0, T, 32):
                ss, = gate(h_ss[r:r + 32, :])
                yield store_row_norm(jnp.sum(ss, axis=-1, keepdims=True), h_inv, s_ref, r)
            yield from a7_pieces(h_stage, h_inv, h7)
        return _Phase(T // 32 + TH // 16 * NF // 2, gen())

    def ffn_down(t, h7=ha7, s_ref=sh):
        return add_residual(t, h7, s_ref, w27, 32)

    def move_halo(ref, src, dst):
        for c in range(NC):
            ref[c, pl.ds(dst, HALO), :] = ref[c, pl.ds(src, HALO), :]

    k0, k1, k2 = HALO, HALO + T, HALO + 2 * T
    wait(x_copy(0))
    solo(layernorm(0, xa7, sa))
    plain_lhs()
    wait(wq_copy(0))
    solo(qkv_skew(0, 0, D // 2))
    for c in range(NC):
        gather_lanes(c, 0)
    solo(first_q(0))
    wait(wq_copy(1))
    solo(qkv_skew(0, D // 2, D), gather_bottom(0, 2))
    wait(x_copy(1))
    run(first_q(1), _mix(layernorm(1, xb7, sb), _chain(gather_bottom(2, NC), qkv_combine(wq7))), lead=0, lag=9)
    q1 = project(xb7, sb, wq7, qb, 0)
    solo(_take(q1, 1))
    wait(wkv_copy(1))
    run(_chain(_take(q1, 3), project(xa7, sa, wk7, kk, k0)), qkv_skew(1), qkv_finish(wk7, 0, 4), lead=3, lag=2)
    for c in range(NC):
        kk[c, 0:HALO, :] = jnp.zeros((HALO, 128), f32)
    wait(x_copy(2))
    run(project(xb7, sb, wk7, kk, k1), layernorm(2, xf7, sf), attn_scores(qa, 0, 1, 0, 160, 4), lag=9)
    wait(wkv_copy(2))
    run(project(xf7, sf, wk7, kk, k2), qkv_skew(2), qkv_finish(wv7, 0, 2), lead=0)
    wait(wo_copy)
    run(project(xa7, sa, wv7, vv, k0), qkv_finish(wv7, 2, 4), attn_scores(qa, 0, 1, 160, T, 4), wo_stage(), lead=0)
    for c in range(NC):
        vv[c, 0:HALO, :] = jnp.broadcast_to(vv[c, HALO:HALO + 1, :], (HALO, 128))
    wait(x_copy(3))
    run(project(xb7, sb, wv7, vv, k1), wo_finish(), attn_mix(0, oa7, soa, 0, 160, 4), lead=0, lag=9)
    run(project(xf7, sf, wq7, qa, 0), attn_mix(0, oa7, soa, 160, T, 4), attn_scores(qb, T, None, 0, 192, 4),
        lead=0, lag=9)
    wait(b1_copy)
    wait(b2_copy)
    wait(w1_copy)
    bias[0:NF, :] = b1_raw[...].astype(f32)
    bias[32:32 + NC, :] = b2_raw[...].astype(f32)
    run(project(xf7, sf, wv7, vv, k2), attn_scores(qb, T, None, 192, T, 4), attn_mix(T, ob7, sob, 0, 96, 4),
        ffn_prepare(w1_raw, w17, 0, 4, 16), lead=0)
    run(attn_out(0, oa7, soa), attn_mix(T, ob7, sob, 96, T, 4), ffn_prepare(w1_raw, w17, 4, 6, 16), lead=0)
    run(attn_out(1, ob7, sob), _mix(layernorm(0, xf7, sf), ffn_prepare(w1_raw, w17, 6, 8)), lead=0, lag=2)
    run(ffn_up(0, 6), ffn_prepare(w1_raw, w17, 8, NF // 2), attn_scores(qa, 2 * T, None, 0, T, 4),
        attn_mix(2 * T, oa7, soa, 0, 224, 4), lead=0, lag=9)
    move_halo(kk, 3 * T, T)
    wait(w2_copy)
    run(ffn_up(6, UP_SPLIT), attn_mix(2 * T, oa7, soa, 224, T, 4), layernorm(3, xa7, sa),
        ffn_prepare(w2_raw, w27, 0, 2, 16), lead=0)
    move_halo(vv, 3 * T, T)
    run(attn_out(2, oa7, soa), ffn_prepare(w2_raw, w27, 2, NC // 2, 16), lead=0)

    sched.barrier()
    tuning[:] = 1024, 1

    def step(i, _):
        t_attn = (i + SKEW) % NT
        first = (t_attn == 0).astype(jnp.int32)

        @pl.when(i + SKEW + 1 < NT)
        def _():
            x_copy(i + SKEW + 1).wait()

        move_halo(kk, T, 0)
        move_halo(vv, T, 0)
        solo(ffn_up(UP_SPLIT))
        run(_chain(project(xa7, sa, wq7, qa, 0), project(xa7, sa, wk7, kk, k0)),
            layernorm((i + 1) % NT, xf7, sf), ffn_mid(), lag=2)
        run(project(xa7, sa, wv7, vv, k0), attn_scores(qa, 0, first, 0, 112, 8), lead=0, lag=2)
        for c in range(NC):
            v0 = jnp.broadcast_to(vv[c, HALO:HALO + 1, :], (HALO, 128))
            vv[c, 0:HALO, :] = jnp.where(t_attn == 0, v0, vv[c, 0:HALO, :])
        run(ffn_down(i % NT), attn_scores(qa, 0, first, 112, T, 4), attn_mix(0, oa7, soa, 0, T, 4), lag=2)
        solo(attn_out(t_attn, oa7, soa))
        run(ffn_up(0, UP_SPLIT), layernorm((i + SKEW + 1) % NT, xa7, sa), lead=4)
        sched.barrier()

        @pl.when(i >= NT)
        def _():
            o_copy(i - NT).start()
        return 0

    lax.fori_loop(0, 2 * NT - SKEW, step, 0)

    down_a, down_b = ffn_down(NT - 3), ffn_down(NT - 2, hb7, sob)
    solo(ffn_up(UP_SPLIT), ffn_mid())
    run(_take(down_a, 2), layernorm(NT - 2, xf7, sf), lead=0)
    run(ffn_up(), layernorm(NT - 1, xa7, sa), lead=6)
    run(_chain(_take(down_a, 2), _take(down_b, 1)), ffn_mid(hb7, sob), lead=2)
    solo(ffn_up(a7=xa7, s_ref=sa))
    run(_take(down_b, 3), ffn_mid(), lead=0)
    sched.barrier()
    o_copy(NT - 3).start()
    o_copy(NT - 2).start()
    down_c = ffn_down(NT - 1)
    last = []
    for j in range(NC // 2):
        solo(_take(down_c, 1))
        for c in (j, NC // 2 + j):
            at = (pl.ds((NT - 1) * T, T), pl.ds(c * 128, 128))
            last.append(pltpu.make_async_copy(xb.at[at], o_hbm.at[at], sem_o.at[NT - 1 + c]))
            last[-1].start()
    for copy in [o_copy(t) for t in range(NT - 1)] + last:
        copy.wait()


def _scratch_shapes():
    vmem = pltpu.VMEM
    lhs = vmem((7, T // 4, D // 2), u32)
    square = vmem((7, D // 4, D // 2), u32)
    per_row = vmem((T, 128), f32)
    chunks = vmem((NC, T, 128), f32)
    window = vmem((NC, HALO + 3 * T, 128), f32)
    return [
        vmem((S, D), bf16),
        vmem((3, D, D), bf16), vmem((D, D), bf16),
        vmem((D, F), bf16), vmem((F, D), bf16),
        vmem((NF, 128), bf16), vmem((NC, 128), bf16),
        vmem((NC, D // 2, 128), u32),
        vmem((NC, PAD * D // 64, 128), u32),
        square, square, square, square,
        vmem((7, D // 4, F // 2), u32), vmem((7, F // 4, D // 2), u32),
        vmem((40, 128), f32),
        lhs, lhs, lhs, lhs, lhs,
        vmem((7, T // 4, F // 2), u32), vmem((7, T // 4, F // 2), u32),
        per_row, per_row, per_row, per_row, per_row, per_row,
        chunks, per_row, vmem((NF, T, 128), f32), per_row, per_row,
        chunks, chunks, window, window, vmem((W, T, 128), f32),
        vmem((8, 128), u32),
        pltpu.SemaphoreType.DMA((NT,)), pltpu.SemaphoreType.DMA((9,)), pltpu.SemaphoreType.DMA((NT + NC,)),
    ]


@jax.jit
def pallas_interleave_layers__sliding_local_dilated__dense_activation_squared_relu__prompt_kernel(
    A_x: jax.Array,
    A_wqkv: jax.Array,
    A_wo: jax.Array,
    B_x: jax.Array,
    B_w1: jax.Array,
    B_b1: jax.Array,
    B_w2: jax.Array,
    B_b2: jax.Array,
):
    del B_x
    hbm = pl.BlockSpec(memory_space=pl.ANY)
    out = pl.pallas_call(
        _kernel,
        in_specs=[hbm] * 7,
        out_specs=hbm,
        out_shape=jax.ShapeDtypeStruct((S, D), bf16),
        scratch_shapes=_scratch_shapes(),
        compiler_params=pltpu.CompilerParams(vmem_limit_bytes=110 * 2 ** 20),
    )(A_x.reshape(S, D), A_wqkv, A_wo, B_w1, B_b1.reshape(NF, 128), B_w2, B_b2.reshape(NC, 128))
    return out.reshape(1, S, D)
```
